```python
import jax
import jax.numpy as jnp

def _softmax(x, axis=-1):
    return jax.nn.softmax(x, axis=axis)
def _gelu(x):
    return jax.nn.gelu(x, approximate=True)
def _silu(x):
    return jax.nn.silu(x)
def _sigmoid(x):
    return jax.nn.sigmoid(x)
def _layernorm(x, axis=-1, eps=1e-5):
    m = jnp.mean(x, axis=axis, keepdims=True)
    v = jnp.var(x, axis=axis, keepdims=True)
    return (x - m) / jnp.sqrt(v + eps)
def _scatter_add(tgt, idx, src, axis=0):
    return tgt.at[idx].add(src)
def _segment_sum(src, seg, n):
    return jax.ops.segment_sum(src, seg, n)
class _Rng:
    def __init__(self, key):
        self._k = key
    def _next(self):
        self._k, sub = jax.random.split(self._k)
        return sub
    def normal(self, shape):
        return jax.random.normal(self._next(), shape, dtype=jnp.bfloat16)
    def randint(self, lo, hi, shape):
        return jax.random.randint(self._next(), shape, lo, hi, dtype=jnp.int32)
    def uniform(self, shape, lo=0.0, hi=1.0):
        return jax.random.uniform(self._next(), shape, jnp.bfloat16, lo, hi)
    def permutation(self, n):
        return jax.random.permutation(self._next(), n)


kernel_name = 'concat_heads__linear_attn_block__ssm_conv_h3__prompt'

def setup_inputs():
    _rng = _Rng(jax.random.key(int.from_bytes(__import__("os").urandom(4), "little")))
    _w = (lambda a: (lambda t: t.astype(jnp.bfloat16) if jnp.issubdtype(t.dtype, jnp.floating) else t)(jnp.asarray(a)))
    def _A_setup():
        B, S, D = 1, 2048, 1024
        return {
            "x": _w((lambda *s: _rng.normal(s) * 0.05)(B, S, D)),
            "wqkv": _w((lambda *s: _rng.normal(s) * 0.05)(D, 3 * D)),
            "wo": _w((lambda *s: _rng.normal(s) * 0.05)(D, D)),
        }
    _A_in = _A_setup()

    def _B_setup():
        B, S, D = 1, 2048, 1024
        ks = 4
        return {
            "q": _w((lambda *s: _rng.normal(s) * 0.05)(B, S, D)),
            "k": _w((lambda *s: _rng.normal(s) * 0.05)(B, S, D)),
            "v": _w((lambda *s: _rng.normal(s) * 0.05)(B, S, D)),
            "shift_k": _w((lambda *s: _rng.normal(s) * 0.05)(D, ks) * 0.5),
            "ssm_k": _w((lambda *s: _rng.normal(s) * 0.05)(D, S) * (1.0 / S ** 0.5)),
            "ssm_D": _w((lambda *s: _rng.normal(s) * 0.05)(D)),
        }
    _B_in = _B_setup()

    return {
        "A_x": _A_in["x"],
        "A_wqkv": _A_in["wqkv"],
        "A_wo": _A_in["wo"],
        "B_q": _B_in["q"],
        "B_k": _B_in["k"],
        "B_v": _B_in["v"],
        "B_shift_k": _B_in["shift_k"],
        "B_ssm_k": _B_in["ssm_k"],
        "B_ssm_D": _B_in["ssm_D"],
    }

def reference(A_x, A_wqkv, A_wo, B_q, B_k, B_v, B_shift_k, B_ssm_k, B_ssm_D):
    def _A_ref(x, wqkv, wo):
        B, S, D = x.shape
        H = 32; Dh = D // H
        qkv = (lambda x, *d: x.transpose(*d))((x @ wqkv).reshape(B, S, 3, H, Dh), 2, 0, 3, 1, 4)
        q, k, v = qkv[0], qkv[1], qkv[2]
        phi = lambda t: jnp.where(t > 0, t + 1, jnp.exp(t)) + 1e-6
        pq, pk = phi(q), phi(k)
        kv = jnp.einsum("bhsd,bhse->bhde", pk, v)
        z = jnp.einsum("bhsd->bhd", pk)
        num = jnp.einsum("bhqd,bhde->bhqe", pq, kv)
        den = jnp.einsum("bhqd,bhd->bhq", pq, z)[..., None] + 1e-6
        o = num / den
        return (lambda x, *d: x.transpose(*d))(o, 0, 2, 1, 3).reshape(B, S, D) @ wo

    def _B_ref(q, k, v, shift_k, ssm_k, ssm_D):
        B, S, D = q.shape
        ks = shift_k.shape[-1]
        k_pad = jnp.pad(k, ((0, 0), (ks - 1, 0), (0, 0)))
        k_shift = jnp.zeros_like(k)
        for t in range(ks):
            k_shift = k_shift + k_pad[:, t:t + S, :] * shift_k[:, ks - 1 - t][None, None, :]
        kv = k_shift * v
        L = 2 * S
        kv_pad = jnp.pad(kv, ((0, 0), (0, S), (0, 0)))
        kf_pad = jnp.pad(ssm_k, ((0, 0), (0, S)))
        kv_f = (lambda x, axes=(-2,-1): jnp.fft.rfft2(x.astype(jnp.float32), axes=axes))(kv_pad[:, None, :, :], axes=(1, 2))
        kf_f = (lambda x, axes=(-2,-1): jnp.fft.rfft2(x.astype(jnp.float32), axes=axes))(kf_pad[:, None, :], axes=(1, 2))
        kf_f = (lambda x, *d: x.transpose(*d))(kf_f, 1, 2, 0)
        y_f = kv_f * kf_f[None, :, :, :]
        y = (lambda x, s, axes=(-2,-1): jnp.fft.irfft2(x, s=s, axes=axes).astype(jnp.bfloat16))(y_f, (1, L), axes=(1, 2))[:, 0, :S, :]
        y = y + kv * ssm_D[None, None, :]
        return q * y

    a = _A_ref(A_x, A_wqkv, A_wo)
    b = _B_ref(B_q, B_k, B_v, B_shift_k, B_ssm_k, B_ssm_D)
    return jnp.concatenate([a, b], axis=-1)
```

```python
import jax
import jax.numpy as jnp
import numpy as np
from jax import lax
import jax.experimental.pallas as pl
import jax.experimental.pallas.tpu as pltpu

S = 2048
D = 1024
DH = 32
C = 128
NB = S // C
NG = D // 128
ST = 512
NT = S // ST
HALO = 16

F32 = jnp.float32
BF16 = jnp.bfloat16


def _dft_matrices():
    n = np.arange(C, dtype=np.float64)
    theta = np.pi * (4.0 * np.arange(C, dtype=np.float64) + 1.0) / (2.0 * C)
    ang = theta[:, None] * n[None, :]
    fwd = np.concatenate([np.cos(ang), -np.sin(ang)], 0)
    inv = np.stack([np.cos(ang).T.reshape(C, C // 8, 8),
                    -np.sin(ang).T.reshape(C, C // 8, 8)], axis=2).reshape(C, 2 * C) / C
    return fwd.astype(np.float32), inv.astype(np.float32)


_FWD, _INV = _dft_matrices()

_NT_DIMS = (((1,), (1,)), ((), ()))
_TN_DIMS = (((0,), (0,)), ((), ()))


def _phi(t):
    return jnp.where(t > 0, t + 1.0, jnp.exp(t)) + 1e-6


def _unpack(words, index):
    return pltpu.unpack_elementwise(words, index=index, packed_dtype=BF16, unpacked_dtype=F32)


def _interleave(*streams):
    streams = [s for s in streams]
    live = [True] * len(streams)
    done = [0] * len(streams)
    total = max(n for _, n in streams)
    for step in range(1, total + 1):
        for i, (gen, n) in enumerate(streams):
            while live[i] and done[i] * total < step * n:
                try:
                    next(gen)
                    done[i] += 1
                except StopIteration:
                    live[i] = False
    for gen, _ in streams:
        for _ in gen:
            pass


def _conv_group(g, slot, kb, vb, qb, skb, shift_ref, d_ref, fwd_ref, inv_ref,
                kv_s, xp, kp, z_s, ob):
    lanes = pl.ds(pl.multiple_of(g * 128, 128), 128)
    w = shift_ref[:, lanes].astype(F32)
    w0, w1, w2, w3 = (jnp.broadcast_to(w[j:j + 1], (8, 128)) for j in range(4))
    skip = jnp.broadcast_to(d_ref[:, lanes].astype(F32), (C, 128))
    kw = kb.bitcast(jnp.uint32)
    vw = vb.bitcast(jnp.uint32)
    kvw = kv_s.bitcast(jnp.uint32)

    prev = None
    for m0 in range(0, NB, 4):
        blk = jnp.concatenate([skb[slot, :, (m0 + j) * C:(m0 + j + 1) * C] for j in range(4)], 0)
        spec = lax.dot_general(fwd_ref[...], blk, _NT_DIMS, preferred_element_type=F32)
        for j in range(4):
            re = spec[:C, j * 128:(j + 1) * 128]
            im = spec[C:, j * 128:(j + 1) * 128]
            if prev is None:
                re = re + skip
                re2, im2 = re, im
            else:
                re2, im2 = re - prev[1], im + prev[0]
            prev = (re, im)
            kp[0, m0 + j] = re2
            kp[1, m0 + j] = im2 - re2
            kp[2, m0 + j] = im2 + re2
        yield

    for c in range(NB):
        for i in range(c * C // 16, (c + 1) * C // 16):
            base = HALO // 2 + 8 * i
            p0 = kw[slot, base:base + 8, :]
            p1 = kw[slot, base - 1:base + 7, :]
            p2 = kw[slot, base - 2:base + 6, :]
            pv = vw[slot, 8 * i:8 * i + 8, :]
            e0, o0 = _unpack(p0, 0), _unpack(p0, 1)
            e1, o1 = _unpack(p1, 0), _unpack(p1, 1)
            o2 = _unpack(p2, 1)
            even = (w0 * e0 + w1 * o1 + w2 * e1 + w3 * o2) * _unpack(pv, 0)
            odd = (w0 * o0 + w1 * e0 + w2 * o1 + w3 * e1) * _unpack(pv, 1)
            kvw[8 * i:8 * i + 8, :] = pltpu.pack_elementwise(
                [even, odd], packed_dtype=BF16).astype(jnp.uint32)
        if c % 4 == 3:
            c0 = c - 3
            blk = jnp.concatenate([kv_s[(c0 + j) * C:(c0 + j + 1) * C, :] for j in range(4)], 1)
            spec = jnp.dot(fwd_ref[...], blk, preferred_element_type=F32)
            for j in range(4):
                re = spec[:C, j * 128:(j + 1) * 128]
                im = spec[C:, j * 128:(j + 1) * 128]
                xp[0, c0 + j] = re + im
                xp[1, c0 + j] = re
                xp[2, c0 + j] = im
        yield

    for r in range(C // 8):
        rows = slice(8 * r, 8 * r + 8)

        def plane(p, init, sign):
            ks = [kp[p, m, rows, :] for m in range(NB)]
            acc = list(init)
            for c in range(NB):
                xc = xp[p, c, rows, :]
                for a in range(c, NB):
                    t = xc * ks[a - c]
                    if acc[a] is None:
                        acc[a] = t
                    else:
                        acc[a] = acc[a] + t if sign > 0 else acc[a] - t
            return acc

        p1 = plane(0, [None] * NB, 1)
        yield
        zi = plane(1, p1, 1)
        yield
        zr = plane(2, p1, -1)
        for a in range(NB):
            z_s[a, 16 * r:16 * r + 16, :] = jnp.concatenate([zr[a], zi[a]], 0).astype(BF16)
        yield

    for a0 in range(0, NB, 4):
        blk = jnp.concatenate([z_s[a0 + j] for j in range(4)], 1)
        y = jnp.dot(inv_ref[...], blk, preferred_element_type=F32)
        for j in range(4):
            rows = slice((a0 + j) * C, (a0 + j + 1) * C)
            ob[slot, rows, :] = (qb[slot, rows, :].astype(F32) * y[:, j * 128:(j + 1) * 128]).astype(BF16)
        yield


_CONV_CHUNKS = NB // 4 + NB + 3 * (C // 8) + NB // 4


def _kernel(x_hbm, wqkv_hbm, wo_hbm, q_hbm, k_hbm, v_hbm, shift_ref, sk_hbm, d_ref, fwd_ref, inv_ref,
            out_hbm,
            x_v, w_v, wo_v, wt, g_acc, z_acc, m_v, pk_s, oa,
            kb, vb, qb, skb, kv_s, xp, kp, z_s, ob,
            sem_x, sem_w, sem_b, sem_oa, sem_ob):

    def x_copy(t):
        rows = pl.ds(pl.multiple_of(t * ST, ST), ST)
        return pltpu.make_async_copy(x_hbm.at[rows, :], x_v.at[rows, :], sem_x.at[t])

    def w_copy(j):
        return pltpu.make_async_copy(wqkv_hbm.at[:, pl.ds(j * D, D)], w_v.at[j], sem_w.at[j])

    wo_copy = pltpu.make_async_copy(wo_hbm, wo_v, sem_w.at[3])

    def b_copies(g, slot):
        lanes = pl.ds(pl.multiple_of(g * 128, 128), 128)
        return (
            pltpu.make_async_copy(sk_hbm.at[lanes, :], skb.at[slot], sem_b.at[slot, 0]),
            pltpu.make_async_copy(k_hbm.at[:, lanes], kb.at[slot, pl.ds(HALO, S), :], sem_b.at[slot, 1]),
            pltpu.make_async_copy(v_hbm.at[:, lanes], vb.at[slot], sem_b.at[slot, 2]),
            pltpu.make_async_copy(q_hbm.at[:, lanes], qb.at[slot], sem_b.at[slot, 3]),
        )

    def oa_copy(t, slot):
        rows = pl.ds(pl.multiple_of(t * ST, ST), ST)
        return pltpu.make_async_copy(oa.at[slot], out_hbm.at[rows, pl.ds(0, D)], sem_oa.at[slot])

    def ob_copy(g, slot):
        lanes = pl.ds(pl.multiple_of(D + g * 128, 128), 128)
        return pltpu.make_async_copy(ob.at[slot], out_hbm.at[:, lanes], sem_ob.at[slot])

    def conv(g, slot):
        return _conv_group(g, slot, kb, vb, qb, skb, shift_ref, d_ref, fwd_ref, inv_ref,
                           kv_s, xp, kp, z_s, ob)

    def conv_begin(g, slot):
        @pl.when(g + 1 < NG)
        def _():
            for cp in b_copies(g + 1, 1 - slot):
                cp.start()
        for cp in b_copies(g, slot):
            cp.wait()

        @pl.when(g >= 2)
        def _():
            ob_copy(g - 2, slot).wait()

    def transpose_weight(j):
        for i in range(D // 128):
            wt[i * 128:(i + 1) * 128, :] = w_v[j, :, i * 128:(i + 1) * 128].T

    w_copy(1).start()
    x_copy(0).start()
    for cp in b_copies(0, 0):
        cp.start()
    for slot in range(2):
        kb[slot, 0:HALO, :] = jnp.zeros((HALO, 128), BF16)
    g_acc[...] = jnp.zeros_like(g_acc)
    z_acc[...] = jnp.zeros_like(z_acc)
    w_copy(1).wait()
    transpose_weight(1)

    def keys(t):
        rows = pl.ds(pl.multiple_of(t * ST, ST), ST)
        for n in range(ST // 128):
            xs = x_v[pl.ds(pl.multiple_of(t * ST + n * 128, 128), 128), :]
            pk = _phi(lax.dot_general(wt[...], xs, _NT_DIMS, preferred_element_type=F32))
            z_acc[...] += pk
            pk_s[:, n * 128:(n + 1) * 128] = pk.astype(BF16)
            yield
        for n in range(D // 256):
            cols = slice(n * 256, (n + 1) * 256)
            g_acc[:, cols] += jnp.dot(pk_s[...], x_v[rows, cols], preferred_element_type=F32)
            yield

    def phase1(t, carry):
        slot = t % 2

        @pl.when(t + 1 < NT)
        def _():
            x_copy(t + 1).start()

        @pl.when(t == 0)
        def _():
            w_copy(2).start()
            wo_copy.start()
            w_copy(0).start()

        conv_begin(t, slot)
        x_copy(t).wait()
        _interleave((keys(t), ST // 128 + D // 256), (conv(t, slot), _CONV_CHUNKS))
        ob_copy(t, slot).start()
        return carry

    lax.fori_loop(0, NT, phase1, 0)

    w_copy(2).wait()
    wo_copy.wait()
    w_copy(0).wait()
    same_head = (lax.broadcasted_iota(jnp.int32, (128, 128), 0) // DH
                 == lax.broadcasted_iota(jnp.int32, (128, 128), 1) // DH)
    for i in range(D // 128):
        blk = slice(i * 128, (i + 1) * 128)
        kv = jnp.dot(g_acc[blk, :].astype(BF16), w_v[2, :, blk], preferred_element_type=F32)
        kv = jnp.where(same_head, kv, 0.0).astype(BF16)
        m_v[blk, :] = jnp.dot(kv, wo_v[blk, :], preferred_element_type=F32).astype(BF16)
    z_acc[...] = jnp.broadcast_to(jnp.sum(z_acc[...], axis=1, keepdims=True), (D, 128))
    transpose_weight(0)

    def queries(t, slot):
        for n in range(ST // 128):
            xs = x_v[pl.ds(pl.multiple_of(t * ST + n * 128, 128), 128), :]
            pq = _phi(lax.dot_general(wt[...], xs, _NT_DIMS, preferred_element_type=F32))
            den = jnp.sum((pq * z_acc[...]).reshape(D // DH, DH, 128), axis=1, keepdims=True) + 1e-6
            o = pq.reshape(D // DH, DH, 128) * (1.0 / den)
            pk_s[:, n * 128:(n + 1) * 128] = o.reshape(D, 128).astype(BF16)
            yield
        for n in range(D // 256):
            cols = slice(n * 256, (n + 1) * 256)
            oa[slot, :, cols] = lax.dot_general(
                pk_s[...], m_v[:, cols], _TN_DIMS, preferred_element_type=F32).astype(BF16)
            yield

    def phase2(t, carry):
        slot = t % 2
        conv_begin(NT + t, slot)

        @pl.when(t >= 2)
        def _():
            oa_copy(t - 2, slot).wait()

        _interleave((queries(t, slot), ST // 128 + D // 256), (conv(NT + t, slot), _CONV_CHUNKS))
        oa_copy(t, slot).start()
        ob_copy(NT + t, slot).start()
        return carry

    lax.fori_loop(0, NT, phase2, 0)
    for t in range(NT - 2, NT):
        oa_copy(t, t % 2).wait()
        ob_copy(NT + t, t % 2).wait()


@jax.jit
def pallas_concat_heads__linear_attn_block__ssm_conv_h3__prompt_kernel(
    A_x: jax.Array,
    A_wqkv: jax.Array,
    A_wo: jax.Array,
    B_q: jax.Array,
    B_k: jax.Array,
    B_v: jax.Array,
    B_shift_k: jax.Array,
    B_ssm_k: jax.Array,
    B_ssm_D: jax.Array,
):
    assert A_x.shape == (1, S, D) and B_shift_k.shape == (D, 4) and NG == 2 * NT
    hbm = pl.BlockSpec(memory_space=pl.ANY)
    vmem = pl.BlockSpec(memory_space=pltpu.VMEM)
    out = pl.pallas_call(
        _kernel,
        out_shape=jax.ShapeDtypeStruct((S, 2 * D), BF16),
        in_specs=[hbm, hbm, hbm, hbm, hbm, hbm, vmem, hbm, vmem, vmem, vmem],
        out_specs=hbm,
        scratch_shapes=[
            pltpu.VMEM((S, D), BF16),
            pltpu.VMEM((3, D, D), BF16),
            pltpu.VMEM((D, D), BF16),
            pltpu.VMEM((D, D), BF16),
            pltpu.VMEM((D, D), F32),
            pltpu.VMEM((D, 128), F32),
            pltpu.VMEM((D, D), BF16),
            pltpu.VMEM((D, ST), BF16),
            pltpu.VMEM((2, ST, D), BF16),
            pltpu.VMEM((2, HALO + S, 128), BF16),
            pltpu.VMEM((2, S, 128), BF16),
            pltpu.VMEM((2, S, 128), BF16),
            pltpu.VMEM((2, 128, S), BF16),
            pltpu.VMEM((S, 128), BF16),
            pltpu.VMEM((3, NB, C, 128), F32),
            pltpu.VMEM((3, NB, C, 128), F32),
            pltpu.VMEM((NB, 2 * C, 128), BF16),
            pltpu.VMEM((2, S, 128), BF16),
            pltpu.SemaphoreType.DMA((NT,)),
            pltpu.SemaphoreType.DMA((4,)),
            pltpu.SemaphoreType.DMA((2, 4)),
            pltpu.SemaphoreType.DMA((2,)),
            pltpu.SemaphoreType.DMA((2,)),
        ],
        compiler_params=pltpu.CompilerParams(vmem_limit_bytes=100 * 2**20),
        name="linattn_h3",
    )(
        A_x.reshape(S, D), A_wqkv, A_wo,
        B_q.reshape(S, D), B_k.reshape(S, D), B_v.reshape(S, D),
        B_shift_k.T, B_ssm_k, B_ssm_D.reshape(1, D),
        jnp.asarray(_FWD, BF16), jnp.asarray(_INV, BF16),
    )
    return out.reshape(1, S, 2 * D)
```

```python
import jax
import jax.numpy as jnp
import numpy as np
from jax import lax
import jax.experimental.pallas as pl
import jax.experimental.pallas.tpu as pltpu

S = 2048
D = 1024
DH = 32
C = 128
NB = S // C
NG = D // 128
ST = 512
NT = S // ST
UNITS = 2 * (ST // 128) * (D // 128)
MAC_BLOCK = 16
HEAD_UNITS = 4
TAIL_UNITS = 7
PACE = True
PACE_EVERY = 1
OUT_PARTS = 8
HALO = 16

F32 = jnp.float32
BF16 = jnp.bfloat16


def _dft_matrices():
    n = np.arange(C, dtype=np.float64)
    theta = np.pi * (4.0 * np.arange(C, dtype=np.float64) + 1.0) / (2.0 * C)
    ang = theta[:, None] * n[None, :]
    fwd = np.concatenate([np.cos(ang), -np.sin(ang)], 0)
    inv = np.stack([np.cos(ang).T, -np.sin(ang).T], axis=2).reshape(C, 2 * C) / C
    inv = inv.reshape(C // 16, 8, 2, 2 * C).transpose(0, 2, 1, 3).reshape(C, 2 * C)
    return fwd.astype(np.float32), inv.astype(np.float32)


_FWD, _INV = _dft_matrices()

_NT_DIMS = (((1,), (1,)), ((), ()))
_TN_DIMS = (((0,), (0,)), ((), ()))


def _packed(*shape):
    return pltpu.VMEM((*shape[:-2], shape[-2] // 2, shape[-1]), jnp.uint32)


def _phi(t):
    return jnp.where(t > 0, t + 1.0, jnp.exp(t)) + 1e-6


def _unpack(words, index):
    return pltpu.unpack_elementwise(words, index=index, packed_dtype=BF16, unpacked_dtype=F32)


def _rows(start, size):
    if isinstance(start, int):
        return pl.ds(start // 2, size // 2)
    return pl.ds(pl.multiple_of(start // 2, 8), size // 2)


def _bf16(words):
    return pltpu.bitcast(words, BF16)


def _words(x):
    return pltpu.bitcast(x.astype(BF16), jnp.uint32)


def _pack(lo, hi):
    return pltpu.pack_elementwise([lo, hi], packed_dtype=BF16).astype(jnp.uint32)


def _riffle(x):
    return jnp.concatenate(
        [_pack(x[i:i + 8], x[i + 8:i + 16]) for i in range(0, x.shape[0], 16)], 0)


class _ConvGroup:
    def __init__(self, g, slot, kb, vb, qb, skb, shift_ref, d_ref, fwd_s, inv_s, kv_s, xp, kp, z_s, ob):
        self.slot, self.kb, self.vb, self.qb, self.skb = slot, kb, vb, qb, skb
        self.fwd_s, self.inv_s, self.kv_s, self.xp, self.kp, self.z_s, self.ob = (
            fwd_s, inv_s, kv_s, xp, kp, z_s, ob)
        lanes = pl.ds(pl.multiple_of(g * 128, 128), 128)
        w = shift_ref[:, lanes].astype(F32)
        self.taps = [jnp.broadcast_to(w[j:j + 1], (8, 128)) for j in range(4)]
        self.skip = d_ref[:, lanes].astype(F32)
        self.prev = None

    def filter_spectrum(self, i):
        blk = jnp.concatenate(
            [_bf16(self.skb[self.slot, :, m * C:(m + 1) * C]) for m in range(4 * i, 4 * i + 4)], 0)
        spec = lax.dot_general(_bf16(self.fwd_s[...]), blk, _NT_DIMS, preferred_element_type=F32)
        for j in range(4):
            re = spec[:C, j * 128:(j + 1) * 128]
            im = spec[C:, j * 128:(j + 1) * 128]
            if self.prev is None:
                re = re + self.skip
                re2, im2 = re, im
            else:
                re2, im2 = re - self.prev[1], im + self.prev[0]
            self.prev = (re, im)
            self.kp[0, 4 * i + j] = re2
            self.kp[1, 4 * i + j] = im2 - re2
            self.kp[2, 4 * i + j] = im2 + re2

    def gate_keys(self, lo, hi):
        w0, w1, w2, w3 = self.taps
        for i in range(lo, hi):
            base = HALO // 2 + 8 * i
            p0 = self.kb[self.slot, base:base + 8, :]
            p1 = self.kb[self.slot, base - 1:base + 7, :]
            p2 = self.kb[self.slot, base - 2:base + 6, :]
            pv = self.vb[self.slot, 8 * i:8 * i + 8, :]
            e0, o0 = _unpack(p0, 0), _unpack(p0, 1)
            e1, o1 = _unpack(p1, 0), _unpack(p1, 1)
            o2 = _unpack(p2, 1)
            even = (w0 * e0 + w1 * o1 + w2 * e1 + w3 * o2) * _unpack(pv, 0)
            odd = (w0 * o0 + w1 * e0 + w2 * o1 + w3 * e1) * _unpack(pv, 1)
            self.kv_s[8 * i:8 * i + 8, :] = _pack(even, odd)

    def signal_spectrum(self, i):
        blk = jnp.concatenate(
            [_bf16(self.kv_s[_rows(c * C, C), :]) for c in range(4 * i, 4 * i + 4)], 1)
        spec = jnp.dot(_bf16(self.fwd_s[...]), blk, preferred_element_type=F32)
        for j in range(4):
            re = spec[:C, j * 128:(j + 1) * 128]
            im = spec[C:, j * 128:(j + 1) * 128]
            self.xp[0, 4 * i + j] = re + im
            self.xp[1, 4 * i + j] = re
            self.xp[2, 4 * i + j] = im

    def combine(self):
        for r in range(C // 8):
            rows = slice(8 * r, 8 * r + 8)

            def plane(p, init, subtract):
                acc = list(init)
                for a0 in range(NB - MAC_BLOCK, -1, -MAC_BLOCK):
                    for c in range(a0 + MAC_BLOCK):
                        xc = self.xp[p, c, rows, :]
                        for a in range(max(c, a0), a0 + MAC_BLOCK):
                            t = xc * self.kp[p, a - c, rows, :]
                            if acc[a] is None:
                                acc[a] = t
                            else:
                                acc[a] = acc[a] - t if subtract else acc[a] + t
                            yield
                return acc

            p1 = yield from plane(0, [None] * NB, False)
            zi = yield from plane(1, p1, False)
            zr = yield from plane(2, p1, True)
            for a in range(NB):
                self.z_s[a, rows, :] = _pack(zr[a], zi[a])

    def finish(self, i):
        blk = jnp.concatenate([_bf16(self.z_s[a]) for a in range(4 * i, 4 * i + 4)], 1)
        y = jnp.dot(_bf16(self.inv_s[...]), blk, preferred_element_type=F32)
        for j in range(4):
            for u in range(C // 16):
                rows = _rows((4 * i + j) * C + 16 * u, 16)
                q = self.qb[self.slot, rows, :]
                self.ob[self.slot, rows, :] = _pack(
                    _unpack(q, 0) * y[16 * u:16 * u + 8, j * 128:(j + 1) * 128],
                    _unpack(q, 1) * y[16 * u + 8:16 * u + 16, j * 128:(j + 1) * 128])


def _run_step(matmuls, n_matmuls, conv, conv_done, pace):
    left = [n_matmuls]

    def matmul(paced=False):
        result = next(matmuls)
        if paced and PACE:
            pace(result[:8, :128])
        left[0] -= 1

    tiles = S // 16 // 4
    for i in range(4):
        conv.filter_spectrum(i)
        for u in range(HEAD_UNITS):
            matmul()
            if u == 0 and i > 0:
                conv.signal_spectrum(i - 1)
            conv.gate_keys(i * tiles + u * tiles // HEAD_UNITS, i * tiles + (u + 1) * tiles // HEAD_UNITS)
    matmul()
    conv.signal_spectrum(3)
    matmul()
    products = 3 * (C // 8) * NB * (NB + 1) // 2
    units = left[0] - TAIL_UNITS
    combine = conv.combine()
    for u in range(units):
        for _ in range(u * products // units, (u + 1) * products // units):
            next(combine)
        if u == units - 1:
            for _ in combine:
                pass
        matmul(paced=u % PACE_EVERY == 0)
    for i in range(4):
        conv.finish(i)
        if i == 3:
            conv_done()
        if left[0]:
            matmul()
    while left[0]:
        matmul()
    for _ in matmuls:
        pass


def _kernel(x_hbm, wqkv_hbm, wo_hbm, q_hbm, k_hbm, v_hbm, shift_ref, sk_hbm, d_ref, fwd_ref, inv_ref,
            out_hbm,
            x_v, w_v, wo_v, wkt, wqt, g_acc, z_acc, m_v, pk_s, o_s, oa, fwd_s, inv_s,
            kb, vb, qb, skb, kv_s, xp, kp, z_s, ob, zero,
            sem_x, sem_w, sem_wk, sem_b, sem_oa, sem_ob):

    def x_copy(t):
        rows = pl.ds(pl.multiple_of(t * ST, ST), ST)
        return pltpu.make_async_copy(x_hbm.at[rows, :], x_v.bitcast(BF16).at[rows, :], sem_x.at[t])

    def w_copy(j):
        return pltpu.make_async_copy(
            wqkv_hbm.at[:, pl.ds(j * D, D)], w_v.bitcast(BF16).at[j], sem_w.at[j])

    def wk_copy(i):
        return pltpu.make_async_copy(
            wqkv_hbm.at[:, pl.ds(D + i * 128, 128)], w_v.bitcast(BF16).at[1, :, pl.ds(i * 128, 128)],
            sem_wk.at[i])

    wo_copy = pltpu.make_async_copy(wo_hbm, wo_v.bitcast(BF16), sem_w.at[3])

    def b_copies(g, slot):
        lanes = pl.ds(pl.multiple_of(g * 128, 128), 128)
        return (
            pltpu.make_async_copy(sk_hbm.at[lanes, :], skb.bitcast(BF16).at[slot], sem_b.at[slot, 0]),
            pltpu.make_async_copy(
                k_hbm.at[:, lanes], kb.bitcast(BF16).at[slot, pl.ds(HALO, S), :], sem_b.at[slot, 1]),
            pltpu.make_async_copy(v_hbm.at[:, lanes], vb.bitcast(BF16).at[slot], sem_b.at[slot, 2]),
            pltpu.make_async_copy(q_hbm.at[:, lanes], qb.bitcast(BF16).at[slot], sem_b.at[slot, 3]),
        )

    def oa_copy(t, slot, n):
        rows = pl.ds(pl.multiple_of(t * ST, ST), ST)
        cols = pl.ds(n * (D // OUT_PARTS), D // OUT_PARTS)
        return pltpu.make_async_copy(oa.at[slot, :, cols], out_hbm.at[rows, cols], sem_oa.at[slot, n])

    def ob_copy(g, slot):
        lanes = pl.ds(pl.multiple_of(D + g * 128, 128), 128)
        return pltpu.make_async_copy(ob.bitcast(BF16).at[slot], out_hbm.at[:, lanes], sem_ob.at[slot])

    def conv(g, slot):
        return _ConvGroup(g, slot, kb, vb, qb, skb, shift_ref, d_ref, fwd_s, inv_s,
                           kv_s, xp, kp, z_s, ob)

    def conv_begin(g, slot):
        for cp in b_copies(g, slot):
            cp.wait()

        @pl.when(g + 1 < NG)
        def _():
            for cp in b_copies(g + 1, 1 - slot):
                cp.start()

        @pl.when(g >= 2)
        def _():
            ob_copy(g - 2, slot).wait()

    def transpose_weight(j, dst, i):
        dst[_rows(i * 128, 128), :] = _words(_bf16(w_v[j, :, i * 128:(i + 1) * 128]).T)

    def pace(tile):
        xp[3, 0, pl.ds(pl.multiple_of(zero[0], 8), 8), :] = tile

    zero[0] = 0
    for i in range(D // 128):
        wk_copy(i).start()
    x_copy(0).start()
    for cp in b_copies(0, 0):
        cp.start()
    for slot in range(2):
        kb[slot, 0:HALO // 2, :] = jnp.zeros((HALO // 2, 128), jnp.uint32)
    fwd_s[...] = _words(fwd_ref[...])
    inv_s[...] = _words(inv_ref[...])
    g_acc[...] = jnp.zeros_like(g_acc)
    z_acc[...] = jnp.zeros_like(z_acc)
    for i in range(D // 128):
        wk_copy(i).wait()
        transpose_weight(1, wkt, i)

    def keys(t):
        def project(j):
            w = _bf16(wkt[_rows(j * 128, 128), :])
            pk = []
            for n in range(ST // 128):
                xs = _bf16(x_v[_rows(t * ST + n * 128, 128), :])
                pk.append(_phi(lax.dot_general(w, xs, _NT_DIMS, preferred_element_type=F32)))
                if n == ST // 128 - 1:
                    z_acc[j * 128:(j + 1) * 128, :] += sum(pk[1:], pk[0])
                    pk_s[_rows(j * 128, 128), :] = _riffle(jnp.concatenate(pk, 1))
                yield pk[-1]

        def accumulate(j):
            for n in range(D // 256):
                cols = slice(n * 256, (n + 1) * 256)
                g = jnp.dot(_bf16(pk_s[_rows(j * 128, 128), :]), _bf16(x_v[_rows(t * ST, ST), cols]),
                            preferred_element_type=F32)
                g_acc[j * 128:(j + 1) * 128, cols] += g
                yield g

        yield from project(0)
        for j in range(1, D // 128):
            yield from project(j)
            yield from accumulate(j - 1)
        yield from accumulate(D // 128 - 1)

    def phase1(t, carry):
        slot = t % 2

        x_copy(t).wait()
        conv_begin(t, slot)

        @pl.when(t + 1 < NT)
        def _():
            x_copy(t + 1).start()

        @pl.when(t == 0)
        def _():
            w_copy(2).start()
            wo_copy.start()
            w_copy(0).start()

        _run_step(keys(t), UNITS, conv(t, slot), lambda: ob_copy(t, slot).start(), pace)
        return carry

    lax.fori_loop(0, NT, phase1, 0)

    w_copy(2).wait()
    wo_copy.wait()
    w_copy(0).wait()
    same_head = (lax.broadcasted_iota(jnp.int32, (128, 128), 0) // DH
                 == lax.broadcasted_iota(jnp.int32, (128, 128), 1) // DH)
    kvs = []
    for i in range(D // 128):
        blk = slice(i * 128, (i + 1) * 128)
        kv = jnp.dot(g_acc[blk, :].astype(BF16), _bf16(w_v[2, :, blk]), preferred_element_type=F32)
        kvs.append(jnp.where(same_head, kv, 0.0).astype(BF16))
        transpose_weight(0, wqt, i)
    for i in range(D // 128):
        m_v[_rows(i * 128, 128), :] = _words(
            jnp.dot(kvs[i], _bf16(wo_v[_rows(i * 128, 128), :]), preferred_element_type=F32))
    z_acc[...] = jnp.broadcast_to(jnp.sum(z_acc[...], axis=1, keepdims=True), (D, 128))

    def queries(t, slot):
        for n in range(ST // 128):
            xs = _bf16(x_v[_rows(t * ST + n * 128, 128), :])
            for j in range(D // 128):
                pq = _phi(lax.dot_general(
                    _bf16(wqt[_rows(j * 128, 128), :]), xs, _NT_DIMS, preferred_element_type=F32))
                pz = (pq * z_acc[j * 128:(j + 1) * 128, :]).reshape(128 // DH, DH, 128)
                den = jnp.sum(pz, axis=1, keepdims=True) + 1e-6
                o = (pq.reshape(128 // DH, DH, 128) * (1.0 / den)).reshape(128, 128)
                o_s[_rows(n * 128, 128), j * 128:(j + 1) * 128] = _words(_bf16(_riffle(o)).T)
                yield pq
        for j in range(D // 128):
            cols = slice(j * 128, (j + 1) * 128)
            for n in range(ST // 128):
                res = jnp.dot(_bf16(o_s[_rows(n * 128, 128), :]), _bf16(m_v[:, cols]),
                              preferred_element_type=F32)
                oa[slot, n * 128:(n + 1) * 128, cols] = res.astype(BF16)
                if n == ST // 128 - 1 and (j + 1) % (D // 128 // OUT_PARTS) == 0:
                    oa_copy(t, slot, j // (D // 128 // OUT_PARTS)).start()
                yield res

    def phase2(t, carry):
        slot = t % 2
        conv_begin(NT + t, slot)

        @pl.when(t >= 2)
        def _():
            for n in range(OUT_PARTS):
                oa_copy(t - 2, slot, n).wait()

        _run_step(queries(t, slot), UNITS, conv(NT + t, slot), lambda: ob_copy(NT + t, slot).start(), pace)
        return carry

    lax.fori_loop(0, NT, phase2, 0)
    for t in range(NT - 2, NT):
        ob_copy(NT + t, t % 2).wait()
        for n in range(OUT_PARTS):
            oa_copy(t, t % 2, n).wait()


@jax.jit
def pallas_concat_heads__linear_attn_block__ssm_conv_h3__prompt_kernel(
    A_x: jax.Array,
    A_wqkv: jax.Array,
    A_wo: jax.Array,
    B_q: jax.Array,
    B_k: jax.Array,
    B_v: jax.Array,
    B_shift_k: jax.Array,
    B_ssm_k: jax.Array,
    B_ssm_D: jax.Array,
):
    assert A_x.shape == (1, S, D) and B_shift_k.shape == (D, 4) and NG == 2 * NT
    hbm = pl.BlockSpec(memory_space=pl.ANY)
    vmem = pl.BlockSpec(memory_space=pltpu.VMEM)
    out = pl.pallas_call(
        _kernel,
        out_shape=jax.ShapeDtypeStruct((S, 2 * D), BF16),
        in_specs=[hbm, hbm, hbm, hbm, hbm, hbm, vmem, hbm, vmem, vmem, vmem],
        out_specs=hbm,
        scratch_shapes=[
            _packed(S, D),
            _packed(3, D, D),
            _packed(D, D),
            _packed(D, D),
            _packed(D, D),
            pltpu.VMEM((D, D), F32),
            pltpu.VMEM((D, 128), F32),
            _packed(D, D),
            _packed(D, ST),
            _packed(ST, D),
            pltpu.VMEM((2, ST, D), BF16),
            _packed(2 * C, C),
            _packed(C, 2 * C),
            _packed(2, HALO + S, 128),
            _packed(2, S, 128),
            _packed(2, S, 128),
            _packed(2, 128, S),
            _packed(S, 128),
            pltpu.VMEM((4, NB, C, 128), F32),
            pltpu.VMEM((3, NB, C, 128), F32),
            _packed(NB, 2 * C, 128),
            _packed(2, S, 128),
            pltpu.SMEM((1,), jnp.int32),
            pltpu.SemaphoreType.DMA((NT,)),
            pltpu.SemaphoreType.DMA((4,)),
            pltpu.SemaphoreType.DMA((D // 128,)),
            pltpu.SemaphoreType.DMA((2, 4)),
            pltpu.SemaphoreType.DMA((2, OUT_PARTS)),
            pltpu.SemaphoreType.DMA((2,)),
        ],
        compiler_params=pltpu.CompilerParams(vmem_limit_bytes=100 * 2**20),
        name="linattn_h3",
    )(
        A_x.reshape(S, D), A_wqkv, A_wo,
        B_q.reshape(S, D), B_k.reshape(S, D), B_v.reshape(S, D),
        B_shift_k.T, B_ssm_k, B_ssm_D.reshape(1, D),
        jnp.asarray(_FWD, BF16), jnp.asarray(_INV, BF16),
    )
    return out.reshape(1, S, 2 * D)
```

```python
import jax
import jax.numpy as jnp
import numpy as np
from jax import lax
import jax.experimental.pallas as pl
import jax.experimental.pallas.tpu as pltpu

S = 2048
D = 1024
DH = 32
C = 128
NB = S // C
NG = D // 128
ST = 512
NT = S // ST
UNITS = 2 * (ST // 128) * (D // 128)
HEAD1 = 4
TAIL1 = 4
HEAD2 = 4
TAIL2 = 7
FIRST_HEAD = 3
FIRST_TAIL = 4
PACE = True
PACE_EVERY = 1
K_ROWS = 256
G_COLS = 128
Q_ROWS = 256
O_ROWS = 256
O_COLS = 128
FIRST_CHUNKS = ((0, 128), (128, 128), (256, 256), (512, 256), (768, 256))
OUT_PARTS = D // O_COLS
FIRST_BATCHES = ((0, (0,)), (1, (1,)), (10, (2, 3)), (10 + 2 * FIRST_HEAD, (4, 5, 6, 7)))
HALO = 16

F32 = jnp.float32
BF16 = jnp.bfloat16


def _dft_matrices():
    n = np.arange(C, dtype=np.float64)
    theta = np.pi * (4.0 * np.arange(C, dtype=np.float64) + 1.0) / (2.0 * C)
    ang = theta[:, None] * n[None, :]
    fwd = np.concatenate([np.cos(ang), -np.sin(ang)], 0)
    inv = np.stack([np.cos(ang).T, -np.sin(ang).T], axis=2).reshape(C, 2 * C) / C
    inv = inv.reshape(C // 16, 8, 2, 2 * C).transpose(0, 2, 1, 3).reshape(C, 2 * C)
    return fwd.astype(np.float32), inv.astype(np.float32)


_FWD, _INV = _dft_matrices()

_NT_DIMS = (((1,), (1,)), ((), ()))
_TN_DIMS = (((0,), (0,)), ((), ()))


def _packed(*shape):
    return pltpu.VMEM((*shape[:-2], shape[-2] // 2, shape[-1]), jnp.uint32)


def _phi(t):
    return jnp.where(t > 0, t + 1.0, jnp.exp(t)) + 1e-6


def _unpack(words, index):
    return pltpu.unpack_elementwise(words, index=index, packed_dtype=BF16, unpacked_dtype=F32)


def _rows(start, size):
    if isinstance(start, int):
        return pl.ds(start // 2, size // 2)
    return pl.ds(pl.multiple_of(start // 2, 8), size // 2)


def _lanes(g):
    return pl.ds(g * 128 if isinstance(g, int) else pl.multiple_of(g * 128, 128), 128)


def _bf16(words):
    return pltpu.bitcast(words, BF16)


def _words(x):
    return pltpu.bitcast(x.astype(BF16), jnp.uint32)


def _pack(lo, hi):
    return pltpu.pack_elementwise([lo, hi], packed_dtype=BF16).astype(jnp.uint32)


def _riffle(x):
    return jnp.concatenate(
        [_pack(x[i:i + 8], x[i + 8:i + 16]) for i in range(0, x.shape[0], 16)], 0)


class _ConvGroup:
    def __init__(self, g, slot, kb, vb, qb, skb, shift_ref, d_ref, fwd_s, inv_s, kv_s, xp, kp, z_s, ob):
        self.slot, self.kb, self.vb, self.qb, self.skb = slot, kb, vb, qb, skb
        self.fwd_s, self.inv_s, self.kv_s, self.xp, self.kp, self.z_s, self.ob = (
            fwd_s, inv_s, kv_s, xp, kp, z_s, ob)
        lanes = _lanes(g)
        w = shift_ref[:, lanes].astype(F32)
        self.taps = [jnp.broadcast_to(w[j:j + 1], (8, 128)) for j in range(4)]
        self.skip = d_ref[:, lanes]
        self.prev = None

    def filter_spectrum(self, i):
        blk = jnp.concatenate(
            [_bf16(self.skb[self.slot, :, m * C:(m + 1) * C]) for m in range(4 * i, 4 * i + 4)], 0)
        spec = lax.dot_general(_bf16(self.fwd_s[...]), blk, _NT_DIMS, preferred_element_type=F32)
        for j in range(4):
            re = spec[:C, j * 128:(j + 1) * 128]
            im = spec[C:, j * 128:(j + 1) * 128]
            if self.prev is None:
                re = re + self.skip
                re2, im2 = re, im
            else:
                re2, im2 = re - self.prev[1], im + self.prev[0]
            self.prev = (re, im)
            self.kp[0, 4 * i + j] = re2
            self.kp[1, 4 * i + j] = im2

    def gate_keys(self, lo, hi):
        w0, w1, w2, w3 = self.taps
        for i in range(lo, hi):
            base = HALO // 2 + 8 * i
            p0 = self.kb[self.slot, base:base + 8, :]
            p1 = self.kb[self.slot, base - 1:base + 7, :]
            p2 = self.kb[self.slot, base - 2:base + 6, :]
            pv = self.vb[self.slot, 8 * i:8 * i + 8, :]
            e0, o0 = _unpack(p0, 0), _unpack(p0, 1)
            e1, o1 = _unpack(p1, 0), _unpack(p1, 1)
            o2 = _unpack(p2, 1)
            even = (w0 * e0 + w1 * o1 + w2 * e1 + w3 * o2) * _unpack(pv, 0)
            odd = (w0 * o0 + w1 * e0 + w2 * o1 + w3 * e1) * _unpack(pv, 1)
            self.kv_s[8 * i:8 * i + 8, :] = _pack(even, odd)

    def signal_spectrum(self, i):
        blk = jnp.concatenate(
            [_bf16(self.kv_s[_rows(c * C, C), :]) for c in range(4 * i, 4 * i + 4)], 1)
        spec = jnp.dot(_bf16(self.fwd_s[...]), blk, preferred_element_type=F32)
        for j in range(4):
            self.xp[0, 4 * i + j] = spec[:C, j * 128:(j + 1) * 128]
            self.xp[1, 4 * i + j] = spec[C:, j * 128:(j + 1) * 128]

    def combine(self):
        for r in range(C // 8):
            rows = slice(8 * r, 8 * r + 8)

            def product(signal, taps, init, subtract):
                ks = [taps(self.kp[0, m, rows, :], self.kp[1, m, rows, :]) for m in range(NB)]
                acc = list(init)
                for c in range(NB):
                    xc = signal(c)
                    for a in range(c, NB):
                        t = xc * ks[a - c]
                        if acc[a] is None:
                            acc[a] = t
                        else:
                            acc[a] = acc[a] - t if subtract else acc[a] + t
                        yield
                return acc

            def x_re(c):
                return self.xp[0, c, rows, :]

            def x_im(c):
                return self.xp[1, c, rows, :]

            shared = yield from product(
                lambda c: x_re(c) + x_im(c), lambda re, im: re, [None] * NB, False)
            zi = yield from product(x_re, lambda re, im: im - re, shared, False)
            zr = yield from product(x_im, lambda re, im: im + re, shared, True)
            for a in range(NB):
                self.z_s[a, rows, :] = _pack(zr[a], zi[a])

    def finish(self, i):
        blk = jnp.concatenate([_bf16(self.z_s[a]) for a in range(4 * i, 4 * i + 4)], 1)
        y = jnp.dot(_bf16(self.inv_s[...]), blk, preferred_element_type=F32)
        for j in range(4):
            for u in range(C // 16):
                rows = _rows((4 * i + j) * C + 16 * u, 16)
                q = self.qb[self.slot, rows, :]
                self.ob[self.slot, rows, :] = _pack(
                    _unpack(q, 0) * y[16 * u:16 * u + 8, j * 128:(j + 1) * 128],
                    _unpack(q, 1) * y[16 * u + 8:16 * u + 16, j * 128:(j + 1) * 128])


def _run_step(matmuls, conv, conv_done, pace, lead, head, tail, before_unit=lambda u: None):
    left = [UNITS]

    def matmul(paced=False):
        before_unit(UNITS - left[0])
        result = next(matmuls)
        if paced and PACE:
            pace(result[:8, :128])
        left[0] -= 1

    for _ in range(lead):
        matmul()
    tiles = S // 16 // 4
    for i in range(4):
        conv.filter_spectrum(i)
        for u in range(head):
            matmul()
            if u == 0 and i > 0:
                conv.signal_spectrum(i - 1)
            conv.gate_keys(i * tiles + u * tiles // head, i * tiles + (u + 1) * tiles // head)
    matmul()
    conv.signal_spectrum(3)
    matmul()
    products = 3 * (C // 8) * NB * (NB + 1) // 2
    units = left[0] - tail
    combine = conv.combine()
    for u in range(units):
        for _ in range(u * products // units, (u + 1) * products // units):
            next(combine)
        if u == units - 1:
            for _ in combine:
                pass
        matmul(paced=u % PACE_EVERY == 0)
    for i in range(4):
        conv.finish(i)
        if i == 3:
            conv_done()
        if left[0]:
            matmul()
    while left[0]:
        matmul()
    for _ in matmuls:
        pass


def _kernel(x_hbm, wqkv_hbm, wo_hbm, q_hbm, k_hbm, v_hbm, shift_ref, sk_hbm, d_ref, fwd_ref, inv_ref,
            out_hbm,
            x_v, w_v, wo_v, wkt, wqt, g_acc, z_acc, m_v, pk_s, o_s, oa, fwd_s, inv_s,
            kb, vb, qb, skb, kv_s, xp, kp, z_s, ob, skip_s, zero,
            sem_x, sem_w, sem_first, sem_b, sem_oa, sem_ob):

    def x_copy(t):
        rows = pl.ds(t * ST if isinstance(t, int) else pl.multiple_of(t * ST, ST), ST)
        return pltpu.make_async_copy(x_hbm.at[rows, :], x_v.bitcast(BF16).at[rows, :], sem_x.at[t])

    def w_copy(j):
        return pltpu.make_async_copy(
            wqkv_hbm.at[:, pl.ds(j * D, D)], w_v.bitcast(BF16).at[j], sem_w.at[j])

    def first_batch(b):
        def wk(lo, hi, sem):
            return pltpu.make_async_copy(
                wqkv_hbm.at[:, pl.ds(D + lo * 128, (hi - lo) * 128)],
                w_v.bitcast(BF16).at[1, :, pl.ds(lo * 128, (hi - lo) * 128)], sem_first.at[sem])

        def x(lo, hi, sem):
            rows = pl.ds(lo * 128, (hi - lo) * 128)
            return pltpu.make_async_copy(
                x_hbm.at[rows, :], x_v.bitcast(BF16).at[rows, :], sem_first.at[sem])

        def conv_half(h, sem):
            lanes, span = pl.ds(0, 128), pl.ds(h * S // 2, S // 2)
            return [
                pltpu.make_async_copy(
                    sk_hbm.at[lanes, span], skb.bitcast(BF16).at[0, :, span], sem_first.at[sem]),
                pltpu.make_async_copy(
                    k_hbm.at[span, lanes], kb.bitcast(BF16).at[0, pl.ds(HALO + h * S // 2, S // 2), :],
                    sem_first.at[sem + 1]),
                pltpu.make_async_copy(
                    v_hbm.at[span, lanes], vb.bitcast(BF16).at[0, span, :], sem_first.at[sem + 2]),
            ]

        if b == 0:
            return [wk(0, 1, 0), x(0, 1, 1)]
        if b == 1:
            return [x(1, ST // 128, 2), wk(1, 2, 3)]
        if b == 2:
            return [wk(2, 4, 4)] + conv_half(0, 5)
        return conv_half(1, 8) + [wk(4, D // 128, 11), b_copy(0, 0, 3)]

    wo_copy = pltpu.make_async_copy(wo_hbm, wo_v.bitcast(BF16), sem_w.at[3])

    def b_copy(g, slot, i):
        lanes = _lanes(g)
        src, dst = (
            (sk_hbm.at[lanes, :], skb.bitcast(BF16).at[slot]),
            (k_hbm.at[:, lanes], kb.bitcast(BF16).at[slot, pl.ds(HALO, S), :]),
            (v_hbm.at[:, lanes], vb.bitcast(BF16).at[slot]),
            (q_hbm.at[:, lanes], qb.bitcast(BF16).at[slot]),
        )[i]
        return pltpu.make_async_copy(src, dst, sem_b.at[slot, i])

    def b_copies(g, slot):
        return [b_copy(g, slot, i) for i in range(4)]

    def oa_copy(t, slot, n):
        rows = pl.ds(pl.multiple_of(t * ST, ST), ST)
        cols = pl.ds(n * (D // OUT_PARTS), D // OUT_PARTS)
        return pltpu.make_async_copy(oa.at[slot, :, cols], out_hbm.at[rows, cols], sem_oa.at[slot, n])

    def ob_copy(g, slot):
        lanes = _lanes(NG + g)
        return pltpu.make_async_copy(ob.bitcast(BF16).at[slot], out_hbm.at[:, lanes], sem_ob.at[slot])

    def conv(g, slot):
        return _ConvGroup(g, slot, kb, vb, qb, skb, shift_ref, skip_s, fwd_s, inv_s,
                           kv_s, xp, kp, z_s, ob)

    def conv_begin(g, slot):
        for cp in b_copies(g, slot):
            cp.wait()

        @pl.when(g + 1 < NG)
        def _():
            for cp in b_copies(g + 1, 1 - slot):
                cp.start()

        @pl.when(g >= 2)
        def _():
            ob_copy(g - 2, slot).wait()

    def transpose_weight(j, dst, i):
        dst[_rows(i * 128, 128), :] = _words(_bf16(w_v[j, :, i * 128:(i + 1) * 128]).T)

    def pace(tile):
        xp[2, 0, pl.ds(pl.multiple_of(zero[0], 8), 8), :] = tile

    zero[0] = 0
    for cp in first_batch(0) + first_batch(1):
        cp.start()
    for slot in range(2):
        kb[slot, 0:HALO // 2, :] = jnp.zeros((HALO // 2, 128), jnp.uint32)
    skip_s[...] = d_ref[...].astype(F32).reshape(1, D)
    fwd_s[...] = _words(fwd_ref[...])
    inv_s[...] = _words(inv_ref[...])

    def pieces(result):
        height, width = result.shape
        for i in range(max(height // 128, 1)):
            for j in range(width // 128):
                yield result[i * 128:, j * 128:]

    def keys(t, first):
        def project(lo, height):
            pk = []
            for n in range(ST // 128):
                xs = _bf16(x_v[_rows(t * ST + n * 128, 128), :])
                pk.append(_phi(lax.dot_general(
                    _bf16(wkt[_rows(lo, height), :]), xs, _NT_DIMS, preferred_element_type=F32)))
                if n == ST // 128 - 1:
                    rows, total = slice(lo, lo + height), sum(pk[1:], pk[0])
                    z_acc[rows, :] = total if first else z_acc[rows, :] + total
                    pk_s[_rows(lo, height), :] = _riffle(jnp.concatenate(pk, 1))
                yield from pieces(pk[-1])

        def accumulate(lo, height):
            width = max(G_COLS, 256 * 128 // height)
            for n in range(D // width):
                rows, cols = slice(lo, lo + height), slice(n * width, (n + 1) * width)
                g = jnp.dot(_bf16(pk_s[_rows(lo, height), :]), _bf16(x_v[_rows(t * ST, ST), cols]),
                            preferred_element_type=F32)
                g_acc[rows, cols] = g if first else g_acc[rows, cols] + g
                yield from list(pieces(g))[::2]

        chunks = FIRST_CHUNKS if first else [(lo, K_ROWS) for lo in range(0, D, K_ROWS)]
        yield from project(*chunks[0])
        for prev, cur in zip(chunks, chunks[1:]):
            yield from project(*cur)
            yield from accumulate(*prev)
        yield from accumulate(*chunks[-1])

    def arrivals(unit):
        for b, (at, chunks) in enumerate(FIRST_BATCHES):
            if unit == at:
                for cp in first_batch(b):
                    cp.wait()
                for cp in (first_batch(b + 2) if b < 2 else
                           [x_copy(1)] if b == 2 else b_copies(1, 1)):
                    cp.start()
            if unit - at in range(len(chunks)):
                transpose_weight(1, wkt, chunks[unit - at])

    _run_step(keys(0, True), conv(0, 0), lambda: ob_copy(0, 0).start(), pace,
              FIRST_BATCHES[2][0] + 1, FIRST_HEAD, FIRST_TAIL, arrivals)
    w_copy(2).start()
    wo_copy.start()
    w_copy(0).start()

    def phase1(t, carry):
        slot = t % 2
        x_copy(t).wait()
        conv_begin(t, slot)

        @pl.when(t + 1 < NT)
        def _():
            x_copy(t + 1).start()

        _run_step(keys(t, False), conv(t, slot), lambda: ob_copy(t, slot).start(), pace, 0, HEAD1, TAIL1)
        return carry

    lax.fori_loop(1, NT, phase1, 0)

    w_copy(2).wait()
    wo_copy.wait()
    w_copy(0).wait()
    same_head = (lax.broadcasted_iota(jnp.int32, (128, 128), 0) // DH
                 == lax.broadcasted_iota(jnp.int32, (128, 128), 1) // DH)
    kvs = []
    for i in range(D // 128):
        blk = slice(i * 128, (i + 1) * 128)
        kv = jnp.dot(g_acc[blk, :].astype(BF16), _bf16(w_v[2, :, blk]), preferred_element_type=F32)
        kvs.append(jnp.where(same_head, kv, 0.0).astype(BF16))
        transpose_weight(0, wqt, i)
    for i in range(D // 128):
        m_v[_rows(i * 128, 128), :] = _words(
            jnp.dot(kvs[i], _bf16(wo_v[_rows(i * 128, 128), :]), preferred_element_type=F32))
    z_acc[...] = jnp.broadcast_to(jnp.sum(z_acc[...], axis=1, keepdims=True), (D, 128))

    def queries(t, slot):
        for n in range(ST // 128):
            xs = _bf16(x_v[_rows(t * ST + n * 128, 128), :])
            for j in range(D // Q_ROWS):
                chans = slice(j * Q_ROWS, (j + 1) * Q_ROWS)
                pq = _phi(lax.dot_general(
                    _bf16(wqt[_rows(j * Q_ROWS, Q_ROWS), :]), xs, _NT_DIMS, preferred_element_type=F32))
                pz = (pq * z_acc[chans, :]).reshape(Q_ROWS // DH, DH, 128)
                den = jnp.sum(pz, axis=1, keepdims=True) + 1e-6
                o = (pq.reshape(Q_ROWS // DH, DH, 128) * (1.0 / den)).reshape(Q_ROWS, 128)
                o_s[_rows(n * 128, 128), chans] = _words(_bf16(_riffle(o)).T)
                yield from pieces(pq)
        for j in range(D // O_COLS):
            cols = slice(j * O_COLS, (j + 1) * O_COLS)
            for n in range(ST // O_ROWS):
                rows = _rows(n * O_ROWS, O_ROWS)
                res = jnp.dot(_bf16(o_s[rows, :]), _bf16(m_v[:, cols]), preferred_element_type=F32)
                oa[slot, n * O_ROWS:(n + 1) * O_ROWS, cols] = res.astype(BF16)
                if n == ST // O_ROWS - 1:
                    oa_copy(t, slot, j).start()
                yield from pieces(res)

    def phase2(t, carry):
        slot = t % 2
        conv_begin(NT + t, slot)

        @pl.when(t >= 2)
        def _():
            for n in range(OUT_PARTS):
                oa_copy(t - 2, slot, n).wait()

        _run_step(queries(t, slot), conv(NT + t, slot), lambda: ob_copy(NT + t, slot).start(), pace,
                  0, HEAD2, TAIL2)
        return carry

    lax.fori_loop(0, NT, phase2, 0)
    for t in range(NT - 2, NT):
        ob_copy(NT + t, t % 2).wait()
        for n in range(OUT_PARTS):
            oa_copy(t, t % 2, n).wait()


@jax.jit
def pallas_concat_heads__linear_attn_block__ssm_conv_h3__prompt_kernel(
    A_x: jax.Array,
    A_wqkv: jax.Array,
    A_wo: jax.Array,
    B_q: jax.Array,
    B_k: jax.Array,
    B_v: jax.Array,
    B_shift_k: jax.Array,
    B_ssm_k: jax.Array,
    B_ssm_D: jax.Array,
):
    assert A_x.shape == (1, S, D) and B_shift_k.shape == (D, 4) and NG == 2 * NT
    hbm = pl.BlockSpec(memory_space=pl.ANY)
    vmem = pl.BlockSpec(memory_space=pltpu.VMEM)
    out = pl.pallas_call(
        _kernel,
        out_shape=jax.ShapeDtypeStruct((S, 2 * D), BF16),
        in_specs=[hbm, hbm, hbm, hbm, hbm, hbm, vmem, hbm, vmem, vmem, vmem],
        out_specs=hbm,
        scratch_shapes=[
            _packed(S, D),
            _packed(3, D, D),
            _packed(D, D),
            _packed(D, D),
            _packed(D, D),
            pltpu.VMEM((D, D), F32),
            pltpu.VMEM((D, 128), F32),
            _packed(D, D),
            _packed(D, ST),
            _packed(ST, D),
            pltpu.VMEM((2, ST, D), BF16),
            _packed(2 * C, C),
            _packed(C, 2 * C),
            _packed(2, HALO + S, 128),
            _packed(2, S, 128),
            _packed(2, S, 128),
            _packed(2, 128, S),
            _packed(S, 128),
            pltpu.VMEM((3, NB, C, 128), F32),
            pltpu.VMEM((2, NB, C, 128), F32),
            _packed(NB, 2 * C, 128),
            _packed(2, S, 128),
            pltpu.VMEM((1, D), F32),
            pltpu.SMEM((1,), jnp.int32),
            pltpu.SemaphoreType.DMA((NT,)),
            pltpu.SemaphoreType.DMA((4,)),
            pltpu.SemaphoreType.DMA((D // 128 + ST // 128 + 12,)),
            pltpu.SemaphoreType.DMA((2, 4)),
            pltpu.SemaphoreType.DMA((2, OUT_PARTS)),
            pltpu.SemaphoreType.DMA((2,)),
        ],
        compiler_params=pltpu.CompilerParams(vmem_limit_bytes=100 * 2**20),
        name="linattn_h3",
    )(
        A_x.reshape(S, D), A_wqkv, A_wo,
        B_q.reshape(S, D), B_k.reshape(S, D), B_v.reshape(S, D),
        B_shift_k.T, B_ssm_k, B_ssm_D,
        jnp.asarray(_FWD, BF16), jnp.asarray(_INV, BF16),
    )
    return out.reshape(1, S, 2 * D)
```

```python
import jax
import jax.numpy as jnp
import numpy as np
from jax import lax
import jax.experimental.pallas as pl
import jax.experimental.pallas.tpu as pltpu

S = 2048
D = 1024
DH = 32
C = 128
NB = S // C
NG = D // 128
ST = 512
NT = S // ST
UNITS = 2 * (ST // 128) * (D // 128)
MAC_BLOCK = 16
HEAD1 = 4
TAIL1 = 5
HEAD2 = 4
TAIL2 = 10
FIRST_HEAD = 4
FIRST_TAIL = 5
GATES = 1
SELF = 34
LAG = 10
K_ROWS = 256
G_COLS = 256
Q_ROWS = 256
O_ROWS = 256
O_COLS = 128
FIRST_CHUNKS = ((0, 128), (128, 128), (256, 256), (512, 256), (768, 256))
OUT_PARTS = D // O_COLS
FIRST_BATCHES = ((0, (0,)), (2, (1,)), (11, (2, 3)), (11 + 2 * FIRST_HEAD, (4, 5)), (37, (6, 7)))
HALO = 16

F32 = jnp.float32
BF16 = jnp.bfloat16


def _dft_matrices():
    n = np.arange(C, dtype=np.float64)
    theta = np.pi * (4.0 * np.arange(C, dtype=np.float64) + 1.0) / (2.0 * C)
    plain = theta[:, None] * n[None, :]
    centred = theta[:, None] * (n[None, :] - (C - 1) / 2)
    inv = np.concatenate([np.cos(centred).T[:C // 2], -np.sin(centred).T[:C // 2]], 0) / C
    inv = inv.reshape(C // 16, 8, 2, C // 16, 2, 8).transpose(0, 2, 1, 3, 5, 4).reshape(C, C)
    return np.concatenate(
        [np.cos(plain), -np.sin(plain), np.cos(centred), -np.sin(centred), inv], 0).astype(np.float32)


_DFT = _dft_matrices()

_NT_DIMS = (((1,), (1,)), ((), ()))
_TN_DIMS = (((0,), (0,)), ((), ()))


def _packed(*shape):
    return pltpu.VMEM((*shape[:-2], shape[-2] // 2, shape[-1]), jnp.uint32)


def _phi(t):
    return jnp.where(t > 0, t + 1.0, jnp.exp(t)) + 1e-6


def _unpack(words, index):
    return pltpu.unpack_elementwise(words, index=index, packed_dtype=BF16, unpacked_dtype=F32)


def _rows(start, size):
    if isinstance(start, int):
        return pl.ds(start // 2, size // 2)
    return pl.ds(pl.multiple_of(start // 2, 8), size // 2)


def _lanes(g):
    return pl.ds(g * 128 if isinstance(g, int) else pl.multiple_of(g * 128, 128), 128)


def _bf16(words):
    return pltpu.bitcast(words, BF16)


def _words(x):
    return pltpu.bitcast(x.astype(BF16), jnp.uint32)


def _pack(lo, hi):
    return pltpu.pack_elementwise([lo, hi], packed_dtype=BF16).astype(jnp.uint32)


def _riffle(x):
    return jnp.concatenate(
        [_pack(x[i:i + 8], x[i + 8:i + 16]) for i in range(0, x.shape[0], 16)], 0)


def _flip(tile):
    return jnp.take_along_axis(tile, 7 - lax.broadcasted_iota(jnp.int32, (8, 128), 0), axis=0)


class _ConvGroup:
    def __init__(self, g, slot, kb, vb, qb, skb, shift_ref, d_ref, dft, kv_s, xp, kp, held, z_s, ob):
        self.slot, self.kb, self.vb, self.qb, self.skb = slot, kb, vb, qb, skb
        self.dft, self.kv_s, self.xp, self.kp, self.held, self.z_s, self.ob = (
            dft, kv_s, xp, kp, held, z_s, ob)
        lanes = _lanes(g)
        w = shift_ref[:, lanes].astype(F32)
        self.taps = [jnp.broadcast_to(w[j:j + 1], (8, 128)) for j in range(4)]
        self.skip = d_ref[:, lanes]
        self.prev = None

    def filter_spectrum(self, i):
        blk = jnp.concatenate(
            [_bf16(self.skb[self.slot, :, m * C:(m + 1) * C]) for m in range(4 * i, 4 * i + 4)], 0)
        spec = lax.dot_general(_bf16(self.dft[_rows(0, 2 * C), :]), blk, _NT_DIMS,
                               preferred_element_type=F32)
        for j in range(4):
            re = spec[:C, j * 128:(j + 1) * 128]
            im = spec[C:, j * 128:(j + 1) * 128]
            if self.prev is None:
                re = re + self.skip
                re2, im2 = re, im
            else:
                re2, im2 = re - self.prev[1], im + self.prev[0]
            self.prev = (re, im)
            self.kp[0, 4 * i + j] = re2
            self.kp[1, 4 * i + j] = im2

    def gate_keys(self, lo, hi):
        w0, w1, w2, w3 = self.taps
        for i in range(lo, hi):
            base = HALO // 2 + 8 * i
            p0 = self.kb[self.slot, base:base + 8, :]
            p1 = self.kb[self.slot, base - 1:base + 7, :]
            p2 = self.kb[self.slot, base - 2:base + 6, :]
            pv = self.vb[self.slot, 8 * i:8 * i + 8, :]
            e0, o0 = _unpack(p0, 0), _unpack(p0, 1)
            e1, o1 = _unpack(p1, 0), _unpack(p1, 1)
            o2 = _unpack(p2, 1)
            even = (w0 * e0 + w1 * o1 + w2 * e1 + w3 * o2) * _unpack(pv, 0)
            odd = (w0 * o0 + w1 * e0 + w2 * o1 + w3 * e1) * _unpack(pv, 1)
            self.kv_s[8 * i:8 * i + 8, :] = _pack(even, odd)

    def signal_spectrum(self, i):
        blk = jnp.concatenate(
            [_bf16(self.kv_s[_rows(c * C, C), :]) for c in range(4 * i, 4 * i + 4)], 1)
        spec = jnp.dot(_bf16(self.dft[_rows(2 * C, 2 * C), :]), blk, preferred_element_type=F32)
        for j in range(4):
            self.xp[0, 4 * i + j] = spec[:C, j * 128:(j + 1) * 128]
            self.xp[1, 4 * i + j] = spec[C:, j * 128:(j + 1) * 128]

    def combine(self):
        for r in range(C // 8):
            rows = slice(8 * r, 8 * r + 8)

            def product(outputs, signal, taps, init, subtract):
                ks, acc = {}, dict(init)
                for c in range(outputs[-1] + 1):
                    xc = signal(c)
                    for a in outputs:
                        if a < c:
                            continue
                        if a - c not in ks:
                            ks[a - c] = taps(self.kp[0, a - c, rows, :], self.kp[1, a - c, rows, :])
                        t = xc * ks[a - c]
                        if a not in acc:
                            acc[a] = t
                        else:
                            acc[a] = acc[a] - t if subtract else acc[a] + t
                        yield acc[a]
                return acc

            def keep(part, z):
                for a in z:
                    if r % 2 == 0:
                        self.held[part, a] = z[a]
                    else:
                        self.z_s[part, a, _rows(16 * (r // 2), 16), :] = _pack(self.held[part, a], z[a])

            def x_re(c):
                return self.xp[0, c, rows, :]

            def x_im(c):
                return self.xp[1, c, rows, :]

            for lo in range(0, NB, MAC_BLOCK):
                outputs = range(lo, lo + MAC_BLOCK)
                shared = yield from product(
                    outputs, lambda c: x_re(c) + x_im(c), lambda re, im: re, {}, False)
                keep(1, (yield from product(outputs, x_re, lambda re, im: im - re, shared, False)))
                keep(0, (yield from product(outputs, x_im, lambda re, im: im + re, shared, True)))

    def finish(self, i):
        cos, sin = (
            jnp.dot(_bf16(self.dft[_rows(4 * C + part * C // 2, C // 2), :]),
                    jnp.concatenate([_bf16(self.z_s[part, a]) for a in range(4 * i, 4 * i + 4)], 1),
                    preferred_element_type=F32)
            for part in range(2))
        for j in range(4):
            for u in range(C // 32):
                even = (slice(16 * u, 16 * u + 8), slice(j * 128, (j + 1) * 128))
                odd = (slice(16 * u + 8, 16 * u + 16), slice(j * 128, (j + 1) * 128))
                rows = _rows((4 * i + j) * C + 16 * u, 16)
                q = self.qb[self.slot, rows, :]
                self.ob[self.slot, rows, :] = _pack(
                    _unpack(q, 0) * (cos[even] + sin[even]), _unpack(q, 1) * (cos[odd] + sin[odd]))
                rows = _rows((4 * i + j + 1) * C - 16 * (u + 1), 16)
                q = _flip(self.qb[self.slot, rows, :])
                self.ob[self.slot, rows, :] = _flip(_pack(
                    _unpack(q, 0) * (cos[odd] - sin[odd]), _unpack(q, 1) * (cos[even] - sin[even])))


def _run_step(matmuls, conv, conv_done, pace, lead, head, tail, before_unit=lambda u: None):
    left = [UNITS]

    def matmul():
        before_unit(UNITS - left[0])
        left[0] -= 1
        return next(matmuls)

    for _ in range(lead):
        matmul()
    tiles = S // 16 // 4
    for i in range(4):
        conv.filter_spectrum(i)
        for u in range(head):
            matmul()
            if u == 0 and i > 0:
                conv.signal_spectrum(i - 1)
            conv.gate_keys(i * tiles + u * tiles // head, i * tiles + (u + 1) * tiles // head)
    matmul()
    conv.signal_spectrum(3)
    products = 3 * (C // 8) * NB * (NB + 1) // 2
    batches = (left[0] - tail) * GATES
    combine = conv.combine()
    for u in range(batches):
        if u % GATES == 0:
            result = matmul()
        if u:
            pace(result[u % GATES * 128 // GATES:][:8, :128])
        recent = []
        for i in range(u * products // batches, (u + 1) * products // batches):
            recent.append(next(combine))
            if SELF and len(recent) % SELF == 0:
                pace(recent[-LAG])
    for _ in combine:
        pass
    matmul()
    for i in range(4):
        conv.finish(i)
        conv_done(i)
        if left[0]:
            matmul()
    while left[0]:
        matmul()
    for _ in matmuls:
        pass


def _kernel(x_hbm, wqkv_hbm, wo_hbm, q_hbm, k_hbm, v_hbm, shift_ref, sk_hbm, d_ref, dft_ref,
            out_hbm,
            x_v, w_v, wo_v, wkt, wqt, g_acc, z_acc, m_v, pk_s, o_s, oa, dft,
            kb, vb, qb, skb, kv_s, xp, kp, held, z_s, ob, skip_s, zero,
            sem_x, sem_w, sem_first, sem_b, sem_oa, sem_ob):

    def x_copy(t):
        rows = pl.ds(t * ST if isinstance(t, int) else pl.multiple_of(t * ST, ST), ST)
        return pltpu.make_async_copy(x_hbm.at[rows, :], x_v.bitcast(BF16).at[rows, :], sem_x.at[t])

    def w_copy(j):
        return pltpu.make_async_copy(
            wqkv_hbm.at[:, pl.ds(j * D, D)], w_v.bitcast(BF16).at[j], sem_w.at[j])

    def first_batch(b):
        def wk(lo, hi, sem):
            return pltpu.make_async_copy(
                wqkv_hbm.at[:, pl.ds(D + lo * 128, (hi - lo) * 128)],
                w_v.bitcast(BF16).at[1, :, pl.ds(lo * 128, (hi - lo) * 128)], sem_first.at[sem])

        def x(lo, hi, sem):
            rows = pl.ds(lo * 128, (hi - lo) * 128)
            return pltpu.make_async_copy(
                x_hbm.at[rows, :], x_v.bitcast(BF16).at[rows, :], sem_first.at[sem])

        def conv_half(h, sem):
            lanes, span = pl.ds(0, 128), pl.ds(h * S // 2, S // 2)
            return [
                pltpu.make_async_copy(
                    sk_hbm.at[lanes, span], skb.bitcast(BF16).at[0, :, span], sem_first.at[sem]),
                pltpu.make_async_copy(
                    k_hbm.at[span, lanes], kb.bitcast(BF16).at[0, pl.ds(HALO + h * S // 2, S // 2), :],
                    sem_first.at[sem + 1]),
                pltpu.make_async_copy(
                    v_hbm.at[span, lanes], vb.bitcast(BF16).at[0, span, :], sem_first.at[sem + 2]),
            ]

        if b == 0:
            return [wk(0, 1, 0), x(0, 2, 1)]
        if b == 1:
            return [x(2, ST // 128, 2), wk(1, 2, 3)]
        if b == 2:
            return [wk(2, 4, 4)] + conv_half(0, 5)
        if b == 3:
            return conv_half(1, 8) + [wk(4, 6, 11)]
        if b == 4:
            return [wk(6, 8, 12), b_copy(0, 0, 3)]
        return [x_copy(1)] + b_copies(1, 1)

    wo_copy = pltpu.make_async_copy(wo_hbm, wo_v.bitcast(BF16), sem_w.at[3])

    def b_copy(g, slot, i):
        lanes = _lanes(g)
        src, dst = (
            (sk_hbm.at[lanes, :], skb.bitcast(BF16).at[slot]),
            (k_hbm.at[:, lanes], kb.bitcast(BF16).at[slot, pl.ds(HALO, S), :]),
            (v_hbm.at[:, lanes], vb.bitcast(BF16).at[slot]),
            (q_hbm.at[:, lanes], qb.bitcast(BF16).at[slot]),
        )[i]
        return pltpu.make_async_copy(src, dst, sem_b.at[slot, i])

    def b_copies(g, slot):
        return [b_copy(g, slot, i) for i in range(4)]

    def oa_copy(t, slot, n):
        rows = pl.ds(pl.multiple_of(t * ST, ST), ST)
        cols = pl.ds(n * (D // OUT_PARTS), D // OUT_PARTS)
        return pltpu.make_async_copy(oa.at[slot, :, cols], out_hbm.at[rows, cols], sem_oa.at[slot, n])

    def ob_copy(g, slot, i):
        rows = pl.ds(i * S // 4, S // 4)
        return pltpu.make_async_copy(
            ob.bitcast(BF16).at[slot, rows, :], out_hbm.at[rows, _lanes(NG + g)], sem_ob.at[slot, i])

    def conv(g, slot):
        return _ConvGroup(g, slot, kb, vb, qb, skb, shift_ref, skip_s, dft,
                          kv_s, xp, kp, held, z_s, ob)

    def conv_begin(g, slot):
        for cp in b_copies(g, slot):
            cp.wait()

        @pl.when(g + 1 < NG)
        def _():
            for cp in b_copies(g + 1, 1 - slot):
                cp.start()

        @pl.when(g >= 2)
        def _():
            for i in range(4):
                ob_copy(g - 2, slot, i).wait()

    def transpose_weight(j, dst, i):
        dst[_rows(i * 128, 128), :] = _words(_bf16(w_v[j, :, i * 128:(i + 1) * 128]).T)

    def pace(tile):
        xp[2, 0, pl.ds(pl.multiple_of(zero[0], 8), 8), :] = tile

    zero[0] = 0
    for cp in first_batch(0):
        cp.start()
    for slot in range(2):
        kb[slot, 0:HALO // 2, :] = jnp.zeros((HALO // 2, 128), jnp.uint32)
    skip_s[...] = d_ref[...].astype(F32).reshape(1, D)
    dft[...] = _words(dft_ref[...])

    def pieces(result):
        height, width = result.shape
        for i in range(max(height // 128, 1)):
            for j in range(width // 128):
                yield result[i * 128:, j * 128:]

    def keys(t, first):
        def project(lo, height):
            pk = []
            for n in range(ST // 128):
                xs = _bf16(x_v[_rows(t * ST + n * 128, 128), :])
                pk.append(_phi(lax.dot_general(
                    _bf16(wkt[_rows(lo, height), :]), xs, _NT_DIMS, preferred_element_type=F32)))
                if n == ST // 128 - 1:
                    rows, total = slice(lo, lo + height), sum(pk[1:], pk[0])
                    z_acc[rows, :] = total if first else z_acc[rows, :] + total
                    pk_s[_rows(lo, height), :] = _riffle(jnp.concatenate(pk, 1))
                yield from pieces(pk[-1])

        def accumulate(lo, height):
            width = max(G_COLS, 256 * 128 // height)
            for n in range(D // width):
                rows, cols = slice(lo, lo + height), slice(n * width, (n + 1) * width)
                g = jnp.dot(_bf16(pk_s[_rows(lo, height), :]), _bf16(x_v[_rows(t * ST, ST), cols]),
                            preferred_element_type=F32)
                g_acc[rows, cols] = g if first else g_acc[rows, cols] + g
                yield from list(pieces(g))[::2]

        chunks = FIRST_CHUNKS if first else [(lo, K_ROWS) for lo in range(0, D, K_ROWS)]
        yield from project(*chunks[0])
        for prev, cur in zip(chunks, chunks[1:]):
            yield from project(*cur)
            yield from accumulate(*prev)
        yield from accumulate(*chunks[-1])

    def arrivals(unit):
        for b, (at, chunks) in enumerate(FIRST_BATCHES):
            if unit == at:
                for cp in first_batch(b + 1):
                    cp.start()
                for cp in first_batch(b):
                    cp.wait()
            if unit == at:
                for i in chunks:
                    transpose_weight(1, wkt, i)

    _run_step(keys(0, True), conv(0, 0), lambda i: ob_copy(0, 0, i).start(), pace,
              FIRST_BATCHES[2][0] + 1, FIRST_HEAD, FIRST_TAIL, arrivals)

    def phase1(t, carry):
        slot = t % 2
        x_copy(t).wait()
        conv_begin(t, slot)

        @pl.when(t + 1 < NT)
        def _():
            x_copy(t + 1).start()

        for i, cp in enumerate((w_copy(2), wo_copy, w_copy(0))):
            pl.when(t == i + 1)(cp.start)

        _run_step(keys(t, False), conv(t, slot), lambda i: ob_copy(t, slot, i).start(), pace, 0, HEAD1, TAIL1)
        return carry

    lax.fori_loop(1, NT, phase1, 0)

    w_copy(2).wait()
    wo_copy.wait()
    w_copy(0).wait()
    same_head = (lax.broadcasted_iota(jnp.int32, (128, 128), 0) // DH
                 == lax.broadcasted_iota(jnp.int32, (128, 128), 1) // DH)
    kvs = []
    for i in range(D // 128):
        blk = slice(i * 128, (i + 1) * 128)
        kv = jnp.dot(g_acc[blk, :].astype(BF16), _bf16(w_v[2, :, blk]), preferred_element_type=F32)
        kvs.append(jnp.where(same_head, kv, 0.0).astype(BF16))
        transpose_weight(0, wqt, i)
    for i in range(D // 128):
        m_v[_rows(i * 128, 128), :] = _words(
            jnp.dot(kvs[i], _bf16(wo_v[_rows(i * 128, 128), :]), preferred_element_type=F32))
    z_acc[...] = jnp.broadcast_to(jnp.sum(z_acc[...], axis=1, keepdims=True), (D, 128))

    def queries(t, slot):
        for n in range(ST // 128):
            xs = _bf16(x_v[_rows(t * ST + n * 128, 128), :])
            for j in range(D // Q_ROWS):
                chans = slice(j * Q_ROWS, (j + 1) * Q_ROWS)
                pq = _phi(lax.dot_general(
                    _bf16(wqt[_rows(j * Q_ROWS, Q_ROWS), :]), xs, _NT_DIMS, preferred_element_type=F32))
                pz = (pq * z_acc[chans, :]).reshape(Q_ROWS // DH, DH, 128)
                den = jnp.sum(pz, axis=1, keepdims=True) + 1e-6
                o = (pq.reshape(Q_ROWS // DH, DH, 128) * (1.0 / den)).reshape(Q_ROWS, 128)
                o_s[_rows(n * 128, 128), chans] = _words(_bf16(_riffle(o)).T)
                yield from pieces(pq)
        for j in range(D // O_COLS):
            cols = slice(j * O_COLS, (j + 1) * O_COLS)
            for n in range(ST // O_ROWS):
                rows = _rows(n * O_ROWS, O_ROWS)
                res = jnp.dot(_bf16(o_s[rows, :]), _bf16(m_v[:, cols]), preferred_element_type=F32)
                oa[slot, n * O_ROWS:(n + 1) * O_ROWS, cols] = res.astype(BF16)
                if n == ST // O_ROWS - 1:
                    oa_copy(t, slot, j).start()
                yield from pieces(res)

    def phase2(t, carry):
        slot = t % 2
        conv_begin(NT + t, slot)

        @pl.when(t >= 2)
        def _():
            for n in range(OUT_PARTS):
                oa_copy(t - 2, slot, n).wait()

        _run_step(queries(t, slot), conv(NT + t, slot), lambda i: ob_copy(NT + t, slot, i).start(), pace,
                  0, HEAD2, TAIL2)
        return carry

    lax.fori_loop(0, NT, phase2, 0)
    for t in range(NT - 2, NT):
        for i in range(4):
            ob_copy(NT + t, t % 2, i).wait()
        for n in range(OUT_PARTS):
            oa_copy(t, t % 2, n).wait()


@jax.jit
def pallas_concat_heads__linear_attn_block__ssm_conv_h3__prompt_kernel(
    A_x: jax.Array,
    A_wqkv: jax.Array,
    A_wo: jax.Array,
    B_q: jax.Array,
    B_k: jax.Array,
    B_v: jax.Array,
    B_shift_k: jax.Array,
    B_ssm_k: jax.Array,
    B_ssm_D: jax.Array,
):
    assert A_x.shape == (1, S, D) and B_shift_k.shape == (D, 4) and NG == 2 * NT
    hbm = pl.BlockSpec(memory_space=pl.ANY)
    vmem = pl.BlockSpec(memory_space=pltpu.VMEM)
    out = pl.pallas_call(
        _kernel,
        out_shape=jax.ShapeDtypeStruct((S, 2 * D), BF16),
        in_specs=[hbm, hbm, hbm, hbm, hbm, hbm, vmem, hbm, vmem, vmem],
        out_specs=hbm,
        scratch_shapes=[
            _packed(S, D),
            _packed(3, D, D),
            _packed(D, D),
            _packed(D, D),
            _packed(D, D),
            pltpu.VMEM((D, D), F32),
            pltpu.VMEM((D, 128), F32),
            _packed(D, D),
            _packed(D, ST),
            _packed(ST, D),
            pltpu.VMEM((2, ST, D), BF16),
            _packed(5 * C, C),
            _packed(2, HALO + S, 128),
            _packed(2, S, 128),
            _packed(2, S, 128),
            _packed(2, 128, S),
            _packed(S, 128),
            pltpu.VMEM((3, NB, C, 128), F32),
            pltpu.VMEM((2, NB, C, 128), F32),
            pltpu.VMEM((2, NB, 8, 128), F32),
            _packed(2, NB, C, 128),
            _packed(2, S, 128),
            pltpu.VMEM((1, D), F32),
            pltpu.SMEM((1,), jnp.int32),
            pltpu.SemaphoreType.DMA((NT,)),
            pltpu.SemaphoreType.DMA((4,)),
            pltpu.SemaphoreType.DMA((13,)),
            pltpu.SemaphoreType.DMA((2, 4)),
            pltpu.SemaphoreType.DMA((2, OUT_PARTS)),
            pltpu.SemaphoreType.DMA((2, 4)),
        ],
        compiler_params=pltpu.CompilerParams(vmem_limit_bytes=100 * 2**20),
        name="linattn_h3",
    )(
        A_x.reshape(S, D), A_wqkv, A_wo,
        B_q.reshape(S, D), B_k.reshape(S, D), B_v.reshape(S, D),
        B_shift_k.T, B_ssm_k, B_ssm_D,
        jnp.asarray(_DFT, BF16),
    )
    return out.reshape(1, S, 2 * D)
```

```python
import jax
import jax.numpy as jnp
import numpy as np
from jax import lax
import jax.experimental.pallas as pl
import jax.experimental.pallas.tpu as pltpu

S = 2048
D = 1024
DH = 32
C = 128
NB = S // C
NG = D // 128
ST = 512
NT = S // ST
UNITS = 2 * (ST // 128) * (D // 128)
MAC_BLOCK = 16
HEAD1 = 4
TAIL1 = 5
HEAD2 = 4
TAIL2 = 10
FIRST_HEAD = 4
FIRST_TAIL = 5
GATES = 1
SELF = 34
LAG = 10
K_ROWS = 256
G_COLS = 256
Q_ROWS = 256
O_ROWS = 256
O_COLS = 128
FIRST_CHUNKS = ((0, 128), (128, 128), (256, 256), (512, 256), (768, 256))
FIRST_BATCHES = ((0, (0,)), (2, (1,)), (11, (2, 3)), (11 + 2 * FIRST_HEAD, (4, 5)), (37, (6, 7)))
HALO = 16

F32 = jnp.float32
BF16 = jnp.bfloat16


def _dft_matrices():
    n = np.arange(C, dtype=np.float64)
    theta = np.pi * (4.0 * np.arange(C, dtype=np.float64) + 1.0) / (2.0 * C)
    plain = theta[:, None] * n[None, :]
    centred = theta[:, None] * (n[None, :] - (C - 1) / 2)
    inv = np.concatenate([np.cos(centred).T[:C // 2], -np.sin(centred).T[:C // 2]], 0) / C
    inv = inv.reshape(C // 16, 8, 2, C // 16, 2, 8).transpose(0, 2, 1, 3, 5, 4).reshape(C, C)
    return np.concatenate(
        [np.cos(plain), -np.sin(plain), np.cos(centred), -np.sin(centred), inv], 0).astype(np.float32)


_DFT = _dft_matrices()

_NT_DIMS = (((1,), (1,)), ((), ()))
_TN_DIMS = (((0,), (0,)), ((), ()))


def _packed(*shape):
    return pltpu.VMEM((*shape[:-2], shape[-2] // 2, shape[-1]), jnp.uint32)


def _phi(t):
    return jnp.where(t > 0, t + 1.0, jnp.exp(t)) + 1e-6


def _unpack(words, index):
    return pltpu.unpack_elementwise(words, index=index, packed_dtype=BF16, unpacked_dtype=F32)


def _rows(start, size):
    if isinstance(start, int):
        return pl.ds(start // 2, size // 2)
    return pl.ds(pl.multiple_of(start // 2, 8), size // 2)


def _lanes(g):
    return pl.ds(g * 128 if isinstance(g, int) else pl.multiple_of(g * 128, 128), 128)


def _bf16(words):
    return pltpu.bitcast(words, BF16)


def _words(x):
    return pltpu.bitcast(x.astype(BF16), jnp.uint32)


def _pack(lo, hi):
    return pltpu.pack_elementwise([lo, hi], packed_dtype=BF16).astype(jnp.uint32)


def _riffle(x):
    return jnp.concatenate(
        [_pack(x[i:i + 8], x[i + 8:i + 16]) for i in range(0, x.shape[0], 16)], 0)


def _flip(tile):
    return jnp.take_along_axis(tile, 7 - lax.broadcasted_iota(jnp.int32, (8, 128), 0), axis=0)


class _ConvGroup:
    def __init__(self, g, kb, vb, qb, skb, shift, skip, dft, kv_s, xp, kp, held, z_s, ob):
        self.g, self.kb, self.vb, self.qb, self.skb, self.shift, self.skip = (
            g, kb, vb, qb, skb, shift, skip)
        self.dft, self.kv_s, self.xp, self.kp, self.held, self.z_s, self.ob = (
            dft, kv_s, xp, kp, held, z_s, ob)
        self.prev = None

    def filter_spectrum(self, i):
        blk = jnp.concatenate(
            [_bf16(self.skb[self.g, :, m * C:(m + 1) * C]) for m in range(4 * i, 4 * i + 4)], 0)
        spec = lax.dot_general(_bf16(self.dft[_rows(0, 2 * C), :]), blk, _NT_DIMS,
                               preferred_element_type=F32)
        for j in range(4):
            re = spec[:C, j * 128:(j + 1) * 128]
            im = spec[C:, j * 128:(j + 1) * 128]
            if self.prev is None:
                re = re + self.skip[:, _lanes(self.g)]
                re2, im2 = re, im
            else:
                re2, im2 = re - self.prev[1], im + self.prev[0]
            self.prev = (re, im)
            self.kp[0, 4 * i + j] = re2
            self.kp[1, 4 * i + j] = im2

    def gate_keys(self, lo, hi):
        w = self.shift[:, _lanes(self.g)].astype(F32)
        w0, w1, w2, w3 = (jnp.broadcast_to(w[j:j + 1], (8, 128)) for j in range(4))
        for i in range(lo, hi):
            base = HALO // 2 + 8 * i
            p0 = self.kb[self.g, base:base + 8, :]
            p1 = self.kb[self.g, base - 1:base + 7, :]
            p2 = self.kb[self.g, base - 2:base + 6, :]
            pv = self.vb[self.g, 8 * i:8 * i + 8, :]
            e0, o0 = _unpack(p0, 0), _unpack(p0, 1)
            e1, o1 = _unpack(p1, 0), _unpack(p1, 1)
            o2 = _unpack(p2, 1)
            even = (w0 * e0 + w1 * o1 + w2 * e1 + w3 * o2) * _unpack(pv, 0)
            odd = (w0 * o0 + w1 * e0 + w2 * o1 + w3 * e1) * _unpack(pv, 1)
            self.kv_s[8 * i:8 * i + 8, :] = _pack(even, odd)

    def signal_spectrum(self, i):
        blk = jnp.concatenate(
            [_bf16(self.kv_s[_rows(c * C, C), :]) for c in range(4 * i, 4 * i + 4)], 1)
        spec = jnp.dot(_bf16(self.dft[_rows(2 * C, 2 * C), :]), blk, preferred_element_type=F32)
        for j in range(4):
            self.xp[0, 4 * i + j] = spec[:C, j * 128:(j + 1) * 128]
            self.xp[1, 4 * i + j] = spec[C:, j * 128:(j + 1) * 128]

    def combine(self):
        for r in range(C // 8):
            rows = slice(8 * r, 8 * r + 8)

            def product(outputs, signal, taps, init, subtract):
                ks, acc = {}, dict(init)
                for c in range(outputs[-1] + 1):
                    xc = signal(c)
                    for a in outputs:
                        if a < c:
                            continue
                        if a - c not in ks:
                            ks[a - c] = taps(self.kp[0, a - c, rows, :], self.kp[1, a - c, rows, :])
                        t = xc * ks[a - c]
                        if a not in acc:
                            acc[a] = t
                        else:
                            acc[a] = acc[a] - t if subtract else acc[a] + t
                        yield acc[a]
                return acc

            def keep(part, z):
                for a in z:
                    if r % 2 == 0:
                        self.held[part, a] = z[a]
                    else:
                        self.z_s[part, a, _rows(16 * (r // 2), 16), :] = _pack(self.held[part, a], z[a])

            def x_re(c):
                return self.xp[0, c, rows, :]

            def x_im(c):
                return self.xp[1, c, rows, :]

            for lo in range(0, NB, MAC_BLOCK):
                outputs = range(lo, lo + MAC_BLOCK)
                shared = yield from product(
                    outputs, lambda c: x_re(c) + x_im(c), lambda re, im: re, {}, False)
                keep(1, (yield from product(outputs, x_re, lambda re, im: im - re, shared, False)))
                keep(0, (yield from product(outputs, x_im, lambda re, im: im + re, shared, True)))

    def finish(self, i):
        cos, sin = (
            jnp.dot(_bf16(self.dft[_rows(4 * C + part * C // 2, C // 2), :]),
                    jnp.concatenate([_bf16(self.z_s[part, a]) for a in range(4 * i, 4 * i + 4)], 1),
                    preferred_element_type=F32)
            for part in range(2))
        for j in range(4):
            for u in range(C // 32):
                even = (slice(16 * u, 16 * u + 8), slice(j * 128, (j + 1) * 128))
                odd = (slice(16 * u + 8, 16 * u + 16), slice(j * 128, (j + 1) * 128))
                rows = _rows((4 * i + j) * C + 16 * u, 16)
                q = self.qb[self.g, rows, :]
                self.ob[self.g, rows, :] = _pack(
                    _unpack(q, 0) * (cos[even] + sin[even]), _unpack(q, 1) * (cos[odd] + sin[odd]))
                rows = _rows((4 * i + j + 1) * C - 16 * (u + 1), 16)
                q = _flip(self.qb[self.g, rows, :])
                self.ob[self.g, rows, :] = _flip(_pack(
                    _unpack(q, 0) * (cos[odd] - sin[odd]), _unpack(q, 1) * (cos[even] - sin[even])))


def _run_step(matmuls, conv, conv_done, pace, lead, head, tail, before_unit=lambda u: None):
    left = [UNITS]

    def matmul():
        before_unit(UNITS - left[0])
        left[0] -= 1
        return next(matmuls)

    for _ in range(lead):
        matmul()
    tiles = S // 16 // 4
    for i in range(4):
        conv.filter_spectrum(i)
        for u in range(head):
            matmul()
            if u == 0 and i > 0:
                conv.signal_spectrum(i - 1)
            conv.gate_keys(i * tiles + u * tiles // head, i * tiles + (u + 1) * tiles // head)
    matmul()
    conv.signal_spectrum(3)
    products = 3 * (C // 8) * NB * (NB + 1) // 2
    batches = (left[0] - tail) * GATES
    combine = conv.combine()
    for u in range(batches):
        if u % GATES == 0:
            result = matmul()
        if u:
            pace(result[u % GATES * 128 // GATES:][:8, :128])
        recent = []
        for i in range(u * products // batches, (u + 1) * products // batches):
            recent.append(next(combine))
            if SELF and len(recent) % SELF == 0:
                pace(recent[-LAG])
    for _ in combine:
        pass
    matmul()
    for i in range(4):
        conv.finish(i)
        conv_done(i)
        if left[0]:
            matmul()
    while left[0]:
        matmul()
    for _ in matmuls:
        pass


def _kernel(x_hbm, wqkv_hbm, wo_hbm, q_hbm, k_hbm, v_hbm, shift_hbm, sk_hbm, d_hbm, dft_hbm,
            out_hbm,
            x_v, w_v, wo_v, wkt, wqt, g_acc, z_acc, m_v, pk_s, o_s, oa,
            kb, vb, qb, skb, shift_v, d_v, skip_s, dft, kv_s, xp, kp, held, z_s, ob, zero,
            sem_x, sem_w, sem_first, sem_b, sem_oa, sem_ob):

    def tile_rows(t):
        return pl.ds(t * ST if isinstance(t, int) else pl.multiple_of(t * ST, ST), ST)

    def x_copy(t):
        return pltpu.make_async_copy(
            x_hbm.at[tile_rows(t), :], x_v.bitcast(BF16).at[tile_rows(t), :], sem_x.at[t])

    def w_copy(j):
        return pltpu.make_async_copy(
            wqkv_hbm.at[:, pl.ds(j * D, D)], w_v.bitcast(BF16).at[j], sem_w.at[j])

    def wo_copy():
        return pltpu.make_async_copy(wo_hbm, wo_v.bitcast(BF16), sem_w.at[1])

    def b_copy(g, i):
        lanes = _lanes(g)
        src, dst = (
            (sk_hbm.at[lanes, :], skb.bitcast(BF16).at[g]),
            (k_hbm.at[:, lanes], kb.bitcast(BF16).at[g, pl.ds(HALO, S), :]),
            (v_hbm.at[:, lanes], vb.bitcast(BF16).at[g]),
            (q_hbm.at[:, lanes], qb.bitcast(BF16).at[g]),
        )[i]
        return pltpu.make_async_copy(src, dst, sem_b.at[g, i])

    def b_copies(g):
        return [b_copy(g, i) for i in range(4)]

    def oa_copy(t, j):
        cols = pl.ds(j * O_COLS, O_COLS)
        return pltpu.make_async_copy(
            oa.at[tile_rows(t), cols], out_hbm.at[tile_rows(t), cols], sem_oa.at[t, j])

    def ob_copy(g, i):
        rows = pl.ds(i * S // 4, S // 4)
        return pltpu.make_async_copy(
            ob.bitcast(BF16).at[g, rows, :], out_hbm.at[rows, _lanes(NG + g)], sem_ob.at[g, i])

    def first_batch(b):
        def wk(lo, hi, sem):
            return pltpu.make_async_copy(
                wqkv_hbm.at[:, pl.ds(D + lo * 128, (hi - lo) * 128)],
                w_v.bitcast(BF16).at[1, :, pl.ds(lo * 128, (hi - lo) * 128)], sem_first.at[sem])

        def x(lo, hi, sem):
            rows = pl.ds(lo * 128, (hi - lo) * 128)
            return pltpu.make_async_copy(
                x_hbm.at[rows, :], x_v.bitcast(BF16).at[rows, :], sem_first.at[sem])

        def conv_half(h, sem):
            lanes, span = pl.ds(0, 128), pl.ds(h * S // 2, S // 2)
            return [
                pltpu.make_async_copy(
                    sk_hbm.at[lanes, span], skb.bitcast(BF16).at[0, :, span], sem_first.at[sem]),
                pltpu.make_async_copy(
                    k_hbm.at[span, lanes], kb.bitcast(BF16).at[0, pl.ds(HALO + h * S // 2, S // 2), :],
                    sem_first.at[sem + 1]),
                pltpu.make_async_copy(
                    v_hbm.at[span, lanes], vb.bitcast(BF16).at[0, span, :], sem_first.at[sem + 2]),
            ]

        if b == 0:
            return [wk(0, 1, 0), x(0, 2, 1)]
        if b == 1:
            return [x(2, ST // 128, 2), wk(1, 2, 3)]
        if b == 2:
            return [wk(2, 4, 4)] + conv_half(0, 5) + [
                pltpu.make_async_copy(dft_hbm, dft.bitcast(BF16), sem_first.at[13]),
                pltpu.make_async_copy(shift_hbm, shift_v, sem_first.at[14]),
                pltpu.make_async_copy(d_hbm, d_v, sem_first.at[15])]
        if b == 3:
            return conv_half(1, 8) + [wk(4, 6, 11)]
        return [wk(6, 8, 12), b_copy(0, 3)]

    def later_inputs():
        copies = []
        for t, weight in zip(range(1, NT), (w_copy(2), wo_copy(), w_copy(0))):
            copies += [x_copy(t)] + b_copies(t) + [weight]
        for g in range(NT, NG):
            copies += b_copies(g)
        return copies

    def conv(g):
        return _ConvGroup(g, kb, vb, qb, skb, shift_v, skip_s, dft, kv_s, xp, kp, held, z_s, ob)

    def transpose_weight(j, dst, i):
        dst[_rows(i * 128, 128), :] = _words(_bf16(w_v[j, :, i * 128:(i + 1) * 128]).T)

    def pace(tile):
        xp[2, 0, pl.ds(pl.multiple_of(zero[0], 8), 8), :] = tile

    for cp in first_batch(0) + first_batch(1):
        cp.start()
    zero[0] = 0
    for g in range(NG):
        kb[g, 0:HALO // 2, :] = jnp.zeros((HALO // 2, 128), jnp.uint32)

    def pieces(result):
        height, width = result.shape
        for i in range(max(height // 128, 1)):
            for j in range(width // 128):
                yield result[i * 128:, j * 128:]

    def keys(t, first):
        def project(lo, height):
            pk = []
            for n in range(ST // 128):
                xs = _bf16(x_v[_rows(t * ST + n * 128, 128), :])
                pk.append(_phi(lax.dot_general(
                    _bf16(wkt[_rows(lo, height), :]), xs, _NT_DIMS, preferred_element_type=F32)))
                if n == ST // 128 - 1:
                    rows, total = slice(lo, lo + height), sum(pk[1:], pk[0])
                    z_acc[rows, :] = total if first else z_acc[rows, :] + total
                    pk_s[_rows(lo, height), :] = _riffle(jnp.concatenate(pk, 1))
                yield from pieces(pk[-1])

        def accumulate(lo, height):
            width = max(G_COLS, 256 * 128 // height)
            for n in range(D // width):
                rows, cols = slice(lo, lo + height), slice(n * width, (n + 1) * width)
                g = jnp.dot(_bf16(pk_s[_rows(lo, height), :]), _bf16(x_v[_rows(t * ST, ST), cols]),
                            preferred_element_type=F32)
                g_acc[rows, cols] = g if first else g_acc[rows, cols] + g
                yield from list(pieces(g))[::2]

        chunks = FIRST_CHUNKS if first else [(lo, K_ROWS) for lo in range(0, D, K_ROWS)]
        yield from project(*chunks[0])
        for prev, cur in zip(chunks, chunks[1:]):
            yield from project(*cur)
            yield from accumulate(*prev)
        yield from accumulate(*chunks[-1])

    def arrivals(unit):
        for b, (at, chunks) in enumerate(FIRST_BATCHES):
            if unit == at:
                for cp in first_batch(b):
                    cp.wait()
                ahead = first_batch(b + 2) if b + 2 < len(FIRST_BATCHES) else []
                for cp in ahead + (later_inputs() if b + 3 == len(FIRST_BATCHES) else []):
                    cp.start()
                for i in chunks:
                    transpose_weight(1, wkt, i)
                if b == 2:
                    skip_s[...] = d_v[...].astype(F32).reshape(1, D)

    _run_step(keys(0, True), conv(0), lambda i: ob_copy(0, i).start(), pace,
              FIRST_BATCHES[2][0] + 1, FIRST_HEAD, FIRST_TAIL, arrivals)

    def phase1(t, carry):
        for cp in [x_copy(t)] + b_copies(t):
            cp.wait()
        _run_step(keys(t, False), conv(t), lambda i: ob_copy(t, i).start(), pace, 0, HEAD1, TAIL1)
        return carry

    lax.fori_loop(1, NT, phase1, 0)

    for cp in (w_copy(2), wo_copy(), w_copy(0)):
        cp.wait()
    same_head = (lax.broadcasted_iota(jnp.int32, (128, 128), 0) // DH
                 == lax.broadcasted_iota(jnp.int32, (128, 128), 1) // DH)
    kvs = []
    for i in range(D // 128):
        blk = slice(i * 128, (i + 1) * 128)
        kv = jnp.dot(g_acc[blk, :].astype(BF16), _bf16(w_v[2, :, blk]), preferred_element_type=F32)
        kvs.append(jnp.where(same_head, kv, 0.0).astype(BF16))
        transpose_weight(0, wqt, i)
    for i in range(D // 128):
        m_v[_rows(i * 128, 128), :] = _words(
            jnp.dot(kvs[i], _bf16(wo_v[_rows(i * 128, 128), :]), preferred_element_type=F32))
    z_acc[...] = jnp.broadcast_to(jnp.sum(z_acc[...], axis=1, keepdims=True), (D, 128))

    def queries(t):
        for n in range(ST // 128):
            xs = _bf16(x_v[_rows(t * ST + n * 128, 128), :])
            for j in range(D // Q_ROWS):
                chans = slice(j * Q_ROWS, (j + 1) * Q_ROWS)
                pq = _phi(lax.dot_general(
                    _bf16(wqt[_rows(j * Q_ROWS, Q_ROWS), :]), xs, _NT_DIMS, preferred_element_type=F32))
                pz = (pq * z_acc[chans, :]).reshape(Q_ROWS // DH, DH, 128)
                den = jnp.sum(pz, axis=1, keepdims=True) + 1e-6
                o = (pq.reshape(Q_ROWS // DH, DH, 128) * (1.0 / den)).reshape(Q_ROWS, 128)
                o_s[_rows(n * 128, 128), chans] = _words(_bf16(_riffle(o)).T)
                yield from pieces(pq)
        for j in range(D // O_COLS):
            cols = slice(j * O_COLS, (j + 1) * O_COLS)
            for n in range(ST // O_ROWS):
                rows = _rows(n * O_ROWS, O_ROWS)
                res = jnp.dot(_bf16(o_s[rows, :]), _bf16(m_v[:, cols]), preferred_element_type=F32)
                oa[pl.ds(pl.multiple_of(t * ST + n * O_ROWS, O_ROWS), O_ROWS), cols] = res.astype(BF16)
                if n == ST // O_ROWS - 1:
                    oa_copy(t, j).start()
                yield from pieces(res)

    def phase2(t, carry):
        for cp in b_copies(NT + t):
            cp.wait()
        _run_step(queries(t), conv(NT + t), lambda i: ob_copy(NT + t, i).start(), pace,
                  0, HEAD2, TAIL2)
        return carry

    lax.fori_loop(0, NT, phase2, 0)
    for g in range(NG):
        for i in range(4):
            ob_copy(g, i).wait()
    for t in range(NT):
        for j in range(D // O_COLS):
            oa_copy(t, j).wait()


@jax.jit
def pallas_concat_heads__linear_attn_block__ssm_conv_h3__prompt_kernel(
    A_x: jax.Array,
    A_wqkv: jax.Array,
    A_wo: jax.Array,
    B_q: jax.Array,
    B_k: jax.Array,
    B_v: jax.Array,
    B_shift_k: jax.Array,
    B_ssm_k: jax.Array,
    B_ssm_D: jax.Array,
):
    assert A_x.shape == (1, S, D) and B_shift_k.shape == (D, 4) and NG == 2 * NT
    hbm = pl.BlockSpec(memory_space=pl.ANY)
    out = pl.pallas_call(
        _kernel,
        out_shape=jax.ShapeDtypeStruct((S, 2 * D), BF16),
        in_specs=[hbm] * 10,
        out_specs=hbm,
        scratch_shapes=[
            _packed(S, D),
            _packed(3, D, D),
            _packed(D, D),
            _packed(D, D),
            _packed(D, D),
            pltpu.VMEM((D, D), F32),
            pltpu.VMEM((D, 128), F32),
            _packed(D, D),
            _packed(D, ST),
            _packed(ST, D),
            pltpu.VMEM((S, D), BF16),
            _packed(NG, HALO + S, 128),
            _packed(NG, S, 128),
            _packed(NG, S, 128),
            _packed(NG, 128, S),
            pltpu.VMEM((4, D), BF16),
            pltpu.VMEM((D,), BF16),
            pltpu.VMEM((1, D), F32),
            _packed(5 * C, C),
            _packed(S, 128),
            pltpu.VMEM((3, NB, C, 128), F32),
            pltpu.VMEM((2, NB, C, 128), F32),
            pltpu.VMEM((2, NB, 8, 128), F32),
            _packed(2, NB, C, 128),
            _packed(NG, S, 128),
            pltpu.SMEM((1,), jnp.int32),
            pltpu.SemaphoreType.DMA((NT,)),
            pltpu.SemaphoreType.DMA((3,)),
            pltpu.SemaphoreType.DMA((16,)),
            pltpu.SemaphoreType.DMA((NG, 4)),
            pltpu.SemaphoreType.DMA((NT, D // O_COLS)),
            pltpu.SemaphoreType.DMA((NG, 4)),
        ],
        compiler_params=pltpu.CompilerParams(vmem_limit_bytes=100 * 2**20),
        name="linattn_h3",
    )(
        A_x.reshape(S, D), A_wqkv, A_wo,
        B_q.reshape(S, D), B_k.reshape(S, D), B_v.reshape(S, D),
        B_shift_k.T, B_ssm_k, B_ssm_D,
        jnp.asarray(_DFT, BF16),
    )
    return out.reshape(1, S, 2 * D)
```

```python
import jax
import jax.numpy as jnp
import numpy as np
from jax import lax
import jax.experimental.pallas as pl
import jax.experimental.pallas.tpu as pltpu

S = 2048
D = 1024
DH = 32
C = 128
NB = S // C
NG = D // 128
ST = 512
NT = S // ST
UNITS = 2 * (ST // 128) * (D // 128)
MAC_BLOCK = 16
HEAD1 = 4
TAIL1 = 5
HEAD2 = 4
TAIL2 = 10
FIRST_HEAD = 4
FIRST_TAIL = 5
GATES = 1
SELF = 34
LAG = 10
K_ROWS = 256
G_COLS = 256
Q_ROWS = 256
O_ROWS = 256
O_COLS = 128
FIRST_LEAD = 13
FIRST_BATCHES = ((0, (0,)), (2, (1,)), (FIRST_LEAD, (2, 3)), (FIRST_LEAD + 2 * FIRST_HEAD, (4, 5)), (37, (6, 7)))
HALO = 16

F32 = jnp.float32
BF16 = jnp.bfloat16


def _dft_matrices():
    n = np.arange(C, dtype=np.float64)
    theta = np.pi * (4.0 * np.arange(C, dtype=np.float64) + 1.0) / (2.0 * C)
    plain = theta[:, None] * n[None, :]
    centred = theta[:, None] * (n[None, :] - (C - 1) / 2)
    inv = np.concatenate([np.cos(centred).T[:C // 2], -np.sin(centred).T[:C // 2]], 0) / C
    inv = inv.reshape(C // 16, 8, 2, C // 16, 2, 8).transpose(0, 2, 1, 3, 5, 4).reshape(C, C)
    return np.concatenate(
        [np.cos(plain), -np.sin(plain), np.cos(centred), -np.sin(centred), inv], 0).astype(np.float32)


_DFT = _dft_matrices()

_NT_DIMS = (((1,), (1,)), ((), ()))
_TN_DIMS = (((0,), (0,)), ((), ()))


def _packed(*shape):
    return pltpu.VMEM((*shape[:-2], shape[-2] // 2, shape[-1]), jnp.uint32)


def _phi(t):
    return jnp.where(t > 0, t + 1.0, jnp.exp(t)) + 1e-6


def _unpack(words, index):
    return pltpu.unpack_elementwise(words, index=index, packed_dtype=BF16, unpacked_dtype=F32)


def _rows(start, size):
    if isinstance(start, int):
        return pl.ds(start // 2, size // 2)
    return pl.ds(pl.multiple_of(start // 2, 8), size // 2)


def _lanes(g):
    return pl.ds(g * 128 if isinstance(g, int) else pl.multiple_of(g * 128, 128), 128)


def _bf16(words):
    return pltpu.bitcast(words, BF16)


def _words(x):
    return pltpu.bitcast(x.astype(BF16), jnp.uint32)


def _pack(lo, hi):
    return pltpu.pack_elementwise([lo, hi], packed_dtype=BF16).astype(jnp.uint32)


def _riffle(x):
    return jnp.concatenate(
        [_pack(x[i:i + 8], x[i + 8:i + 16]) for i in range(0, x.shape[0], 16)], 0)


def _flip(tile):
    return jnp.take_along_axis(tile, 7 - lax.broadcasted_iota(jnp.int32, (8, 128), 0), axis=0)


class _ConvGroup:
    def __init__(self, g, kb, vb, qb, skb, shift, skip, dft, kv_s, xp, kp, held, z_s, ob):
        self.g, self.kb, self.vb, self.qb, self.skb, self.shift, self.skip = (
            g, kb, vb, qb, skb, shift, skip)
        self.dft, self.kv_s, self.xp, self.kp, self.held, self.z_s, self.ob = (
            dft, kv_s, xp, kp, held, z_s, ob)
        self.prev = None

    def filter_spectrum(self, i):
        blk = jnp.concatenate(
            [_bf16(self.skb[self.g, :, m * C:(m + 1) * C]) for m in range(4 * i, 4 * i + 4)], 0)
        spec = lax.dot_general(_bf16(self.dft[_rows(0, 2 * C), :]), blk, _NT_DIMS,
                               preferred_element_type=F32)
        for j in range(4):
            re = spec[:C, j * 128:(j + 1) * 128]
            im = spec[C:, j * 128:(j + 1) * 128]
            if self.prev is None:
                re = re + self.skip[:, _lanes(self.g)]
                re2, im2 = re, im
            else:
                re2, im2 = re - self.prev[1], im + self.prev[0]
            self.prev = (re, im)
            self.kp[0, 4 * i + j] = re2
            self.kp[1, 4 * i + j] = im2

    def gate_keys(self, lo, hi):
        w = self.shift[:, _lanes(self.g)].astype(F32)
        w0, w1, w2, w3 = (jnp.broadcast_to(w[j:j + 1], (8, 128)) for j in range(4))
        for i in range(lo, hi):
            base = HALO // 2 + 8 * i
            p0 = self.kb[self.g, base:base + 8, :]
            p1 = self.kb[self.g, base - 1:base + 7, :]
            p2 = self.kb[self.g, base - 2:base + 6, :]
            pv = self.vb[self.g, 8 * i:8 * i + 8, :]
            e0, o0 = _unpack(p0, 0), _unpack(p0, 1)
            e1, o1 = _unpack(p1, 0), _unpack(p1, 1)
            o2 = _unpack(p2, 1)
            even = (w0 * e0 + w1 * o1 + w2 * e1 + w3 * o2) * _unpack(pv, 0)
            odd = (w0 * o0 + w1 * e0 + w2 * o1 + w3 * e1) * _unpack(pv, 1)
            self.kv_s[8 * i:8 * i + 8, :] = _pack(even, odd)

    def signal_spectrum(self, i):
        blk = jnp.concatenate(
            [_bf16(self.kv_s[_rows(c * C, C), :]) for c in range(4 * i, 4 * i + 4)], 1)
        spec = jnp.dot(_bf16(self.dft[_rows(2 * C, 2 * C), :]), blk, preferred_element_type=F32)
        for j in range(4):
            self.xp[0, 4 * i + j] = spec[:C, j * 128:(j + 1) * 128]
            self.xp[1, 4 * i + j] = spec[C:, j * 128:(j + 1) * 128]

    def combine(self):
        for r in range(C // 8):
            rows = slice(8 * r, 8 * r + 8)

            def product(outputs, signal, taps, init, subtract):
                ks, acc = {}, dict(init)
                for c in range(outputs[-1] + 1):
                    xc = signal(c)
                    for a in outputs:
                        if a < c:
                            continue
                        if a - c not in ks:
                            ks[a - c] = taps(self.kp[0, a - c, rows, :], self.kp[1, a - c, rows, :])
                        t = xc * ks[a - c]
                        if a not in acc:
                            acc[a] = t
                        else:
                            acc[a] = acc[a] - t if subtract else acc[a] + t
                        yield acc[a]
                return acc

            def keep(part, z):
                for a in z:
                    if r % 2 == 0:
                        self.held[part, a] = z[a]
                    else:
                        self.z_s[part, a, _rows(16 * (r // 2), 16), :] = _pack(self.held[part, a], z[a])

            def x_re(c):
                return self.xp[0, c, rows, :]

            def x_im(c):
                return self.xp[1, c, rows, :]

            for lo in range(0, NB, MAC_BLOCK):
                outputs = range(lo, lo + MAC_BLOCK)
                shared = yield from product(
                    outputs, lambda c: x_re(c) + x_im(c), lambda re, im: re, {}, False)
                keep(1, (yield from product(outputs, x_re, lambda re, im: im - re, shared, False)))
                keep(0, (yield from product(outputs, x_im, lambda re, im: im + re, shared, True)))

    def finish(self, i):
        cos, sin = (
            jnp.dot(_bf16(self.dft[_rows(4 * C + part * C // 2, C // 2), :]),
                    jnp.concatenate([_bf16(self.z_s[part, a]) for a in range(4 * i, 4 * i + 4)], 1),
                    preferred_element_type=F32)
            for part in range(2))
        for j in range(4):
            for u in range(C // 32):
                even = (slice(16 * u, 16 * u + 8), slice(j * 128, (j + 1) * 128))
                odd = (slice(16 * u + 8, 16 * u + 16), slice(j * 128, (j + 1) * 128))
                rows = _rows((4 * i + j) * C + 16 * u, 16)
                q = self.qb[self.g, rows, :]
                self.ob[self.g, rows, :] = _pack(
                    _unpack(q, 0) * (cos[even] + sin[even]), _unpack(q, 1) * (cos[odd] + sin[odd]))
                rows = _rows((4 * i + j + 1) * C - 16 * (u + 1), 16)
                q = _flip(self.qb[self.g, rows, :])
                self.ob[self.g, rows, :] = _flip(_pack(
                    _unpack(q, 0) * (cos[odd] - sin[odd]), _unpack(q, 1) * (cos[even] - sin[even])))


def _run_step(matmuls, conv, conv_done, pace, lead, head, tail, before_unit=lambda u: None):
    left = [UNITS]

    def matmul():
        before_unit(UNITS - left[0])
        left[0] -= 1
        return next(matmuls)

    for _ in range(lead):
        matmul()
    tiles = S // 16 // 4
    for i in range(4):
        conv.filter_spectrum(i)
        for u in range(head):
            matmul()
            if u == 0 and i > 0:
                conv.signal_spectrum(i - 1)
            conv.gate_keys(i * tiles + u * tiles // head, i * tiles + (u + 1) * tiles // head)
    matmul()
    conv.signal_spectrum(3)
    products = 3 * (C // 8) * NB * (NB + 1) // 2
    batches = (left[0] - tail) * GATES
    combine = conv.combine()
    for u in range(batches):
        if u % GATES == 0:
            result = matmul()
        if u:
            pace(result[u % GATES * 128 // GATES:][:8, :128])
        recent = []
        for i in range(u * products // batches, (u + 1) * products // batches):
            recent.append(next(combine))
            if SELF and len(recent) % SELF == 0:
                pace(recent[-LAG])
    for _ in combine:
        pass
    matmul()
    for i in range(4):
        conv.finish(i)
        conv_done(i)
        if left[0]:
            matmul()
    while left[0]:
        matmul()
    for _ in matmuls:
        pass


def _kernel(x_hbm, wqkv_hbm, wo_hbm, q_hbm, k_hbm, v_hbm, shift_hbm, sk_hbm, d_hbm, dft_hbm,
            out_hbm,
            x_v, w_v, wo_v, wkt, wqt, g_acc, z_acc, m_v, pk_s, o_s, oa,
            kb, vb, qb, skb, shift_v, d_v, skip_s, dft, kv_s, xp, kp, held, z_s, ob, zero,
            sem_x, sem_w, sem_first, sem_b, sem_oa, sem_ob):

    def tile_rows(t):
        return pl.ds(t * ST if isinstance(t, int) else pl.multiple_of(t * ST, ST), ST)

    def x_copy(t):
        return pltpu.make_async_copy(
            x_hbm.at[tile_rows(t), :], x_v.bitcast(BF16).at[tile_rows(t), :], sem_x.at[t])

    def w_copy(j):
        return pltpu.make_async_copy(
            wqkv_hbm.at[:, pl.ds(j * D, D)], w_v.bitcast(BF16).at[j], sem_w.at[j])

    def wo_copy():
        return pltpu.make_async_copy(wo_hbm, wo_v.bitcast(BF16), sem_w.at[1])

    def b_copy(g, i):
        lanes = _lanes(g)
        src, dst = (
            (sk_hbm.at[lanes, :], skb.bitcast(BF16).at[g]),
            (k_hbm.at[:, lanes], kb.bitcast(BF16).at[g, pl.ds(HALO, S), :]),
            (v_hbm.at[:, lanes], vb.bitcast(BF16).at[g]),
            (q_hbm.at[:, lanes], qb.bitcast(BF16).at[g]),
        )[i]
        return pltpu.make_async_copy(src, dst, sem_b.at[g, i])

    def b_copies(g):
        return [b_copy(g, i) for i in range(4)]

    def oa_copy(t, j):
        cols = pl.ds(j * O_COLS, O_COLS)
        return pltpu.make_async_copy(
            oa.at[tile_rows(t), cols], out_hbm.at[tile_rows(t), cols], sem_oa.at[t, j])

    def ob_copy(g, i):
        rows = pl.ds(i * S // 4, S // 4)
        return pltpu.make_async_copy(
            ob.bitcast(BF16).at[g, rows, :], out_hbm.at[rows, _lanes(NG + g)], sem_ob.at[g, i])

    def first_batch(b):
        def wk(lo, hi, sem):
            return pltpu.make_async_copy(
                wqkv_hbm.at[:, pl.ds(D + lo * 128, (hi - lo) * 128)],
                w_v.bitcast(BF16).at[1, :, pl.ds(lo * 128, (hi - lo) * 128)], sem_first.at[sem])

        def x(lo, hi, sem):
            rows = pl.ds(lo * 128, (hi - lo) * 128)
            return pltpu.make_async_copy(
                x_hbm.at[rows, :], x_v.bitcast(BF16).at[rows, :], sem_first.at[sem])

        def conv_half(h, sem):
            lanes, span = pl.ds(0, 128), pl.ds(h * S // 2, S // 2)
            return [
                pltpu.make_async_copy(
                    sk_hbm.at[lanes, span], skb.bitcast(BF16).at[0, :, span], sem_first.at[sem]),
                pltpu.make_async_copy(
                    k_hbm.at[span, lanes], kb.bitcast(BF16).at[0, pl.ds(HALO + h * S // 2, S // 2), :],
                    sem_first.at[sem + 1]),
                pltpu.make_async_copy(
                    v_hbm.at[span, lanes], vb.bitcast(BF16).at[0, span, :], sem_first.at[sem + 2]),
            ]

        if b == 0:
            return [wk(0, 1, 0), x(0, 2, 1)]
        if b == 1:
            return [x(2, ST // 128, 2), wk(1, 2, 3)]
        if b == 2:
            return [wk(2, 4, 4)] + conv_half(0, 5) + [
                pltpu.make_async_copy(dft_hbm, dft.bitcast(BF16), sem_first.at[13]),
                pltpu.make_async_copy(shift_hbm, shift_v, sem_first.at[14]),
                pltpu.make_async_copy(d_hbm, d_v, sem_first.at[15])]
        if b == 3:
            return conv_half(1, 8) + [wk(4, 6, 11)]
        return [wk(6, 8, 12), b_copy(0, 3)]

    def later_inputs():
        copies = []
        for t, weight in zip(range(1, NT), (w_copy(2), wo_copy(), w_copy(0))):
            copies += [x_copy(t)] + b_copies(t) + [weight]
        for g in range(NT, NG):
            copies += b_copies(g)
        return copies

    def conv(g):
        return _ConvGroup(g, kb, vb, qb, skb, shift_v, skip_s, dft, kv_s, xp, kp, held, z_s, ob)

    def transpose_weight(j, dst, i):
        dst[_rows(i * 128, 128), :] = _words(_bf16(w_v[j, :, i * 128:(i + 1) * 128]).T)

    def pace(tile):
        xp[2, 0, pl.ds(pl.multiple_of(zero[0], 8), 8), :] = tile

    for cp in first_batch(0) + first_batch(1):
        cp.start()
    zero[0] = 0
    for g in range(NG):
        kb[g, 0:HALO // 2, :] = jnp.zeros((HALO // 2, 128), jnp.uint32)

    def pieces(result):
        height, width = result.shape
        for i in range(max(height // 128, 1)):
            for j in range(width // 128):
                yield result[i * 128:, j * 128:]

    def keys(t, first):
        def project(lo, height):
            pk = []
            for n in range(ST // 128):
                xs = _bf16(x_v[_rows(t * ST + n * 128, 128), :])
                pk.append(_phi(lax.dot_general(
                    _bf16(wkt[_rows(lo, height), :]), xs, _NT_DIMS, preferred_element_type=F32)))
                if n == ST // 128 - 1:
                    rows, total = slice(lo, lo + height), sum(pk[1:], pk[0])
                    z_acc[rows, :] = total if first else z_acc[rows, :] + total
                    pk_s[_rows(lo, height), :] = _riffle(jnp.concatenate(pk, 1))
                yield from pieces(pk[-1])

        def accumulate(lo, height):
            width = max(G_COLS, 256 * 128 // height)
            for n in range(D // width):
                rows, cols = slice(lo, lo + height), slice(n * width, (n + 1) * width)
                g = jnp.dot(_bf16(pk_s[_rows(lo, height), :]), _bf16(x_v[_rows(t * ST, ST), cols]),
                            preferred_element_type=F32)
                g_acc[rows, cols] = g if first else g_acc[rows, cols] + g
                yield from list(pieces(g))[::2]

        if first:
            for part in (project, accumulate):
                for lo in (0, 128):
                    yield from part(lo, 128)
        starts = range(K_ROWS if first else 0, D, K_ROWS)
        yield from project(starts[0], K_ROWS)
        for lo in starts[1:]:
            yield from project(lo, K_ROWS)
            yield from accumulate(lo - K_ROWS, K_ROWS)
        yield from accumulate(starts[-1], K_ROWS)

    def arrivals(unit):
        for b, (at, chunks) in enumerate(FIRST_BATCHES):
            if unit == at:
                for cp in first_batch(b):
                    cp.wait()
                ahead = first_batch(b + 2) if b + 2 < len(FIRST_BATCHES) else []
                for cp in ahead + (later_inputs() if b + 3 == len(FIRST_BATCHES) else []):
                    cp.start()
                for i in chunks:
                    transpose_weight(1, wkt, i)
                if b == 2:
                    skip_s[...] = d_v[...].astype(F32).reshape(1, D)

    _run_step(keys(0, True), conv(0), lambda i: ob_copy(0, i).start(), pace,
              FIRST_BATCHES[2][0] + 1, FIRST_HEAD, FIRST_TAIL, arrivals)

    def phase1(t, carry):
        for cp in [x_copy(t)] + b_copies(t):
            cp.wait()
        _run_step(keys(t, False), conv(t), lambda i: ob_copy(t, i).start(), pace, 0, HEAD1, TAIL1)
        return carry

    lax.fori_loop(1, NT, phase1, 0)

    for cp in (w_copy(2), wo_copy(), w_copy(0)):
        cp.wait()
    same_head = (lax.broadcasted_iota(jnp.int32, (128, 128), 0) // DH
                 == lax.broadcasted_iota(jnp.int32, (128, 128), 1) // DH)
    kvs = []
    for i in range(D // 128):
        blk = slice(i * 128, (i + 1) * 128)
        kv = jnp.dot(g_acc[blk, :].astype(BF16), _bf16(w_v[2, :, blk]), preferred_element_type=F32)
        kvs.append(jnp.where(same_head, kv, 0.0).astype(BF16))
        transpose_weight(0, wqt, i)
    for i in range(D // 128):
        m_v[_rows(i * 128, 128), :] = _words(
            jnp.dot(kvs[i], _bf16(wo_v[_rows(i * 128, 128), :]), preferred_element_type=F32))
    z_acc[...] = jnp.broadcast_to(jnp.sum(z_acc[...], axis=1, keepdims=True), (D, 128))

    def queries(t):
        for n in range(ST // 128):
            xs = _bf16(x_v[_rows(t * ST + n * 128, 128), :])
            for j in range(D // Q_ROWS):
                chans = slice(j * Q_ROWS, (j + 1) * Q_ROWS)
                pq = _phi(lax.dot_general(
                    _bf16(wqt[_rows(j * Q_ROWS, Q_ROWS), :]), xs, _NT_DIMS, preferred_element_type=F32))
                pz = (pq * z_acc[chans, :]).reshape(Q_ROWS // DH, DH, 128)
                den = jnp.sum(pz, axis=1, keepdims=True) + 1e-6
                o = (pq.reshape(Q_ROWS // DH, DH, 128) * (1.0 / den)).reshape(Q_ROWS, 128)
                o_s[_rows(n * 128, 128), chans] = _words(_bf16(_riffle(o)).T)
                yield from pieces(pq)
        for j in range(D // O_COLS):
            cols = slice(j * O_COLS, (j + 1) * O_COLS)
            for n in range(ST // O_ROWS):
                rows = _rows(n * O_ROWS, O_ROWS)
                res = jnp.dot(_bf16(o_s[rows, :]), _bf16(m_v[:, cols]), preferred_element_type=F32)
                oa[pl.ds(pl.multiple_of(t * ST + n * O_ROWS, O_ROWS), O_ROWS), cols] = res.astype(BF16)
                if n == ST // O_ROWS - 1:
                    oa_copy(t, j).start()
                yield from pieces(res)

    def phase2(t, carry):
        for cp in b_copies(NT + t):
            cp.wait()
        _run_step(queries(t), conv(NT + t), lambda i: ob_copy(NT + t, i).start(), pace,
                  0, HEAD2, TAIL2)
        return carry

    lax.fori_loop(0, NT, phase2, 0)
    for g in range(NG):
        for i in range(4):
            ob_copy(g, i).wait()
    for t in range(NT):
        for j in range(D // O_COLS):
            oa_copy(t, j).wait()


@jax.jit
def pallas_concat_heads__linear_attn_block__ssm_conv_h3__prompt_kernel(
    A_x: jax.Array,
    A_wqkv: jax.Array,
    A_wo: jax.Array,
    B_q: jax.Array,
    B_k: jax.Array,
    B_v: jax.Array,
    B_shift_k: jax.Array,
    B_ssm_k: jax.Array,
    B_ssm_D: jax.Array,
):
    assert A_x.shape == (1, S, D) and B_shift_k.shape == (D, 4) and NG == 2 * NT
    hbm = pl.BlockSpec(memory_space=pl.ANY)
    out = pl.pallas_call(
        _kernel,
        out_shape=jax.ShapeDtypeStruct((S, 2 * D), BF16),
        in_specs=[hbm] * 10,
        out_specs=hbm,
        scratch_shapes=[
            _packed(S, D),
            _packed(3, D, D),
            _packed(D, D),
            _packed(D, D),
            _packed(D, D),
            pltpu.VMEM((D, D), F32),
            pltpu.VMEM((D, 128), F32),
            _packed(D, D),
            _packed(D, ST),
            _packed(ST, D),
            pltpu.VMEM((S, D), BF16),
            _packed(NG, HALO + S, 128),
            _packed(NG, S, 128),
            _packed(NG, S, 128),
            _packed(NG, 128, S),
            pltpu.VMEM((4, D), BF16),
            pltpu.VMEM((D,), BF16),
            pltpu.VMEM((1, D), F32),
            _packed(5 * C, C),
            _packed(S, 128),
            pltpu.VMEM((3, NB, C, 128), F32),
            pltpu.VMEM((2, NB, C, 128), F32),
            pltpu.VMEM((2, NB, 8, 128), F32),
            _packed(2, NB, C, 128),
            _packed(NG, S, 128),
            pltpu.SMEM((1,), jnp.int32),
            pltpu.SemaphoreType.DMA((NT,)),
            pltpu.SemaphoreType.DMA((3,)),
            pltpu.SemaphoreType.DMA((16,)),
            pltpu.SemaphoreType.DMA((NG, 4)),
            pltpu.SemaphoreType.DMA((NT, D // O_COLS)),
            pltpu.SemaphoreType.DMA((NG, 4)),
        ],
        compiler_params=pltpu.CompilerParams(vmem_limit_bytes=100 * 2**20),
        name="linattn_h3",
    )(
        A_x.reshape(S, D), A_wqkv, A_wo,
        B_q.reshape(S, D), B_k.reshape(S, D), B_v.reshape(S, D),
        B_shift_k.T, B_ssm_k, B_ssm_D,
        jnp.asarray(_DFT, BF16),
    )
    return out.reshape(1, S, 2 * D)
```

```python
import jax
import jax.numpy as jnp
import numpy as np
from jax import lax
import jax.experimental.pallas as pl
import jax.experimental.pallas.tpu as pltpu

S = 2048
D = 1024
DH = 32
C = 128
NB = S // C
NG = D // 128
ST = 512
NT = S // ST
UNITS = 2 * (ST // 128) * (D // 128)
MAC_BLOCK = 16
HEAD1 = 4
TAIL1 = 5
HEAD2 = 4
TAIL2 = 8
FIRST_HEAD = 4
FIRST_TAIL = 5
SELF0 = 34
LAG0 = 10
SELF1 = 34
LAG1 = 10
SELF2 = 34
LAG2 = 10
K_ROWS = 256
G_COLS = 256
Q_ROWS = 256
O_ROWS = 256
O_COLS = 128
FIRST_LEAD = 13
FIRST_BATCHES = ((0, (0,)), (2, (1,)), (FIRST_LEAD, (2, 3)), (FIRST_LEAD + 2 * FIRST_HEAD, (4, 5)), (37, (6, 7)))
EDGES = 2
OUT_EDGES = ((0, 768, 896, D), (0, 896, D), (0, 512, 896, D), tuple(range(0, D + 1, 128)))[EDGES]
HALO = 16

F32 = jnp.float32
BF16 = jnp.bfloat16


def _dft_matrices():
    n = np.arange(C, dtype=np.float64)
    theta = np.pi * (4.0 * np.arange(C, dtype=np.float64) + 1.0) / (2.0 * C)
    plain = theta[:, None] * n[None, :]
    centred = theta[:, None] * (n[None, :] - (C - 1) / 2)
    inv = np.concatenate([np.cos(centred).T[:C // 2], -np.sin(centred).T[:C // 2]], 0) / C
    inv = inv.reshape(C // 16, 8, 2, C // 16, 2, 8).transpose(0, 2, 1, 3, 5, 4).reshape(C, C)
    return np.concatenate(
        [np.cos(plain), -np.sin(plain), np.cos(centred), -np.sin(centred), inv], 0).astype(BF16)


_DFT = _dft_matrices()

_NT_DIMS = (((1,), (1,)), ((), ()))
_TN_DIMS = (((0,), (0,)), ((), ()))


def _packed(*shape):
    return pltpu.VMEM((*shape[:-2], shape[-2] // 2, shape[-1]), jnp.uint32)


def _phi(t):
    return jnp.where(t > 0, t + 1.0, jnp.exp(t)) + 1e-6


def _unpack(words, index):
    return pltpu.unpack_elementwise(words, index=index, packed_dtype=BF16, unpacked_dtype=F32)


def _rows(start, size):
    if isinstance(start, int):
        return pl.ds(start // 2, size // 2)
    return pl.ds(pl.multiple_of(start // 2, 8), size // 2)


def _lanes(g):
    return pl.ds(g * 128 if isinstance(g, int) else pl.multiple_of(g * 128, 128), 128)


def _bf16(words):
    return pltpu.bitcast(words, BF16)


def _words(x):
    return pltpu.bitcast(x.astype(BF16), jnp.uint32)


def _pack(lo, hi):
    return pltpu.pack_elementwise([lo, hi], packed_dtype=BF16).astype(jnp.uint32)


def _riffle(x):
    return jnp.concatenate(
        [_pack(x[i:i + 8], x[i + 8:i + 16]) for i in range(0, x.shape[0], 16)], 0)


def _flip(tile):
    return jnp.take_along_axis(tile, 7 - lax.broadcasted_iota(jnp.int32, (8, 128), 0), axis=0)


class _ConvGroup:
    def __init__(self, g, kb, vb, qb, skb, shift, skip, dft, kv_s, xp, kp, held, z_s, ob):
        self.g, self.kb, self.vb, self.qb, self.skb, self.shift, self.skip = (
            g, kb, vb, qb, skb, shift, skip)
        self.dft, self.kv_s, self.xp, self.kp, self.held, self.z_s, self.ob = (
            dft, kv_s, xp, kp, held, z_s, ob)
        self.prev = None

    def filter_spectrum(self, i):
        blk = jnp.concatenate(
            [_bf16(self.skb[self.g, :, m * C:(m + 1) * C]) for m in range(4 * i, 4 * i + 4)], 0)
        spec = lax.dot_general(_bf16(self.dft[_rows(0, 2 * C), :]), blk, _NT_DIMS,
                               preferred_element_type=F32)
        for j in range(4):
            re = spec[:C, j * 128:(j + 1) * 128]
            im = spec[C:, j * 128:(j + 1) * 128]
            if self.prev is None:
                re = re + self.skip[:, _lanes(self.g)]
                re2, im2 = re, im
            else:
                re2, im2 = re - self.prev[1], im + self.prev[0]
            self.prev = (re, im)
            self.kp[0, 4 * i + j] = re2
            self.kp[1, 4 * i + j] = im2

    def gate_keys(self, lo, hi):
        w = self.shift[:, _lanes(self.g)].astype(F32)
        w0, w1, w2, w3 = (jnp.broadcast_to(w[j:j + 1], (8, 128)) for j in range(4))
        for i in range(lo, hi):
            base = HALO // 2 + 8 * i
            p0 = self.kb[self.g, base:base + 8, :]
            p1 = self.kb[self.g, base - 1:base + 7, :]
            p2 = self.kb[self.g, base - 2:base + 6, :]
            pv = self.vb[self.g, 8 * i:8 * i + 8, :]
            e0, o0 = _unpack(p0, 0), _unpack(p0, 1)
            e1, o1 = _unpack(p1, 0), _unpack(p1, 1)
            o2 = _unpack(p2, 1)
            even = (w0 * e0 + w1 * o1 + w2 * e1 + w3 * o2) * _unpack(pv, 0)
            odd = (w0 * o0 + w1 * e0 + w2 * o1 + w3 * e1) * _unpack(pv, 1)
            self.kv_s[8 * i:8 * i + 8, :] = _pack(even, odd)

    def signal_spectrum(self, i):
        blk = jnp.concatenate(
            [_bf16(self.kv_s[_rows(c * C, C), :]) for c in range(4 * i, 4 * i + 4)], 1)
        spec = jnp.dot(_bf16(self.dft[_rows(2 * C, 2 * C), :]), blk, preferred_element_type=F32)
        for j in range(4):
            self.xp[0, 4 * i + j] = spec[:C, j * 128:(j + 1) * 128]
            self.xp[1, 4 * i + j] = spec[C:, j * 128:(j + 1) * 128]

    def combine(self):
        for r in range(C // 8):
            rows = slice(8 * r, 8 * r + 8)

            def product(outputs, signal, taps, init, subtract):
                ks, acc = {}, dict(init)
                for c in range(outputs[-1] + 1):
                    xc = signal(c)
                    for a in outputs:
                        if a < c:
                            continue
                        if a - c not in ks:
                            ks[a - c] = taps(self.kp[0, a - c, rows, :], self.kp[1, a - c, rows, :])
                        t = xc * ks[a - c]
                        if a not in acc:
                            acc[a] = t
                        else:
                            acc[a] = acc[a] - t if subtract else acc[a] + t
                        yield acc[a]
                return acc

            def keep(part, z):
                for a in z:
                    if r % 2 == 0:
                        self.held[part, a] = z[a]
                    else:
                        self.z_s[part, a, _rows(16 * (r // 2), 16), :] = _pack(self.held[part, a], z[a])

            def x_re(c):
                return self.xp[0, c, rows, :]

            def x_im(c):
                return self.xp[1, c, rows, :]

            for lo in range(0, NB, MAC_BLOCK):
                outputs = range(lo, lo + MAC_BLOCK)
                shared = yield from product(
                    outputs, lambda c: x_re(c) + x_im(c), lambda re, im: re, {}, False)
                keep(1, (yield from product(outputs, x_re, lambda re, im: im - re, shared, False)))
                keep(0, (yield from product(outputs, x_im, lambda re, im: im + re, shared, True)))

    def finish(self, i):
        cos, sin = (
            jnp.dot(_bf16(self.dft[_rows(4 * C + part * C // 2, C // 2), :]),
                    jnp.concatenate([_bf16(self.z_s[part, a]) for a in range(4 * i, 4 * i + 4)], 1),
                    preferred_element_type=F32)
            for part in range(2))
        for j in range(4):
            for u in range(C // 32):
                even = (slice(16 * u, 16 * u + 8), slice(j * 128, (j + 1) * 128))
                odd = (slice(16 * u + 8, 16 * u + 16), slice(j * 128, (j + 1) * 128))
                rows = _rows((4 * i + j) * C + 16 * u, 16)
                q = self.qb[self.g, rows, :]
                self.ob[self.g, rows, :] = _pack(
                    _unpack(q, 0) * (cos[even] + sin[even]), _unpack(q, 1) * (cos[odd] + sin[odd]))
                rows = _rows((4 * i + j + 1) * C - 16 * (u + 1), 16)
                q = _flip(self.qb[self.g, rows, :])
                self.ob[self.g, rows, :] = _flip(_pack(
                    _unpack(q, 0) * (cos[odd] - sin[odd]), _unpack(q, 1) * (cos[even] - sin[even])))


def _run_step(matmuls, conv, conv_done, pace, lead, head, tail, every, lag, before_unit=lambda u: None):
    left = [UNITS]

    def matmul():
        before_unit(UNITS - left[0])
        left[0] -= 1
        return next(matmuls)

    for _ in range(lead):
        matmul()
    tiles = S // 16 // 4
    for i in range(4):
        conv.filter_spectrum(i)
        for u in range(head):
            matmul()
            if u == 0 and i > 0:
                conv.signal_spectrum(i - 1)
            conv.gate_keys(i * tiles + u * tiles // head, i * tiles + (u + 1) * tiles // head)
    matmul()
    conv.signal_spectrum(3)
    products = 3 * (C // 8) * NB * (NB + 1) // 2
    batches = left[0] - tail
    combine = conv.combine()
    for u in range(batches):
        result = matmul()
        if u:
            pace(result[:8, :128])
        recent = []
        for i in range(u * products // batches, (u + 1) * products // batches):
            recent.append(next(combine))
            if len(recent) % every == 0:
                pace(recent[-lag])
    for _ in combine:
        pass
    matmul()
    for i in range(4):
        conv.finish(i)
        conv_done(i)
        if left[0]:
            matmul()
    while left[0]:
        matmul()
    for _ in matmuls:
        pass


def _kernel(x_hbm, wqkv_hbm, wo_hbm, q_hbm, k_hbm, v_hbm, shift_hbm, sk_hbm, d_hbm, dft_hbm,
            out_hbm,
            x_v, w_v, wo_v, wkt, wqt, g_acc, z_acc, m_v, pk_s, o_s, oa,
            kb, vb, qb, skb, shift_v, d_v, skip_s, dft, kv_s, xp, kp, held, z_s, ob, zero,
            sem_x, sem_w, sem_first, sem_b, sem_oa, sem_ob):

    def tile_rows(t):
        return pl.ds(t * ST if isinstance(t, int) else pl.multiple_of(t * ST, ST), ST)

    def x_copy(t):
        return pltpu.make_async_copy(
            x_hbm.at[tile_rows(t), :], x_v.bitcast(BF16).at[tile_rows(t), :], sem_x.at[t])

    def w_copy(j):
        return pltpu.make_async_copy(
            wqkv_hbm.at[:, pl.ds(j * D, D)], w_v.bitcast(BF16).at[j], sem_w.at[j])

    def wo_copy():
        return pltpu.make_async_copy(wo_hbm, wo_v.bitcast(BF16), sem_w.at[1])

    def b_copy(g, i):
        lanes = _lanes(g)
        src, dst = (
            (sk_hbm.at[lanes, :], skb.bitcast(BF16).at[g]),
            (k_hbm.at[:, lanes], kb.bitcast(BF16).at[g, pl.ds(HALO, S), :]),
            (v_hbm.at[:, lanes], vb.bitcast(BF16).at[g]),
            (q_hbm.at[:, lanes], qb.bitcast(BF16).at[g]),
        )[i]
        return pltpu.make_async_copy(src, dst, sem_b.at[g, i])

    def b_copies(g):
        return [b_copy(g, i) for i in range(4)]

    def oa_copy(t, j):
        cols = pl.ds(OUT_EDGES[j], OUT_EDGES[j + 1] - OUT_EDGES[j])
        return pltpu.make_async_copy(
            oa.at[tile_rows(t), cols], out_hbm.at[tile_rows(t), cols], sem_oa.at[t, j])

    def ob_copy(g, i):
        rows = pl.ds(i * S // 4, S // 4)
        return pltpu.make_async_copy(
            ob.bitcast(BF16).at[g, rows, :], out_hbm.at[rows, _lanes(NG + g)], sem_ob.at[g, i])

    def first_batch(b):
        def wk(lo, hi, sem):
            return pltpu.make_async_copy(
                wqkv_hbm.at[:, pl.ds(D + lo * 128, (hi - lo) * 128)],
                w_v.bitcast(BF16).at[1, :, pl.ds(lo * 128, (hi - lo) * 128)], sem_first.at[sem])

        def x(lo, hi, sem):
            rows = pl.ds(lo * 128, (hi - lo) * 128)
            return pltpu.make_async_copy(
                x_hbm.at[rows, :], x_v.bitcast(BF16).at[rows, :], sem_first.at[sem])

        def conv_half(h, sem):
            lanes, span = pl.ds(0, 128), pl.ds(h * S // 2, S // 2)
            return [
                pltpu.make_async_copy(
                    sk_hbm.at[lanes, span], skb.bitcast(BF16).at[0, :, span], sem_first.at[sem]),
                pltpu.make_async_copy(
                    k_hbm.at[span, lanes], kb.bitcast(BF16).at[0, pl.ds(HALO + h * S // 2, S // 2), :],
                    sem_first.at[sem + 1]),
                pltpu.make_async_copy(
                    v_hbm.at[span, lanes], vb.bitcast(BF16).at[0, span, :], sem_first.at[sem + 2]),
            ]

        if b == 0:
            return [wk(0, 1, 0), x(0, 2, 1)]
        if b == 1:
            return [x(2, ST // 128, 2), wk(1, 2, 3)]
        if b == 2:
            return [wk(2, 4, 4)] + conv_half(0, 5) + [
                pltpu.make_async_copy(dft_hbm, dft.bitcast(BF16), sem_first.at[13]),
                pltpu.make_async_copy(shift_hbm, shift_v, sem_first.at[14]),
                pltpu.make_async_copy(d_hbm, d_v, sem_first.at[15])]
        if b == 3:
            return conv_half(1, 8) + [wk(4, 6, 11)]
        return [wk(6, 8, 12), b_copy(0, 3)]

    def later_inputs():
        copies = []
        for t, weight in zip(range(1, NT), (w_copy(2), wo_copy(), w_copy(0))):
            copies += [x_copy(t)] + b_copies(t) + [weight]
        for g in range(NT, NG):
            copies += b_copies(g)
        return copies

    def conv(g):
        return _ConvGroup(g, kb, vb, qb, skb, shift_v, skip_s, dft, kv_s, xp, kp, held, z_s, ob)

    def transpose_weight(j, dst, i):
        dst[_rows(i * 128, 128), :] = _words(_bf16(w_v[j, :, i * 128:(i + 1) * 128]).T)

    def pace(tile):
        xp[2, 0, pl.ds(pl.multiple_of(zero[0], 8), 8), :] = tile

    for cp in first_batch(0) + first_batch(1):
        cp.start()
    zero[0] = 0
    for g in range(NG):
        kb[g, 0:HALO // 2, :] = jnp.zeros((HALO // 2, 128), jnp.uint32)

    def pieces(result):
        height, width = result.shape
        for i in range(max(height // 128, 1)):
            for j in range(width // 128):
                yield result[i * 128:, j * 128:]

    def keys(t, first):
        def project(lo, height):
            pk = []
            for n in range(ST // 128):
                xs = _bf16(x_v[_rows(t * ST + n * 128, 128), :])
                pk.append(_phi(lax.dot_general(
                    _bf16(wkt[_rows(lo, height), :]), xs, _NT_DIMS, preferred_element_type=F32)))
                if n == ST // 128 - 1:
                    rows, total = slice(lo, lo + height), sum(pk[1:], pk[0])
                    z_acc[rows, :] = total if first else z_acc[rows, :] + total
                    pk_s[_rows(lo, height), :] = _riffle(jnp.concatenate(pk, 1))
                yield from pieces(pk[-1])

        def accumulate(lo, height):
            width = max(G_COLS, 256 * 128 // height)
            for n in range(D // width):
                rows, cols = slice(lo, lo + height), slice(n * width, (n + 1) * width)
                g = jnp.dot(_bf16(pk_s[_rows(lo, height), :]), _bf16(x_v[_rows(t * ST, ST), cols]),
                            preferred_element_type=F32)
                g_acc[rows, cols] = g if first else g_acc[rows, cols] + g
                yield from list(pieces(g))[::2]

        if first:
            for part in (project, accumulate):
                for lo in (0, 128):
                    yield from part(lo, 128)
        starts = range(K_ROWS if first else 0, D, K_ROWS)
        yield from project(starts[0], K_ROWS)
        for lo in starts[1:]:
            yield from project(lo, K_ROWS)
            yield from accumulate(lo - K_ROWS, K_ROWS)
        yield from accumulate(starts[-1], K_ROWS)

    def arrivals(unit):
        for b, (at, chunks) in enumerate(FIRST_BATCHES):
            if unit == at:
                for cp in first_batch(b):
                    cp.wait()
                ahead = first_batch(b + 2) if b + 2 < len(FIRST_BATCHES) else []
                for cp in ahead + (later_inputs() if b + 3 == len(FIRST_BATCHES) else []):
                    cp.start()
                for i in chunks:
                    transpose_weight(1, wkt, i)
                if b == 2:
                    skip_s[...] = d_v[...].astype(F32).reshape(1, D)

    _run_step(keys(0, True), conv(0), lambda i: ob_copy(0, i).start(), pace,
              FIRST_BATCHES[2][0] + 1, FIRST_HEAD, FIRST_TAIL, SELF0, LAG0, arrivals)

    def phase1(t, carry):
        for cp in [x_copy(t)] + b_copies(t):
            cp.wait()
        _run_step(keys(t, False), conv(t), lambda i: ob_copy(t, i).start(), pace, 0, HEAD1, TAIL1, SELF1, LAG1)
        return carry

    lax.fori_loop(1, NT, phase1, 0)

    for cp in (w_copy(2), wo_copy(), w_copy(0)):
        cp.wait()
    same_head = (lax.broadcasted_iota(jnp.int32, (128, 128), 0) // DH
                 == lax.broadcasted_iota(jnp.int32, (128, 128), 1) // DH)
    kvs = []
    for i in range(D // 128):
        blk = slice(i * 128, (i + 1) * 128)
        kv = jnp.dot(g_acc[blk, :].astype(BF16), _bf16(w_v[2, :, blk]), preferred_element_type=F32)
        kvs.append(jnp.where(same_head, kv, 0.0).astype(BF16))
        transpose_weight(0, wqt, i)
    for i in range(D // 128):
        m_v[_rows(i * 128, 128), :] = _words(
            jnp.dot(kvs[i], _bf16(wo_v[_rows(i * 128, 128), :]), preferred_element_type=F32))
    z_acc[...] = jnp.broadcast_to(jnp.sum(z_acc[...], axis=1, keepdims=True), (D, 128))

    def queries(t):
        for n in range(ST // 128):
            xs = _bf16(x_v[_rows(t * ST + n * 128, 128), :])
            for j in range(D // Q_ROWS):
                chans = slice(j * Q_ROWS, (j + 1) * Q_ROWS)
                pq = _phi(lax.dot_general(
                    _bf16(wqt[_rows(j * Q_ROWS, Q_ROWS), :]), xs, _NT_DIMS, preferred_element_type=F32))
                pz = (pq * z_acc[chans, :]).reshape(Q_ROWS // DH, DH, 128)
                den = jnp.sum(pz, axis=1, keepdims=True) + 1e-6
                o = (pq.reshape(Q_ROWS // DH, DH, 128) * (1.0 / den)).reshape(Q_ROWS, 128)
                o_s[_rows(n * 128, 128), chans] = _words(_bf16(_riffle(o)).T)
                yield from pieces(pq)
        for j in range(D // O_COLS):
            cols = slice(j * O_COLS, (j + 1) * O_COLS)
            for n in range(ST // O_ROWS):
                rows = _rows(n * O_ROWS, O_ROWS)
                res = jnp.dot(_bf16(o_s[rows, :]), _bf16(m_v[:, cols]), preferred_element_type=F32)
                oa[pl.ds(pl.multiple_of(t * ST + n * O_ROWS, O_ROWS), O_ROWS), cols] = res.astype(BF16)
                if n == ST // O_ROWS - 1 and cols.stop in OUT_EDGES:
                    oa_copy(t, OUT_EDGES.index(cols.stop) - 1).start()
                yield from pieces(res)

    def phase2(t, carry):
        for cp in b_copies(NT + t):
            cp.wait()
        _run_step(queries(t), conv(NT + t), lambda i: ob_copy(NT + t, i).start(), pace,
                  0, HEAD2, TAIL2, SELF2, LAG2)
        return carry

    lax.fori_loop(0, NT, phase2, 0)
    for g in range(NG):
        for i in range(4):
            ob_copy(g, i).wait()
    for t in range(NT):
        for j in range(len(OUT_EDGES) - 1):
            oa_copy(t, j).wait()


@jax.jit
def pallas_concat_heads__linear_attn_block__ssm_conv_h3__prompt_kernel(
    A_x: jax.Array,
    A_wqkv: jax.Array,
    A_wo: jax.Array,
    B_q: jax.Array,
    B_k: jax.Array,
    B_v: jax.Array,
    B_shift_k: jax.Array,
    B_ssm_k: jax.Array,
    B_ssm_D: jax.Array,
):
    assert A_x.shape == (1, S, D) and B_shift_k.shape == (D, 4) and NG == 2 * NT
    hbm = pl.BlockSpec(memory_space=pl.ANY)
    out = pl.pallas_call(
        _kernel,
        out_shape=jax.ShapeDtypeStruct((S, 2 * D), BF16),
        in_specs=[hbm] * 10,
        out_specs=hbm,
        scratch_shapes=[
            _packed(S, D),
            _packed(3, D, D),
            _packed(D, D),
            _packed(D, D),
            _packed(D, D),
            pltpu.VMEM((D, D), F32),
            pltpu.VMEM((D, 128), F32),
            _packed(D, D),
            _packed(D, ST),
            _packed(ST, D),
            pltpu.VMEM((S, D), BF16),
            _packed(NG, HALO + S, 128),
            _packed(NG, S, 128),
            _packed(NG, S, 128),
            _packed(NG, 128, S),
            pltpu.VMEM((4, D), BF16),
            pltpu.VMEM((D,), BF16),
            pltpu.VMEM((1, D), F32),
            _packed(5 * C, C),
            _packed(S, 128),
            pltpu.VMEM((3, NB, C, 128), F32),
            pltpu.VMEM((2, NB, C, 128), F32),
            pltpu.VMEM((2, NB, 8, 128), F32),
            _packed(2, NB, C, 128),
            _packed(NG, S, 128),
            pltpu.SMEM((1,), jnp.int32),
            pltpu.SemaphoreType.DMA((NT,)),
            pltpu.SemaphoreType.DMA((3,)),
            pltpu.SemaphoreType.DMA((16,)),
            pltpu.SemaphoreType.DMA((NG, 4)),
            pltpu.SemaphoreType.DMA((NT, len(OUT_EDGES) - 1)),
            pltpu.SemaphoreType.DMA((NG, 4)),
        ],
        compiler_params=pltpu.CompilerParams(vmem_limit_bytes=100 * 2**20),
        name="linattn_h3",
    )(
        A_x.reshape(S, D), A_wqkv, A_wo,
        B_q.reshape(S, D), B_k.reshape(S, D), B_v.reshape(S, D),
        B_shift_k.T, B_ssm_k, B_ssm_D,
        _DFT,
    )
    return out.reshape(1, S, 2 * D)
```

```python
import jax
import jax.numpy as jnp
import numpy as np
from jax import lax
import jax.experimental.pallas as pl
import jax.experimental.pallas.tpu as pltpu

S = 2048
D = 1024
DH = 32
C = 128
NB = S // C
NG = D // 128
ST = 512
NT = S // ST
UNITS = 2 * (ST // 128) * (D // 128)
MAC_BLOCK = 16
HEAD1 = 4
TAIL1 = 5
HEAD2 = 4
TAIL2 = 8
FIRST_HEAD = 4
FIRST_TAIL = 5
SELF0 = 34
LAG0 = 10
SELF1 = 34
LAG1 = 10
SELF2 = 34
LAG2 = 10
K_ROWS = 256
G_COLS = 256
Q_ROWS = 256
O_ROWS = 256
O_COLS = 128
SPLIT = 2
FIRST_LEAD = 13
FIRST_BATCHES = ((0, (0, 1)), (2 * SPLIT, ()), (FIRST_LEAD, (2, 3)), (FIRST_LEAD + 2 * FIRST_HEAD, (4, 5)), (37, (6, 7)))
EDGES = 2
OUT_EDGES = ((0, 768, 896, D), (0, 896, D), (0, 512, 896, D), tuple(range(0, D + 1, 128)))[EDGES]
HALO = 16

F32 = jnp.float32
BF16 = jnp.bfloat16


def _dft_matrices():
    n = np.arange(C, dtype=np.float64)
    theta = np.pi * (4.0 * np.arange(C, dtype=np.float64) + 1.0) / (2.0 * C)
    plain = theta[:, None] * n[None, :]
    centred = theta[:, None] * (n[None, :] - (C - 1) / 2)
    inv = np.concatenate([np.cos(centred).T[:C // 2], -np.sin(centred).T[:C // 2]], 0) / C
    inv = inv.reshape(C // 16, 8, 2, C // 16, 2, 8).transpose(0, 2, 1, 3, 5, 4).reshape(C, C)
    return np.concatenate(
        [np.cos(plain), -np.sin(plain), np.cos(centred), -np.sin(centred), inv], 0).astype(BF16)


_DFT = _dft_matrices()

_NT_DIMS = (((1,), (1,)), ((), ()))
_TN_DIMS = (((0,), (0,)), ((), ()))


def _packed(*shape):
    return pltpu.VMEM((*shape[:-2], shape[-2] // 2, shape[-1]), jnp.uint32)


def _phi(t):
    return jnp.where(t > 0, t + 1.0, jnp.exp(t)) + 1e-6


def _unpack(words, index):
    return pltpu.unpack_elementwise(words, index=index, packed_dtype=BF16, unpacked_dtype=F32)


def _rows(start, size):
    if isinstance(start, int):
        return pl.ds(start // 2, size // 2)
    return pl.ds(pl.multiple_of(start // 2, 8), size // 2)


def _lanes(g):
    return pl.ds(g * 128 if isinstance(g, int) else pl.multiple_of(g * 128, 128), 128)


def _bf16(words):
    return pltpu.bitcast(words, BF16)


def _words(x):
    return pltpu.bitcast(x.astype(BF16), jnp.uint32)


def _pack(lo, hi):
    return pltpu.pack_elementwise([lo, hi], packed_dtype=BF16).astype(jnp.uint32)


def _riffle(x):
    return jnp.concatenate(
        [_pack(x[i:i + 8], x[i + 8:i + 16]) for i in range(0, x.shape[0], 16)], 0)


def _flip(tile):
    return jnp.take_along_axis(tile, 7 - lax.broadcasted_iota(jnp.int32, (8, 128), 0), axis=0)


class _ConvGroup:
    def __init__(self, g, kb, vb, qb, skb, shift, skip, dft, kv_s, xp, kp, held, z_s, ob):
        self.g, self.kb, self.vb, self.qb, self.skb, self.shift, self.skip = (
            g, kb, vb, qb, skb, shift, skip)
        self.dft, self.kv_s, self.xp, self.kp, self.held, self.z_s, self.ob = (
            dft, kv_s, xp, kp, held, z_s, ob)
        self.prev = None

    def filter_spectrum(self, i):
        blk = jnp.concatenate(
            [_bf16(self.skb[self.g, :, m * C:(m + 1) * C]) for m in range(4 * i, 4 * i + 4)], 0)
        spec = lax.dot_general(_bf16(self.dft[_rows(0, 2 * C), :]), blk, _NT_DIMS,
                               preferred_element_type=F32)
        for j in range(4):
            re = spec[:C, j * 128:(j + 1) * 128]
            im = spec[C:, j * 128:(j + 1) * 128]
            if self.prev is None:
                re = re + self.skip[:, _lanes(self.g)]
                re2, im2 = re, im
            else:
                re2, im2 = re - self.prev[1], im + self.prev[0]
            self.prev = (re, im)
            self.kp[0, 4 * i + j] = re2
            self.kp[1, 4 * i + j] = im2

    def gate_keys(self, lo, hi):
        w = self.shift[:, _lanes(self.g)].astype(F32)
        w0, w1, w2, w3 = (jnp.broadcast_to(w[j:j + 1], (8, 128)) for j in range(4))
        for i in range(lo, hi):
            base = HALO // 2 + 8 * i
            p0 = self.kb[self.g, base:base + 8, :]
            p1 = self.kb[self.g, base - 1:base + 7, :]
            p2 = self.kb[self.g, base - 2:base + 6, :]
            pv = self.vb[self.g, 8 * i:8 * i + 8, :]
            e0, o0 = _unpack(p0, 0), _unpack(p0, 1)
            e1, o1 = _unpack(p1, 0), _unpack(p1, 1)
            o2 = _unpack(p2, 1)
            even = (w0 * e0 + w1 * o1 + w2 * e1 + w3 * o2) * _unpack(pv, 0)
            odd = (w0 * o0 + w1 * e0 + w2 * o1 + w3 * e1) * _unpack(pv, 1)
            self.kv_s[8 * i:8 * i + 8, :] = _pack(even, odd)

    def signal_spectrum(self, i):
        blk = jnp.concatenate(
            [_bf16(self.kv_s[_rows(c * C, C), :]) for c in range(4 * i, 4 * i + 4)], 1)
        spec = jnp.dot(_bf16(self.dft[_rows(2 * C, 2 * C), :]), blk, preferred_element_type=F32)
        for j in range(4):
            self.xp[0, 4 * i + j] = spec[:C, j * 128:(j + 1) * 128]
            self.xp[1, 4 * i + j] = spec[C:, j * 128:(j + 1) * 128]

    def combine(self):
        for r in range(C // 8):
            rows = slice(8 * r, 8 * r + 8)

            def product(outputs, signal, taps, init, subtract):
                ks, acc = {}, dict(init)
                for c in range(outputs[-1] + 1):
                    xc = signal(c)
                    for a in outputs:
                        if a < c:
                            continue
                        if a - c not in ks:
                            ks[a - c] = taps(self.kp[0, a - c, rows, :], self.kp[1, a - c, rows, :])
                        t = xc * ks[a - c]
                        if a not in acc:
                            acc[a] = t
                        else:
                            acc[a] = acc[a] - t if subtract else acc[a] + t
                        yield acc[a]
                return acc

            def keep(part, z):
                for a in z:
                    if r % 2 == 0:
                        self.held[part, a] = z[a]
                    else:
                        self.z_s[part, a, _rows(16 * (r // 2), 16), :] = _pack(self.held[part, a], z[a])

            def x_re(c):
                return self.xp[0, c, rows, :]

            def x_im(c):
                return self.xp[1, c, rows, :]

            for lo in range(0, NB, MAC_BLOCK):
                outputs = range(lo, lo + MAC_BLOCK)
                shared = yield from product(
                    outputs, lambda c: x_re(c) + x_im(c), lambda re, im: re, {}, False)
                keep(1, (yield from product(outputs, x_re, lambda re, im: im - re, shared, False)))
                keep(0, (yield from product(outputs, x_im, lambda re, im: im + re, shared, True)))

    def finish(self, i):
        cos, sin = (
            jnp.dot(_bf16(self.dft[_rows(4 * C + part * C // 2, C // 2), :]),
                    jnp.concatenate([_bf16(self.z_s[part, a]) for a in range(4 * i, 4 * i + 4)], 1),
                    preferred_element_type=F32)
            for part in range(2))
        for j in range(4):
            for u in range(C // 32):
                even = (slice(16 * u, 16 * u + 8), slice(j * 128, (j + 1) * 128))
                odd = (slice(16 * u + 8, 16 * u + 16), slice(j * 128, (j + 1) * 128))
                rows = _rows((4 * i + j) * C + 16 * u, 16)
                q = self.qb[self.g, rows, :]
                self.ob[self.g, rows, :] = _pack(
                    _unpack(q, 0) * (cos[even] + sin[even]), _unpack(q, 1) * (cos[odd] + sin[odd]))
                rows = _rows((4 * i + j + 1) * C - 16 * (u + 1), 16)
                q = _flip(self.qb[self.g, rows, :])
                self.ob[self.g, rows, :] = _flip(_pack(
                    _unpack(q, 0) * (cos[odd] - sin[odd]), _unpack(q, 1) * (cos[even] - sin[even])))


def _run_step(matmuls, conv, conv_done, pace, lead, head, tail, every, lag, before_unit=lambda u: None):
    left = [UNITS]

    def matmul():
        before_unit(UNITS - left[0])
        left[0] -= 1
        return next(matmuls)

    for _ in range(lead):
        matmul()
    tiles = S // 16 // 4
    for i in range(4):
        conv.filter_spectrum(i)
        for u in range(head):
            matmul()
            if u == 0 and i > 0:
                conv.signal_spectrum(i - 1)
            conv.gate_keys(i * tiles + u * tiles // head, i * tiles + (u + 1) * tiles // head)
    matmul()
    conv.signal_spectrum(3)
    products = 3 * (C // 8) * NB * (NB + 1) // 2
    batches = left[0] - tail
    combine = conv.combine()
    for u in range(batches):
        result = matmul()
        if u:
            pace(result[:8, :128])
        recent = []
        for i in range(u * products // batches, (u + 1) * products // batches):
            recent.append(next(combine))
            if len(recent) % every == 0:
                pace(recent[-lag])
    for _ in combine:
        pass
    matmul()
    for i in range(4):
        conv.finish(i)
        conv_done(i)
        if left[0]:
            matmul()
    while left[0]:
        matmul()
    for _ in matmuls:
        pass


def _kernel(x_hbm, wqkv_hbm, wo_hbm, q_hbm, k_hbm, v_hbm, shift_hbm, sk_hbm, d_hbm, dft_hbm,
            out_hbm,
            x_v, w_v, wo_v, wkt, wqt, g_acc, z_acc, m_v, pk_s, o_s, oa,
            kb, vb, qb, skb, shift_v, d_v, skip_s, dft, kv_s, xp, kp, held, z_s, ob, zero,
            sem_x, sem_w, sem_first, sem_b, sem_oa, sem_ob):

    def tile_rows(t):
        return pl.ds(t * ST if isinstance(t, int) else pl.multiple_of(t * ST, ST), ST)

    def x_copy(t):
        return pltpu.make_async_copy(
            x_hbm.at[tile_rows(t), :], x_v.bitcast(BF16).at[tile_rows(t), :], sem_x.at[t])

    def w_copy(j):
        return pltpu.make_async_copy(
            wqkv_hbm.at[:, pl.ds(j * D, D)], w_v.bitcast(BF16).at[j], sem_w.at[j])

    def wo_copy():
        return pltpu.make_async_copy(wo_hbm, wo_v.bitcast(BF16), sem_w.at[1])

    def b_copy(g, i):
        lanes = _lanes(g)
        src, dst = (
            (sk_hbm.at[lanes, :], skb.bitcast(BF16).at[g]),
            (k_hbm.at[:, lanes], kb.bitcast(BF16).at[g, pl.ds(HALO, S), :]),
            (v_hbm.at[:, lanes], vb.bitcast(BF16).at[g]),
            (q_hbm.at[:, lanes], qb.bitcast(BF16).at[g]),
        )[i]
        return pltpu.make_async_copy(src, dst, sem_b.at[g, i])

    def b_copies(g):
        return [b_copy(g, i) for i in range(4)]

    def oa_copy(t, j):
        cols = pl.ds(OUT_EDGES[j], OUT_EDGES[j + 1] - OUT_EDGES[j])
        return pltpu.make_async_copy(
            oa.at[tile_rows(t), cols], out_hbm.at[tile_rows(t), cols], sem_oa.at[t, j])

    def ob_copy(g, i):
        rows = pl.ds(i * S // 4, S // 4)
        return pltpu.make_async_copy(
            ob.bitcast(BF16).at[g, rows, :], out_hbm.at[rows, _lanes(NG + g)], sem_ob.at[g, i])

    def first_batch(b):
        def wk(lo, hi, sem):
            return pltpu.make_async_copy(
                wqkv_hbm.at[:, pl.ds(D + lo * 128, (hi - lo) * 128)],
                w_v.bitcast(BF16).at[1, :, pl.ds(lo * 128, (hi - lo) * 128)], sem_first.at[sem])

        def x(lo, hi, sem):
            rows = pl.ds(lo * 128, (hi - lo) * 128)
            return pltpu.make_async_copy(
                x_hbm.at[rows, :], x_v.bitcast(BF16).at[rows, :], sem_first.at[sem])

        def conv_half(h, sem):
            lanes, span = pl.ds(0, 128), pl.ds(h * S // 2, S // 2)
            return [
                pltpu.make_async_copy(
                    sk_hbm.at[lanes, span], skb.bitcast(BF16).at[0, :, span], sem_first.at[sem]),
                pltpu.make_async_copy(
                    k_hbm.at[span, lanes], kb.bitcast(BF16).at[0, pl.ds(HALO + h * S // 2, S // 2), :],
                    sem_first.at[sem + 1]),
                pltpu.make_async_copy(
                    v_hbm.at[span, lanes], vb.bitcast(BF16).at[0, span, :], sem_first.at[sem + 2]),
            ]

        if b == 0:
            return [wk(0, 2, 0), x(0, SPLIT, 1)]
        if b == 1:
            return [x(SPLIT, ST // 128, 2)]
        if b == 2:
            return [wk(2, 4, 4)] + conv_half(0, 5) + [
                pltpu.make_async_copy(dft_hbm, dft.bitcast(BF16), sem_first.at[13]),
                pltpu.make_async_copy(shift_hbm, shift_v, sem_first.at[14]),
                pltpu.make_async_copy(d_hbm, d_v, sem_first.at[15])]
        if b == 3:
            return conv_half(1, 8) + [wk(4, 6, 11)]
        return [wk(6, 8, 12), b_copy(0, 3)]

    def later_inputs():
        copies = []
        for t, weight in zip(range(1, NT), (w_copy(2), wo_copy(), w_copy(0))):
            copies += [x_copy(t)] + b_copies(t) + [weight]
        for g in range(NT, NG):
            copies += b_copies(g)
        return copies

    def conv(g):
        return _ConvGroup(g, kb, vb, qb, skb, shift_v, skip_s, dft, kv_s, xp, kp, held, z_s, ob)

    def transpose_weight(j, dst, i):
        dst[_rows(i * 128, 128), :] = _words(_bf16(w_v[j, :, i * 128:(i + 1) * 128]).T)

    def pace(tile):
        xp[2, 0, pl.ds(pl.multiple_of(zero[0], 8), 8), :] = tile

    for cp in first_batch(0) + first_batch(1):
        cp.start()
    zero[0] = 0
    for g in range(NG):
        kb[g, 0:HALO // 2, :] = jnp.zeros((HALO // 2, 128), jnp.uint32)

    def pieces(result):
        height, width = result.shape
        for i in range(max(height // 128, 1)):
            for j in range(width // 128):
                yield result[i * 128:, j * 128:]

    def keys(t, first):
        def project(lo, height):
            pk = []
            for n in range(ST // 128):
                xs = _bf16(x_v[_rows(t * ST + n * 128, 128), :])
                pk.append(_phi(lax.dot_general(
                    _bf16(wkt[_rows(lo, height), :]), xs, _NT_DIMS, preferred_element_type=F32)))
                if n == ST // 128 - 1:
                    rows, total = slice(lo, lo + height), sum(pk[1:], pk[0])
                    z_acc[rows, :] = total if first else z_acc[rows, :] + total
                    pk_s[_rows(lo, height), :] = _riffle(jnp.concatenate(pk, 1))
                yield from pieces(pk[-1])

        def accumulate(lo, height):
            width = max(G_COLS, 256 * 128 // height)
            for n in range(D // width):
                rows, cols = slice(lo, lo + height), slice(n * width, (n + 1) * width)
                g = jnp.dot(_bf16(pk_s[_rows(lo, height), :]), _bf16(x_v[_rows(t * ST, ST), cols]),
                            preferred_element_type=F32)
                g_acc[rows, cols] = g if first else g_acc[rows, cols] + g
                yield from list(pieces(g))[::2]

        if first:
            for part in (project, accumulate):
                yield from part(0, K_ROWS)
        starts = range(K_ROWS if first else 0, D, K_ROWS)
        yield from project(starts[0], K_ROWS)
        for lo in starts[1:]:
            yield from project(lo, K_ROWS)
            yield from accumulate(lo - K_ROWS, K_ROWS)
        yield from accumulate(starts[-1], K_ROWS)

    def arrivals(unit):
        for b, (at, chunks) in enumerate(FIRST_BATCHES):
            if unit == at:
                for cp in first_batch(b):
                    cp.wait()
                ahead = first_batch(b + 2) if b + 2 < len(FIRST_BATCHES) else []
                for cp in ahead + (later_inputs() if b + 3 == len(FIRST_BATCHES) else []):
                    cp.start()
                for i in chunks:
                    transpose_weight(1, wkt, i)
                if b == 2:
                    skip_s[...] = d_v[...].astype(F32).reshape(1, D)

    _run_step(keys(0, True), conv(0), lambda i: ob_copy(0, i).start(), pace,
              FIRST_BATCHES[2][0] + 1, FIRST_HEAD, FIRST_TAIL, SELF0, LAG0, arrivals)

    def phase1(t, carry):
        for cp in [x_copy(t)] + b_copies(t):
            cp.wait()
        _run_step(keys(t, False), conv(t), lambda i: ob_copy(t, i).start(), pace, 0, HEAD1, TAIL1, SELF1, LAG1)
        return carry

    lax.fori_loop(1, NT, phase1, 0)

    for cp in (w_copy(2), wo_copy(), w_copy(0)):
        cp.wait()
    same_head = (lax.broadcasted_iota(jnp.int32, (128, 128), 0) // DH
                 == lax.broadcasted_iota(jnp.int32, (128, 128), 1) // DH)
    kvs = []
    for i in range(D // 128):
        blk = slice(i * 128, (i + 1) * 128)
        kv = jnp.dot(g_acc[blk, :].astype(BF16), _bf16(w_v[2, :, blk]), preferred_element_type=F32)
        kvs.append(jnp.where(same_head, kv, 0.0).astype(BF16))
        transpose_weight(0, wqt, i)
    for i in range(D // 128):
        m_v[_rows(i * 128, 128), :] = _words(
            jnp.dot(kvs[i], _bf16(wo_v[_rows(i * 128, 128), :]), preferred_element_type=F32))
    z_acc[...] = jnp.broadcast_to(jnp.sum(z_acc[...], axis=1, keepdims=True), (D, 128))

    def queries(t):
        for n in range(ST // 128):
            xs = _bf16(x_v[_rows(t * ST + n * 128, 128), :])
            for j in range(D // Q_ROWS):
                chans = slice(j * Q_ROWS, (j + 1) * Q_ROWS)
                pq = _phi(lax.dot_general(
                    _bf16(wqt[_rows(j * Q_ROWS, Q_ROWS), :]), xs, _NT_DIMS, preferred_element_type=F32))
                pz = (pq * z_acc[chans, :]).reshape(Q_ROWS // DH, DH, 128)
                den = jnp.sum(pz, axis=1, keepdims=True) + 1e-6
                o = (pq.reshape(Q_ROWS // DH, DH, 128) * (1.0 / den)).reshape(Q_ROWS, 128)
                o_s[_rows(n * 128, 128), chans] = _words(_bf16(_riffle(o)).T)
                yield from pieces(pq)
        for j in range(D // O_COLS):
            cols = slice(j * O_COLS, (j + 1) * O_COLS)
            for n in range(ST // O_ROWS):
                rows = _rows(n * O_ROWS, O_ROWS)
                res = jnp.dot(_bf16(o_s[rows, :]), _bf16(m_v[:, cols]), preferred_element_type=F32)
                oa[pl.ds(pl.multiple_of(t * ST + n * O_ROWS, O_ROWS), O_ROWS), cols] = res.astype(BF16)
                if n == ST // O_ROWS - 1 and cols.stop in OUT_EDGES:
                    oa_copy(t, OUT_EDGES.index(cols.stop) - 1).start()
                yield from pieces(res)

    def phase2(t, carry):
        for cp in b_copies(NT + t):
            cp.wait()
        _run_step(queries(t), conv(NT + t), lambda i: ob_copy(NT + t, i).start(), pace,
                  0, HEAD2, TAIL2, SELF2, LAG2)
        return carry

    lax.fori_loop(0, NT, phase2, 0)
    for g in range(NG):
        for i in range(4):
            ob_copy(g, i).wait()
    for t in range(NT):
        for j in range(len(OUT_EDGES) - 1):
            oa_copy(t, j).wait()


@jax.jit
def pallas_concat_heads__linear_attn_block__ssm_conv_h3__prompt_kernel(
    A_x: jax.Array,
    A_wqkv: jax.Array,
    A_wo: jax.Array,
    B_q: jax.Array,
    B_k: jax.Array,
    B_v: jax.Array,
    B_shift_k: jax.Array,
    B_ssm_k: jax.Array,
    B_ssm_D: jax.Array,
):
    assert A_x.shape == (1, S, D) and B_shift_k.shape == (D, 4) and NG == 2 * NT
    hbm = pl.BlockSpec(memory_space=pl.ANY)
    out = pl.pallas_call(
        _kernel,
        out_shape=jax.ShapeDtypeStruct((S, 2 * D), BF16),
        in_specs=[hbm] * 10,
        out_specs=hbm,
        scratch_shapes=[
            _packed(S, D),
            _packed(3, D, D),
            _packed(D, D),
            _packed(D, D),
            _packed(D, D),
            pltpu.VMEM((D, D), F32),
            pltpu.VMEM((D, 128), F32),
            _packed(D, D),
            _packed(D, ST),
            _packed(ST, D),
            pltpu.VMEM((S, D), BF16),
            _packed(NG, HALO + S, 128),
            _packed(NG, S, 128),
            _packed(NG, S, 128),
            _packed(NG, 128, S),
            pltpu.VMEM((4, D), BF16),
            pltpu.VMEM((D,), BF16),
            pltpu.VMEM((1, D), F32),
            _packed(5 * C, C),
            _packed(S, 128),
            pltpu.VMEM((3, NB, C, 128), F32),
            pltpu.VMEM((2, NB, C, 128), F32),
            pltpu.VMEM((2, NB, 8, 128), F32),
            _packed(2, NB, C, 128),
            _packed(NG, S, 128),
            pltpu.SMEM((1,), jnp.int32),
            pltpu.SemaphoreType.DMA((NT,)),
            pltpu.SemaphoreType.DMA((3,)),
            pltpu.SemaphoreType.DMA((16,)),
            pltpu.SemaphoreType.DMA((NG, 4)),
            pltpu.SemaphoreType.DMA((NT, len(OUT_EDGES) - 1)),
            pltpu.SemaphoreType.DMA((NG, 4)),
        ],
        compiler_params=pltpu.CompilerParams(vmem_limit_bytes=100 * 2**20),
        name="linattn_h3",
    )(
        A_x.reshape(S, D), A_wqkv, A_wo,
        B_q.reshape(S, D), B_k.reshape(S, D), B_v.reshape(S, D),
        B_shift_k.T, B_ssm_k, B_ssm_D,
        _DFT,
    )
    return out.reshape(1, S, 2 * D)
```

```python
from typing import NamedTuple

import jax
import jax.numpy as jnp
import numpy as np
from jax import lax
import jax.experimental.pallas as pl
import jax.experimental.pallas.tpu as pltpu

S = 2048
D = 1024
DH = 32
C = 128
NB = S // C
NG = D // 128
ST = 512
NT = S // ST
ROWS = 256
HALO = 16
UNITS = 2 * (ST // 128) * (D // 128)
OUT_EDGES = (0, 512, 896, D)


class Plan(NamedTuple):
    lead: int
    head: int
    tail: int


FIRST_PLAN, KEYS_PLAN, QUERIES_PLAN = Plan(13, 4, 5), Plan(0, 4, 5), Plan(0, 4, 8)
PACE_EVERY, PACE_LAG = 34, 10
FIRST_BATCHES = ((0, (0, 1)), (4, ()), (FIRST_PLAN.lead, (2, 3)),
                 (FIRST_PLAN.lead + 2 * FIRST_PLAN.head, (4, 5)), (37, (6, 7)))

F32 = jnp.float32
BF16 = jnp.bfloat16


def _dft_matrices():
    n = np.arange(C, dtype=np.float64)
    theta = np.pi * (4.0 * np.arange(C, dtype=np.float64) + 1.0) / (2.0 * C)
    plain = theta[:, None] * n[None, :]
    centred = theta[:, None] * (n[None, :] - (C - 1) / 2)
    inv = np.concatenate([np.cos(centred).T[:C // 2], -np.sin(centred).T[:C // 2]], 0) / C
    inv = inv.reshape(C // 16, 8, 2, C // 16, 2, 8).transpose(0, 2, 1, 3, 5, 4).reshape(C, C)
    return np.concatenate(
        [np.cos(plain), -np.sin(plain), np.cos(centred), -np.sin(centred), inv], 0).astype(BF16)


_DFT = _dft_matrices()

_NT_DIMS = (((1,), (1,)), ((), ()))
_TN_DIMS = (((0,), (0,)), ((), ()))


def _packed(*shape):
    return pltpu.VMEM((*shape[:-2], shape[-2] // 2, shape[-1]), jnp.uint32)


def _phi(t):
    return jnp.where(t > 0, t + 1.0, jnp.exp(t)) + 1e-6


def _unpack(words, index):
    return pltpu.unpack_elementwise(words, index=index, packed_dtype=BF16, unpacked_dtype=F32)


def _rows(start, size):
    if isinstance(start, int):
        return pl.ds(start // 2, size // 2)
    return pl.ds(pl.multiple_of(start // 2, 8), size // 2)


def _lanes(g):
    return pl.ds(g * 128 if isinstance(g, int) else pl.multiple_of(g * 128, 128), 128)


def _bf16(words):
    return pltpu.bitcast(words, BF16)


def _words(x):
    return pltpu.bitcast(x.astype(BF16), jnp.uint32)


def _pack(lo, hi):
    return pltpu.pack_elementwise([lo, hi], packed_dtype=BF16).astype(jnp.uint32)


def _riffle(x):
    return jnp.concatenate(
        [_pack(x[i:i + 8], x[i + 8:i + 16]) for i in range(0, x.shape[0], 16)], 0)


def _flip(tile):
    return jnp.take_along_axis(tile, 7 - lax.broadcasted_iota(jnp.int32, (8, 128), 0), axis=0)


class _ConvGroup:
    def __init__(self, g, kb, vb, qb, skb, shift, skip, dft, kv_s, xp, kp, held, z_s, ob):
        self.g, self.kb, self.vb, self.qb, self.skb, self.shift, self.skip = (
            g, kb, vb, qb, skb, shift, skip)
        self.dft, self.kv_s, self.xp, self.kp, self.held, self.z_s, self.ob = (
            dft, kv_s, xp, kp, held, z_s, ob)
        self.prev = None

    def filter_spectrum(self, i):
        blk = jnp.concatenate(
            [_bf16(self.skb[self.g, :, m * C:(m + 1) * C]) for m in range(4 * i, 4 * i + 4)], 0)
        spec = lax.dot_general(_bf16(self.dft[_rows(0, 2 * C), :]), blk, _NT_DIMS,
                               preferred_element_type=F32)
        for j in range(4):
            re = spec[:C, j * 128:(j + 1) * 128]
            im = spec[C:, j * 128:(j + 1) * 128]
            if self.prev is None:
                re = re + self.skip[:, _lanes(self.g)]
                self.kp[0, 0], self.kp[1, 0] = re, im
            else:
                self.kp[0, 4 * i + j] = re - self.prev[1]
                self.kp[1, 4 * i + j] = im + self.prev[0]
            self.prev = (re, im)

    def gate_keys(self, lo, hi):
        w = self.shift[:, _lanes(self.g)].astype(F32)
        w0, w1, w2, w3 = (jnp.broadcast_to(w[j:j + 1], (8, 128)) for j in range(4))
        for i in range(lo, hi):
            base = HALO // 2 + 8 * i
            p0 = self.kb[self.g, base:base + 8, :]
            p1 = self.kb[self.g, base - 1:base + 7, :]
            p2 = self.kb[self.g, base - 2:base + 6, :]
            pv = self.vb[self.g, 8 * i:8 * i + 8, :]
            e0, o0 = _unpack(p0, 0), _unpack(p0, 1)
            e1, o1 = _unpack(p1, 0), _unpack(p1, 1)
            o2 = _unpack(p2, 1)
            even = (w0 * e0 + w1 * o1 + w2 * e1 + w3 * o2) * _unpack(pv, 0)
            odd = (w0 * o0 + w1 * e0 + w2 * o1 + w3 * e1) * _unpack(pv, 1)
            self.kv_s[8 * i:8 * i + 8, :] = _pack(even, odd)

    def signal_spectrum(self, i):
        blk = jnp.concatenate(
            [_bf16(self.kv_s[_rows(c * C, C), :]) for c in range(4 * i, 4 * i + 4)], 1)
        spec = jnp.dot(_bf16(self.dft[_rows(2 * C, 2 * C), :]), blk, preferred_element_type=F32)
        for j in range(4):
            self.xp[0, 4 * i + j] = spec[:C, j * 128:(j + 1) * 128]
            self.xp[1, 4 * i + j] = spec[C:, j * 128:(j + 1) * 128]

    def combine(self):
        for r in range(C // 8):
            rows = slice(8 * r, 8 * r + 8)

            def product(signal, taps, init, subtract):
                ks, acc = {}, dict(init)
                for c in range(NB):
                    xc = signal(c)
                    for a in range(c, NB):
                        if a - c not in ks:
                            ks[a - c] = taps(self.kp[0, a - c, rows, :], self.kp[1, a - c, rows, :])
                        t = xc * ks[a - c]
                        if a not in acc:
                            acc[a] = t
                        else:
                            acc[a] = acc[a] - t if subtract else acc[a] + t
                        yield acc[a]
                return acc

            def keep(part, z):
                for a in range(NB):
                    if r % 2 == 0:
                        self.held[part, a] = z[a]
                    else:
                        self.z_s[part, a, _rows(16 * (r // 2), 16), :] = _pack(self.held[part, a], z[a])

            def x_re(c):
                return self.xp[0, c, rows, :]

            def x_im(c):
                return self.xp[1, c, rows, :]

            shared = yield from product(lambda c: x_re(c) + x_im(c), lambda re, im: re, {}, False)
            keep(1, (yield from product(x_re, lambda re, im: im - re, shared, False)))
            keep(0, (yield from product(x_im, lambda re, im: im + re, shared, True)))

    def finish(self, i):
        cos, sin = (
            jnp.dot(_bf16(self.dft[_rows(4 * C + part * C // 2, C // 2), :]),
                    jnp.concatenate([_bf16(self.z_s[part, a]) for a in range(4 * i, 4 * i + 4)], 1),
                    preferred_element_type=F32)
            for part in range(2))
        for j in range(4):
            for u in range(C // 32):
                even = (slice(16 * u, 16 * u + 8), slice(j * 128, (j + 1) * 128))
                odd = (slice(16 * u + 8, 16 * u + 16), slice(j * 128, (j + 1) * 128))
                rows = _rows((4 * i + j) * C + 16 * u, 16)
                q = self.qb[self.g, rows, :]
                self.ob[self.g, rows, :] = _pack(
                    _unpack(q, 0) * (cos[even] + sin[even]), _unpack(q, 1) * (cos[odd] + sin[odd]))
                rows = _rows((4 * i + j + 1) * C - 16 * (u + 1), 16)
                q = _flip(self.qb[self.g, rows, :])
                self.ob[self.g, rows, :] = _flip(_pack(
                    _unpack(q, 0) * (cos[odd] - sin[odd]), _unpack(q, 1) * (cos[even] - sin[even])))


def _run_step(matmuls, conv, conv_done, pace, plan, before_unit=lambda unit: None):
    left = [UNITS]

    def matmul():
        before_unit(UNITS - left[0])
        left[0] -= 1
        return next(matmuls)

    for _ in range(plan.lead + (plan.lead > 0)):
        matmul()
    tiles = S // 16 // 4
    for i in range(4):
        conv.filter_spectrum(i)
        for u in range(plan.head):
            matmul()
            if u == 0 and i > 0:
                conv.signal_spectrum(i - 1)
            conv.gate_keys(i * tiles + u * tiles // plan.head, i * tiles + (u + 1) * tiles // plan.head)
    matmul()
    conv.signal_spectrum(3)

    products = 3 * (C // 8) * NB * (NB + 1) // 2
    batches = left[0] - plan.tail
    combine = conv.combine()
    for u in range(batches):
        result = matmul()
        if u:
            pace(result[:8, :128])
        recent = []
        for _ in range(u * products // batches, (u + 1) * products // batches):
            recent.append(next(combine))
            if len(recent) % PACE_EVERY == 0:
                pace(recent[-PACE_LAG])
    for _ in combine:
        pass
    matmul()

    for i in range(4):
        conv.finish(i)
        conv_done(i)
        if left[0]:
            matmul()
    while left[0]:
        matmul()


def _kernel(x_hbm, wqkv_hbm, wo_hbm, q_hbm, k_hbm, v_hbm, shift_hbm, sk_hbm, d_hbm, dft_hbm,
            out_hbm,
            x_v, w_v, wo_v, wkt, wqt, g_acc, z_acc, m_v, pk_s, o_s, oa,
            kb, vb, qb, skb, shift_v, d_v, skip_s, dft, kv_s, xp, kp, held, z_s, ob, zero,
            sem_x, sem_w, sem_first, sem_b, sem_oa, sem_ob):

    def tile_rows(t):
        return pl.ds(t * ST if isinstance(t, int) else pl.multiple_of(t * ST, ST), ST)

    def x_copy(t):
        return pltpu.make_async_copy(
            x_hbm.at[tile_rows(t), :], x_v.bitcast(BF16).at[tile_rows(t), :], sem_x.at[t])

    def w_copy(j):
        return pltpu.make_async_copy(
            wqkv_hbm.at[:, pl.ds(j * D, D)], w_v.bitcast(BF16).at[j], sem_w.at[j])

    def wo_copy():
        return pltpu.make_async_copy(wo_hbm, wo_v.bitcast(BF16), sem_w.at[1])

    def b_copy(g, i):
        lanes = _lanes(g)
        src, dst = (
            (sk_hbm.at[lanes, :], skb.bitcast(BF16).at[g]),
            (k_hbm.at[:, lanes], kb.bitcast(BF16).at[g, pl.ds(HALO, S), :]),
            (v_hbm.at[:, lanes], vb.bitcast(BF16).at[g]),
            (q_hbm.at[:, lanes], qb.bitcast(BF16).at[g]),
        )[i]
        return pltpu.make_async_copy(src, dst, sem_b.at[g, i])

    def b_copies(g):
        return [b_copy(g, i) for i in range(4)]

    def oa_copy(t, j):
        cols = pl.ds(OUT_EDGES[j], OUT_EDGES[j + 1] - OUT_EDGES[j])
        return pltpu.make_async_copy(
            oa.at[tile_rows(t), cols], out_hbm.at[tile_rows(t), cols], sem_oa.at[t, j])

    def ob_copy(g, i):
        rows = pl.ds(i * S // 4, S // 4)
        return pltpu.make_async_copy(
            ob.bitcast(BF16).at[g, rows, :], out_hbm.at[rows, _lanes(NG + g)], sem_ob.at[g, i])

    def first_batch(b):
        def wk(lo, hi, sem):
            return pltpu.make_async_copy(
                wqkv_hbm.at[:, pl.ds(D + lo * 128, (hi - lo) * 128)],
                w_v.bitcast(BF16).at[1, :, pl.ds(lo * 128, (hi - lo) * 128)], sem_first.at[sem])

        def x(lo, hi, sem):
            rows = pl.ds(lo * 128, (hi - lo) * 128)
            return pltpu.make_async_copy(
                x_hbm.at[rows, :], x_v.bitcast(BF16).at[rows, :], sem_first.at[sem])

        def conv_half(h, sem):
            lanes, span = pl.ds(0, 128), pl.ds(h * S // 2, S // 2)
            return [
                pltpu.make_async_copy(
                    sk_hbm.at[lanes, span], skb.bitcast(BF16).at[0, :, span], sem_first.at[sem]),
                pltpu.make_async_copy(
                    k_hbm.at[span, lanes], kb.bitcast(BF16).at[0, pl.ds(HALO + h * S // 2, S // 2), :],
                    sem_first.at[sem + 1]),
                pltpu.make_async_copy(
                    v_hbm.at[span, lanes], vb.bitcast(BF16).at[0, span, :], sem_first.at[sem + 2]),
            ]

        if b == 0:
            return [wk(0, 2, 0), x(0, 2, 1)]
        if b == 1:
            return [x(2, ST // 128, 2)]
        if b == 2:
            return [wk(2, 4, 4)] + conv_half(0, 5) + [
                pltpu.make_async_copy(dft_hbm, dft.bitcast(BF16), sem_first.at[13]),
                pltpu.make_async_copy(shift_hbm, shift_v, sem_first.at[14]),
                pltpu.make_async_copy(d_hbm, d_v, sem_first.at[15])]
        if b == 3:
            return conv_half(1, 8) + [wk(4, 6, 11)]
        return [wk(6, 8, 12), b_copy(0, 3)]

    def later_inputs():
        copies = []
        for t, weight in zip(range(1, NT), (w_copy(2), wo_copy(), w_copy(0))):
            copies += [x_copy(t)] + b_copies(t) + [weight]
        for g in range(NT, NG):
            copies += b_copies(g)
        return copies

    def conv(g):
        return _ConvGroup(g, kb, vb, qb, skb, shift_v, skip_s, dft, kv_s, xp, kp, held, z_s, ob)

    def transpose_weight(j, dst, i):
        dst[_rows(i * 128, 128), :] = _words(_bf16(w_v[j, :, i * 128:(i + 1) * 128]).T)

    def pace(tile):
        xp[2, 0, pl.ds(pl.multiple_of(zero[0], 8), 8), :] = tile

    for cp in first_batch(0) + first_batch(1):
        cp.start()
    zero[0] = 0
    for g in range(NG):
        kb[g, 0:HALO // 2, :] = jnp.zeros((HALO // 2, 128), jnp.uint32)

    def pieces(result, units):
        for i in range(units):
            yield result[i * 128:]

    def keys(t, first):
        def project(lo):
            pk = []
            for n in range(ST // 128):
                xs = _bf16(x_v[_rows(t * ST + n * 128, 128), :])
                pk.append(_phi(lax.dot_general(
                    _bf16(wkt[_rows(lo, ROWS), :]), xs, _NT_DIMS, preferred_element_type=F32)))
                if n == ST // 128 - 1:
                    rows, total = slice(lo, lo + ROWS), sum(pk[1:], pk[0])
                    z_acc[rows, :] = total if first else z_acc[rows, :] + total
                    pk_s[_rows(lo, ROWS), :] = _riffle(jnp.concatenate(pk, 1))
                yield from pieces(pk[-1], ROWS // 128)

        def accumulate(lo):
            for n in range(D // 256):
                rows, cols = slice(lo, lo + ROWS), slice(n * 256, (n + 1) * 256)
                g = jnp.dot(_bf16(pk_s[_rows(lo, ROWS), :]), _bf16(x_v[_rows(t * ST, ST), cols]),
                            preferred_element_type=F32)
                g_acc[rows, cols] = g if first else g_acc[rows, cols] + g
                yield from pieces(g, ROWS // 128)

        if first:
            yield from project(0)
            yield from accumulate(0)
        starts = range(ROWS if first else 0, D, ROWS)
        yield from project(starts[0])
        for lo in starts[1:]:
            yield from project(lo)
            yield from accumulate(lo - ROWS)
        yield from accumulate(starts[-1])

    def arrivals(unit):
        for b, (at, chunks) in enumerate(FIRST_BATCHES):
            if unit == at:
                for cp in first_batch(b):
                    cp.wait()
                ahead = first_batch(b + 2) if b + 2 < len(FIRST_BATCHES) else []
                for cp in ahead + (later_inputs() if b + 3 == len(FIRST_BATCHES) else []):
                    cp.start()
                for i in chunks:
                    transpose_weight(1, wkt, i)
                if b == 2:
                    skip_s[...] = d_v[...].astype(F32).reshape(1, D)

    _run_step(keys(0, True), conv(0), lambda i: ob_copy(0, i).start(), pace, FIRST_PLAN, arrivals)

    def phase1(t, carry):
        for cp in [x_copy(t)] + b_copies(t):
            cp.wait()
        _run_step(keys(t, False), conv(t), lambda i: ob_copy(t, i).start(), pace, KEYS_PLAN)
        return carry

    lax.fori_loop(1, NT, phase1, 0)

    for cp in (w_copy(2), wo_copy(), w_copy(0)):
        cp.wait()
    same_head = (lax.broadcasted_iota(jnp.int32, (128, 128), 0) // DH
                 == lax.broadcasted_iota(jnp.int32, (128, 128), 1) // DH)
    kvs = []
    for i in range(D // 128):
        blk = slice(i * 128, (i + 1) * 128)
        kv = jnp.dot(g_acc[blk, :].astype(BF16), _bf16(w_v[2, :, blk]), preferred_element_type=F32)
        kvs.append(jnp.where(same_head, kv, 0.0).astype(BF16))
        transpose_weight(0, wqt, i)
    for i in range(D // 128):
        m_v[_rows(i * 128, 128), :] = _words(
            jnp.dot(kvs[i], _bf16(wo_v[_rows(i * 128, 128), :]), preferred_element_type=F32))
    z_acc[...] = jnp.broadcast_to(jnp.sum(z_acc[...], axis=1, keepdims=True), (D, 128))

    def queries(t):
        for n in range(ST // 128):
            xs = _bf16(x_v[_rows(t * ST + n * 128, 128), :])
            for j in range(D // ROWS):
                chans = slice(j * ROWS, (j + 1) * ROWS)
                pq = _phi(lax.dot_general(
                    _bf16(wqt[_rows(j * ROWS, ROWS), :]), xs, _NT_DIMS, preferred_element_type=F32))
                pz = (pq * z_acc[chans, :]).reshape(ROWS // DH, DH, 128)
                den = jnp.sum(pz, axis=1, keepdims=True) + 1e-6
                o = (pq.reshape(ROWS // DH, DH, 128) * (1.0 / den)).reshape(ROWS, 128)
                o_s[_rows(n * 128, 128), chans] = _words(_bf16(_riffle(o)).T)
                yield from pieces(pq, ROWS // 128)
        for j in range(D // 128):
            cols = slice(j * 128, (j + 1) * 128)
            for n in range(ST // ROWS):
                rows = _rows(n * ROWS, ROWS)
                res = jnp.dot(_bf16(o_s[rows, :]), _bf16(m_v[:, cols]), preferred_element_type=F32)
                oa[pl.ds(pl.multiple_of(t * ST + n * ROWS, ROWS), ROWS), cols] = res.astype(BF16)
                if n == ST // ROWS - 1 and cols.stop in OUT_EDGES:
                    oa_copy(t, OUT_EDGES.index(cols.stop) - 1).start()
                yield from pieces(res, ROWS // 128)

    def phase2(t, carry):
        for cp in b_copies(NT + t):
            cp.wait()
        _run_step(queries(t), conv(NT + t), lambda i: ob_copy(NT + t, i).start(), pace, QUERIES_PLAN)
        return carry

    lax.fori_loop(0, NT, phase2, 0)
    for g in range(NG):
        for i in range(4):
            ob_copy(g, i).wait()
    for t in range(NT):
        for j in range(len(OUT_EDGES) - 1):
            oa_copy(t, j).wait()


@jax.jit
def pallas_concat_heads__linear_attn_block__ssm_conv_h3__prompt_kernel(
    A_x: jax.Array,
    A_wqkv: jax.Array,
    A_wo: jax.Array,
    B_q: jax.Array,
    B_k: jax.Array,
    B_v: jax.Array,
    B_shift_k: jax.Array,
    B_ssm_k: jax.Array,
    B_ssm_D: jax.Array,
):
    assert A_x.shape == (1, S, D) and B_shift_k.shape == (D, 4) and NG == 2 * NT
    hbm = pl.BlockSpec(memory_space=pl.ANY)
    out = pl.pallas_call(
        _kernel,
        out_shape=jax.ShapeDtypeStruct((S, 2 * D), BF16),
        in_specs=[hbm] * 10,
        out_specs=hbm,
        scratch_shapes=[
            _packed(S, D),
            _packed(3, D, D),
            _packed(D, D),
            _packed(D, D),
            _packed(D, D),
            pltpu.VMEM((D, D), F32),
            pltpu.VMEM((D, 128), F32),
            _packed(D, D),
            _packed(D, ST),
            _packed(ST, D),
            pltpu.VMEM((S, D), BF16),
            _packed(NG, HALO + S, 128),
            _packed(NG, S, 128),
            _packed(NG, S, 128),
            _packed(NG, 128, S),
            pltpu.VMEM((4, D), BF16),
            pltpu.VMEM((D,), BF16),
            pltpu.VMEM((1, D), F32),
            _packed(5 * C, C),
            _packed(S, 128),
            pltpu.VMEM((3, NB, C, 128), F32),
            pltpu.VMEM((2, NB, C, 128), F32),
            pltpu.VMEM((2, NB, 8, 128), F32),
            _packed(2, NB, C, 128),
            _packed(NG, S, 128),
            pltpu.SMEM((1,), jnp.int32),
            pltpu.SemaphoreType.DMA((NT,)),
            pltpu.SemaphoreType.DMA((3,)),
            pltpu.SemaphoreType.DMA((16,)),
            pltpu.SemaphoreType.DMA((NG, 4)),
            pltpu.SemaphoreType.DMA((NT, len(OUT_EDGES) - 1)),
            pltpu.SemaphoreType.DMA((NG, 4)),
        ],
        compiler_params=pltpu.CompilerParams(vmem_limit_bytes=100 * 2**20),
        name="linattn_h3",
    )(
        A_x.reshape(S, D), A_wqkv, A_wo,
        B_q.reshape(S, D), B_k.reshape(S, D), B_v.reshape(S, D),
        B_shift_k.T, B_ssm_k, B_ssm_D,
        _DFT,
    )
    return out.reshape(1, S, 2 * D)
```

```python
from typing import NamedTuple

import jax
import jax.numpy as jnp
import numpy as np
from jax import lax
import jax.experimental.pallas as pl
import jax.experimental.pallas.tpu as pltpu

S = 2048
D = 1024
DH = 32
C = 128
NB = S // C
NG = D // 128
ST = 512
NT = S // ST
ROWS = 256
HALO = 16
UNITS = 2 * (ST // 128) * (D // 128)
OUT_EDGES = (0, 512, 896, D)


class Plan(NamedTuple):
    lead: int
    head: int
    tail: int


FIRST_PLAN, KEYS_PLAN, QUERIES_PLAN = Plan(13, 4, 5), Plan(0, 4, 4), Plan(0, 4, 8)
PACE_EVERY, PACE_LAG = 34, 10
FIRST_BATCHES = ((0, (0, 1)), (4, ()), (FIRST_PLAN.lead, (2, 3)),
                 (FIRST_PLAN.lead + 2 * FIRST_PLAN.head, (4, 5)), (37, (6, 7)))

F32 = jnp.float32
BF16 = jnp.bfloat16


def _dft_matrices():
    n = np.arange(C, dtype=np.float64)
    theta = np.pi * (4.0 * np.arange(C, dtype=np.float64) + 1.0) / (2.0 * C)
    plain = theta[:, None] * n[None, :]
    centred = theta[:, None] * (n[None, :] - (C - 1) / 2)
    inv = np.concatenate([np.cos(centred).T[:C // 2], -np.sin(centred).T[:C // 2]], 0) / C
    centred = centred[:, np.arange(C).reshape(C // 16, 8, 2).transpose(0, 2, 1).reshape(C)]
    return np.concatenate(
        [np.cos(plain), -np.sin(plain), np.cos(centred), -np.sin(centred), inv], 0).astype(BF16)


_DFT = _dft_matrices()

_NT_DIMS = (((1,), (1,)), ((), ()))
_TN_DIMS = (((0,), (0,)), ((), ()))


def _packed(*shape):
    return pltpu.VMEM((*shape[:-2], shape[-2] // 2, shape[-1]), jnp.uint32)


def _phi(t):
    return jnp.where(t > 0, t + 1.0, jnp.exp(t)) + 1e-6


def _even_rows(words):
    return pltpu.bitcast(words << 16, F32)


def _odd_rows(words):
    return pltpu.bitcast(words & np.uint32(0xFFFF0000), F32)


def _rows(start, size):
    if isinstance(start, int):
        return pl.ds(start // 2, size // 2)
    return pl.ds(pl.multiple_of(start // 2, 8), size // 2)


def _lanes(g):
    return pl.ds(g * 128 if isinstance(g, int) else pl.multiple_of(g * 128, 128), 128)


def _bf16(words):
    return pltpu.bitcast(words, BF16)


def _words(x):
    return pltpu.bitcast(x.astype(BF16), jnp.uint32)


def _flip(x):
    order = 7 - lax.broadcasted_iota(jnp.int32, (8, 128), 0)
    return jnp.concatenate(
        [jnp.take_along_axis(x[:, j:j + 128], order, axis=0) for j in range(0, x.shape[1], 128)], 1)


class _ConvGroup:
    def __init__(self, g, kb, vb, qb, skb, shift, skip, dft, kv_s, xp, kp, z_s, ob):
        self.g, self.kb, self.vb, self.qb, self.skb, self.shift, self.skip = (
            g, kb, vb, qb, skb, shift, skip)
        self.dft, self.kv_s, self.xp, self.kp, self.z_s, self.ob = (
            dft, kv_s, xp, kp, z_s, ob)
        self.prev = None

    def filter_spectrum(self, i):
        blk = jnp.concatenate(
            [_bf16(self.skb[self.g, :, m * C:(m + 1) * C]) for m in range(4 * i, 4 * i + 4)], 0)
        spec = lax.dot_general(_bf16(self.dft[_rows(0, 2 * C), :]), blk, _NT_DIMS,
                               preferred_element_type=F32)
        for j in range(4):
            re = spec[:C, j * 128:(j + 1) * 128]
            im = spec[C:, j * 128:(j + 1) * 128]
            if self.prev is None:
                re = re + self.skip[:, _lanes(self.g)]
                self.kp[0, 0], self.kp[1, 0] = re, im
            else:
                self.kp[0, 4 * i + j] = re - self.prev[1]
                self.kp[1, 4 * i + j] = im + self.prev[0]
            self.prev = (re, im)

    def gate_keys(self, lo, hi):
        w = self.shift[:, _lanes(self.g)].astype(F32)
        w0, w1, w2, w3 = (jnp.broadcast_to(w[j:j + 1], (8, 128)) for j in range(4))
        for i in range(lo, hi):
            base = HALO // 2 + 8 * i
            p0 = self.kb[self.g, base:base + 8, :]
            p1 = self.kb[self.g, base - 1:base + 7, :]
            p2 = self.kb[self.g, base - 2:base + 6, :]
            pv = self.vb[self.g, 8 * i:8 * i + 8, :]
            e0, o0 = _even_rows(p0), _odd_rows(p0)
            e1, o1 = _even_rows(p1), _odd_rows(p1)
            o2 = _odd_rows(p2)
            even = (w0 * e0 + w1 * o1 + w2 * e1 + w3 * o2) * _even_rows(pv)
            odd = (w0 * o0 + w1 * e0 + w2 * o1 + w3 * e1) * _odd_rows(pv)
            self.kv_s[_rows(16 * i, 16), :] = _words(jnp.concatenate([even, odd], 0))

    def signal_spectrum(self, i):
        blk = jnp.concatenate(
            [_bf16(self.kv_s[_rows(c * C, C), :]) for c in range(4 * i, 4 * i + 4)], 1)
        spec = jnp.dot(_bf16(self.dft[_rows(2 * C, 2 * C), :]), blk, preferred_element_type=F32)
        for j in range(4):
            self.xp[0, 4 * i + j] = spec[:C, j * 128:(j + 1) * 128]
            self.xp[1, 4 * i + j] = spec[C:, j * 128:(j + 1) * 128]

    def combine(self):
        for r in range(C // 8):
            rows = slice(8 * r, 8 * r + 8)

            def product(signal, taps, init, subtract):
                ks, acc = {}, dict(init)
                for c in range(NB):
                    xc = signal(c)
                    for a in range(c, NB):
                        if a - c not in ks:
                            ks[a - c] = taps(self.kp[0, a - c, rows, :], self.kp[1, a - c, rows, :])
                        t = xc * ks[a - c]
                        if a not in acc:
                            acc[a] = t
                        else:
                            acc[a] = acc[a] - t if subtract else acc[a] + t
                        yield acc[a]
                return acc

            def keep(part, z):
                for a in range(NB):
                    self.z_s[part, a, rows, :] = z[a].astype(BF16)

            def x_re(c):
                return self.xp[0, c, rows, :]

            def x_im(c):
                return self.xp[1, c, rows, :]

            shared = yield from product(lambda c: x_re(c) + x_im(c), lambda re, im: re, {}, False)
            keep(1, (yield from product(x_re, lambda re, im: im - re, shared, False)))
            keep(0, (yield from product(x_im, lambda re, im: im + re, shared, True)))

    def finish(self, i):
        cos, sin = (
            jnp.dot(_bf16(self.dft[_rows(4 * C + part * C // 2, C // 2), :]),
                    jnp.concatenate([self.z_s[part, a] for a in range(4 * i, 4 * i + 4)], 1),
                    preferred_element_type=F32)
            for part in range(2))
        first, last = cos + sin, cos - sin
        y = jnp.concatenate(
            [first] + [_flip(last[n - 8:n]) for n in range(C // 2, 0, -8)], 0)
        for j in range(4):
            a = 4 * i + j
            q = _bf16(self.qb[self.g, _rows(a * C, C), :]).astype(F32)
            self.ob[self.g, a * C:(a + 1) * C, :] = (q * y[:, j * 128:(j + 1) * 128]).astype(BF16)


def _run_step(matmuls, conv, conv_done, pace, plan, before_unit=lambda unit: None):
    left = [UNITS]

    def matmul():
        before_unit(UNITS - left[0])
        left[0] -= 1
        return next(matmuls)

    for _ in range(plan.lead + (plan.lead > 0)):
        matmul()
    tiles = S // 16 // 4
    for i in range(4):
        conv.filter_spectrum(i)
        for u in range(plan.head):
            matmul()
            if u == 0 and i > 0:
                conv.signal_spectrum(i - 1)
            conv.gate_keys(i * tiles + u * tiles // plan.head, i * tiles + (u + 1) * tiles // plan.head)
    matmul()
    conv.signal_spectrum(3)

    products = 3 * (C // 8) * NB * (NB + 1) // 2
    batches = left[0] - plan.tail
    combine = conv.combine()
    for u in range(batches):
        result = matmul()
        if u:
            pace(result[:8, :128])
        recent = []
        for _ in range(u * products // batches, (u + 1) * products // batches):
            recent.append(next(combine))
            if len(recent) % PACE_EVERY == 0:
                pace(recent[-PACE_LAG])
    for _ in combine:
        pass
    matmul()

    for i in range(4):
        conv.finish(i)
        conv_done(i)
        if left[0]:
            matmul()
    while left[0]:
        matmul()


def _kernel(x_hbm, wqkv_hbm, wo_hbm, q_hbm, k_hbm, v_hbm, shift_hbm, sk_hbm, d_hbm, dft_hbm,
            out_hbm,
            x_v, w_v, wo_v, wkt, wqt, g_acc, z_acc, m_v, pk_s, o_s, oa,
            kb, vb, qb, skb, shift_v, d_v, skip_s, dft, kv_s, xp, kp, z_s, ob, zero,
            sem_x, sem_w, sem_first, sem_b, sem_oa, sem_ob):

    def tile_rows(t):
        return pl.ds(t * ST if isinstance(t, int) else pl.multiple_of(t * ST, ST), ST)

    def x_copy(t):
        return pltpu.make_async_copy(
            x_hbm.at[tile_rows(t), :], x_v.bitcast(BF16).at[tile_rows(t), :], sem_x.at[t])

    def w_copy(j):
        return pltpu.make_async_copy(
            wqkv_hbm.at[:, pl.ds(j * D, D)], w_v.bitcast(BF16).at[j], sem_w.at[j])

    def wo_copy():
        return pltpu.make_async_copy(wo_hbm, wo_v.bitcast(BF16), sem_w.at[1])

    def b_copy(g, i):
        lanes = _lanes(g)
        src, dst = (
            (sk_hbm.at[lanes, :], skb.bitcast(BF16).at[g]),
            (k_hbm.at[:, lanes], kb.bitcast(BF16).at[g, pl.ds(HALO, S), :]),
            (v_hbm.at[:, lanes], vb.bitcast(BF16).at[g]),
            (q_hbm.at[:, lanes], qb.bitcast(BF16).at[g]),
        )[i]
        return pltpu.make_async_copy(src, dst, sem_b.at[g, i])

    def b_copies(g):
        return [b_copy(g, i) for i in range(4)]

    def oa_copy(t, j):
        cols = pl.ds(OUT_EDGES[j], OUT_EDGES[j + 1] - OUT_EDGES[j])
        return pltpu.make_async_copy(
            oa.at[tile_rows(t), cols], out_hbm.at[tile_rows(t), cols], sem_oa.at[t, j])

    def ob_copy(g, i):
        rows = pl.ds(i * S // 4, S // 4)
        return pltpu.make_async_copy(
            ob.at[g, rows, :], out_hbm.at[rows, _lanes(NG + g)], sem_ob.at[g, i])

    def first_batch(b):
        def wk(lo, hi, sem):
            return pltpu.make_async_copy(
                wqkv_hbm.at[:, pl.ds(D + lo * 128, (hi - lo) * 128)],
                w_v.bitcast(BF16).at[1, :, pl.ds(lo * 128, (hi - lo) * 128)], sem_first.at[sem])

        def x(lo, hi, sem):
            rows = pl.ds(lo * 128, (hi - lo) * 128)
            return pltpu.make_async_copy(
                x_hbm.at[rows, :], x_v.bitcast(BF16).at[rows, :], sem_first.at[sem])

        def conv_half(h, sem):
            lanes, span = pl.ds(0, 128), pl.ds(h * S // 2, S // 2)
            return [
                pltpu.make_async_copy(
                    sk_hbm.at[lanes, span], skb.bitcast(BF16).at[0, :, span], sem_first.at[sem]),
                pltpu.make_async_copy(
                    k_hbm.at[span, lanes], kb.bitcast(BF16).at[0, pl.ds(HALO + h * S // 2, S // 2), :],
                    sem_first.at[sem + 1]),
                pltpu.make_async_copy(
                    v_hbm.at[span, lanes], vb.bitcast(BF16).at[0, span, :], sem_first.at[sem + 2]),
            ]

        if b == 0:
            return [wk(0, 2, 0), x(0, 2, 1)]
        if b == 1:
            return [x(2, ST // 128, 2)]
        if b == 2:
            return [wk(2, 4, 4)] + conv_half(0, 5) + [
                pltpu.make_async_copy(dft_hbm, dft.bitcast(BF16), sem_first.at[13]),
                pltpu.make_async_copy(shift_hbm, shift_v, sem_first.at[14]),
                pltpu.make_async_copy(d_hbm, d_v, sem_first.at[15])]
        if b == 3:
            return conv_half(1, 8) + [wk(4, 6, 11)]
        return [wk(6, 8, 12), b_copy(0, 3)]

    def later_inputs():
        copies = []
        for t, weight in zip(range(1, NT), (w_copy(2), wo_copy(), w_copy(0))):
            copies += [x_copy(t)] + b_copies(t) + [weight]
        for g in range(NT, NG):
            copies += b_copies(g)
        return copies

    def conv(g):
        return _ConvGroup(g, kb, vb, qb, skb, shift_v, skip_s, dft, kv_s, xp, kp, z_s, ob)

    def transpose_weight(j, dst, i):
        dst[_rows(i * 128, 128), :] = _words(_bf16(w_v[j, :, i * 128:(i + 1) * 128]).T)

    def pace(tile):
        xp[2, 0, pl.ds(pl.multiple_of(zero[0], 8), 8), :] = tile

    for cp in first_batch(0) + first_batch(1):
        cp.start()
    zero[0] = 0
    for g in range(NG):
        kb[g, 0:HALO // 2, :] = jnp.zeros((HALO // 2, 128), jnp.uint32)

    def pieces(result, units):
        for i in range(units):
            yield result[i * 128:]

    def keys(t, first):
        def project(lo):
            pk = []
            for n in range(ST // 128):
                xs = _bf16(x_v[_rows(t * ST + n * 128, 128), :])
                pk.append(_phi(lax.dot_general(
                    _bf16(wkt[_rows(lo, ROWS), :]), xs, _NT_DIMS, preferred_element_type=F32)))
                if n == ST // 128 - 1:
                    rows, total = slice(lo, lo + ROWS), sum(pk[1:], pk[0])
                    z_acc[rows, :] = total if first else z_acc[rows, :] + total
                    pk_s[_rows(lo, ROWS), :] = _words(jnp.concatenate(pk, 1))
                yield from pieces(pk[-1], ROWS // 128)

        def accumulate(lo):
            for n in range(D // 256):
                rows, cols = slice(lo, lo + ROWS), slice(n * 256, (n + 1) * 256)
                g = jnp.dot(_bf16(pk_s[_rows(lo, ROWS), :]), _bf16(x_v[_rows(t * ST, ST), cols]),
                            preferred_element_type=F32)
                g_acc[rows, cols] = g if first else g_acc[rows, cols] + g
                yield from pieces(g, ROWS // 128)

        if first:
            yield from project(0)
            yield from accumulate(0)
        starts = range(ROWS if first else 0, D, ROWS)
        yield from project(starts[0])
        for lo in starts[1:]:
            yield from project(lo)
            yield from accumulate(lo - ROWS)
        yield from accumulate(starts[-1])

    def arrivals(unit):
        for b, (at, chunks) in enumerate(FIRST_BATCHES):
            if unit == at:
                for cp in first_batch(b):
                    cp.wait()
                ahead = first_batch(b + 2) if b + 2 < len(FIRST_BATCHES) else []
                for cp in ahead + (later_inputs() if b + 3 == len(FIRST_BATCHES) else []):
                    cp.start()
                for i in chunks:
                    transpose_weight(1, wkt, i)
                if b == 2:
                    skip_s[...] = d_v[...].astype(F32).reshape(1, D)

    _run_step(keys(0, True), conv(0), lambda i: ob_copy(0, i).start(), pace, FIRST_PLAN, arrivals)

    def phase1(t, carry):
        for cp in [x_copy(t)] + b_copies(t):
            cp.wait()
        _run_step(keys(t, False), conv(t), lambda i: ob_copy(t, i).start(), pace, KEYS_PLAN)
        return carry

    lax.fori_loop(1, NT, phase1, 0)

    for cp in (w_copy(2), wo_copy(), w_copy(0)):
        cp.wait()
    same_head = (lax.broadcasted_iota(jnp.int32, (128, 128), 0) // DH
                 == lax.broadcasted_iota(jnp.int32, (128, 128), 1) // DH)
    kvs = []
    for i in range(D // 128):
        blk = slice(i * 128, (i + 1) * 128)
        kv = jnp.dot(g_acc[blk, :].astype(BF16), _bf16(w_v[2, :, blk]), preferred_element_type=F32)
        kvs.append(jnp.where(same_head, kv, 0.0).astype(BF16))
        transpose_weight(0, wqt, i)
    for i in range(D // 128):
        m_v[_rows(i * 128, 128), :] = _words(
            jnp.dot(kvs[i], _bf16(wo_v[_rows(i * 128, 128), :]), preferred_element_type=F32))
    z_acc[...] = jnp.broadcast_to(jnp.sum(z_acc[...], axis=1, keepdims=True), (D, 128))

    def queries(t):
        for n in range(ST // 128):
            xs = _bf16(x_v[_rows(t * ST + n * 128, 128), :])
            for j in range(D // ROWS):
                chans = slice(j * ROWS, (j + 1) * ROWS)
                pq = _phi(lax.dot_general(
                    _bf16(wqt[_rows(j * ROWS, ROWS), :]), xs, _NT_DIMS, preferred_element_type=F32))
                pz = (pq * z_acc[chans, :]).reshape(ROWS // DH, DH, 128)
                den = jnp.sum(pz, axis=1, keepdims=True) + 1e-6
                o = (pq.reshape(ROWS // DH, DH, 128) * (1.0 / den)).reshape(ROWS, 128)
                o_s[_rows(n * 128, 128), chans] = _words(o.astype(BF16).T)
                yield from pieces(pq, ROWS // 128)
        for j in range(D // 128):
            cols = slice(j * 128, (j + 1) * 128)
            for n in range(ST // ROWS):
                rows = _rows(n * ROWS, ROWS)
                res = jnp.dot(_bf16(o_s[rows, :]), _bf16(m_v[:, cols]), preferred_element_type=F32)
                oa[pl.ds(pl.multiple_of(t * ST + n * ROWS, ROWS), ROWS), cols] = res.astype(BF16)
                if n == ST // ROWS - 1 and cols.stop in OUT_EDGES:
                    oa_copy(t, OUT_EDGES.index(cols.stop) - 1).start()
                yield from pieces(res, ROWS // 128)

    def phase2(t, carry):
        for cp in b_copies(NT + t):
            cp.wait()
        _run_step(queries(t), conv(NT + t), lambda i: ob_copy(NT + t, i).start(), pace, QUERIES_PLAN)
        return carry

    lax.fori_loop(0, NT, phase2, 0)
    for g in range(NG):
        for i in range(4):
            ob_copy(g, i).wait()
    for t in range(NT):
        for j in range(len(OUT_EDGES) - 1):
            oa_copy(t, j).wait()


@jax.jit
def pallas_concat_heads__linear_attn_block__ssm_conv_h3__prompt_kernel(
    A_x: jax.Array,
    A_wqkv: jax.Array,
    A_wo: jax.Array,
    B_q: jax.Array,
    B_k: jax.Array,
    B_v: jax.Array,
    B_shift_k: jax.Array,
    B_ssm_k: jax.Array,
    B_ssm_D: jax.Array,
):
    assert A_x.shape == (1, S, D) and B_shift_k.shape == (D, 4) and NG == 2 * NT
    hbm = pl.BlockSpec(memory_space=pl.ANY)
    out = pl.pallas_call(
        _kernel,
        out_shape=jax.ShapeDtypeStruct((S, 2 * D), BF16),
        in_specs=[hbm] * 10,
        out_specs=hbm,
        scratch_shapes=[
            _packed(S, D),
            _packed(3, D, D),
            _packed(D, D),
            _packed(D, D),
            _packed(D, D),
            pltpu.VMEM((D, D), F32),
            pltpu.VMEM((D, 128), F32),
            _packed(D, D),
            _packed(D, ST),
            _packed(ST, D),
            pltpu.VMEM((S, D), BF16),
            _packed(NG, HALO + S, 128),
            _packed(NG, S, 128),
            _packed(NG, S, 128),
            _packed(NG, 128, S),
            pltpu.VMEM((4, D), BF16),
            pltpu.VMEM((D,), BF16),
            pltpu.VMEM((1, D), F32),
            _packed(5 * C, C),
            _packed(S, 128),
            pltpu.VMEM((3, NB, C, 128), F32),
            pltpu.VMEM((2, NB, C, 128), F32),
            pltpu.VMEM((2, NB, C, 128), BF16),
            pltpu.VMEM((NG, S, 128), BF16),
            pltpu.SMEM((1,), jnp.int32),
            pltpu.SemaphoreType.DMA((NT,)),
            pltpu.SemaphoreType.DMA((3,)),
            pltpu.SemaphoreType.DMA((16,)),
            pltpu.SemaphoreType.DMA((NG, 4)),
            pltpu.SemaphoreType.DMA((NT, len(OUT_EDGES) - 1)),
            pltpu.SemaphoreType.DMA((NG, 4)),
        ],
        compiler_params=pltpu.CompilerParams(vmem_limit_bytes=100 * 2**20),
        name="linattn_h3",
    )(
        A_x.reshape(S, D), A_wqkv, A_wo,
        B_q.reshape(S, D), B_k.reshape(S, D), B_v.reshape(S, D),
        B_shift_k.T, B_ssm_k, B_ssm_D,
        _DFT,
    )
    return out.reshape(1, S, 2 * D)
```

```python
from typing import NamedTuple

import jax
import jax.numpy as jnp
import numpy as np
from jax import lax
import jax.experimental.pallas as pl
import jax.experimental.pallas.tpu as pltpu

S = 2048
D = 1024
DH = 32
C = 128
NB = S // C
NG = D // 128
ST = 512
NT = S // ST
ROWS = 256
HALO = 16
UNITS = 2 * (ST // 128) * (D // 128)
OUT_EDGES = (0, 512, 896, D)


class Plan(NamedTuple):
    lead: int
    head: int
    tail: int


FIRST_PLAN, KEYS_PLAN, QUERIES_PLAN = Plan(13, 4, 5), Plan(0, 4, 4), Plan(0, 4, 8)
PACE_EVERY, PACE_LAG = 34, 10
FIRST_BATCHES = ((0, (0, 1)), (4, ()), (FIRST_PLAN.lead, (2, 3)),
                 (FIRST_PLAN.lead + 2 * FIRST_PLAN.head, (4, 5)), (37, (6, 7)))

F32 = jnp.float32
BF16 = jnp.bfloat16


def _dft_matrices():
    n = np.arange(C, dtype=np.float64)
    theta = np.pi * (4.0 * np.arange(C, dtype=np.float64) + 1.0) / (2.0 * C)
    plain = theta[:, None] * n[None, :]
    centred = theta[:, None] * (n[None, :] - (C - 1) / 2)
    inv = np.concatenate([np.cos(centred).T[:C // 2], -np.sin(centred).T[:C // 2]], 0) / C
    centred = centred[:, np.arange(C).reshape(C // 16, 8, 2).transpose(0, 2, 1).reshape(C)]
    return np.concatenate(
        [np.cos(plain), -np.sin(plain), np.cos(centred), -np.sin(centred), inv], 0).astype(BF16)


_DFT = _dft_matrices()

_NT_DIMS = (((1,), (1,)), ((), ()))


def _packed(*shape):
    return pltpu.VMEM((*shape[:-2], shape[-2] // 2, shape[-1]), jnp.uint32)


def _phi(t):
    return jnp.where(t > 0, t + 1.0, jnp.exp(t)) + 1e-6


def _even_rows(words):
    return pltpu.bitcast(words << 16, F32)


def _odd_rows(words):
    return pltpu.bitcast(words & np.uint32(0xFFFF0000), F32)


def _rows(start, size):
    if isinstance(start, int):
        return pl.ds(start // 2, size // 2)
    return pl.ds(pl.multiple_of(start // 2, 8), size // 2)


def _lanes(g):
    return pl.ds(g * 128 if isinstance(g, int) else pl.multiple_of(g * 128, 128), 128)


def _bf16(words):
    return pltpu.bitcast(words, BF16)


def _words(x):
    return pltpu.bitcast(x.astype(BF16), jnp.uint32)


def _flip(x):
    order = 7 - lax.broadcasted_iota(jnp.int32, (8, 128), 0)
    return jnp.concatenate(
        [jnp.take_along_axis(x[:, j:j + 128], order, axis=0) for j in range(0, x.shape[1], 128)], 1)


class _ConvGroup:
    def __init__(self, g, kb, vb, qb, skb, shift, skip, dft, kv_s, xp, kp, z_s, ob):
        self.g, self.kb, self.vb, self.qb, self.skb, self.shift, self.skip = (
            g, kb, vb, qb, skb, shift, skip)
        self.dft, self.kv_s, self.xp, self.kp, self.z_s, self.ob = (
            dft, kv_s, xp, kp, z_s, ob)
        self.prev = None

    def filter_spectrum(self, i):
        blk = jnp.concatenate(
            [_bf16(self.skb[self.g, :, m * C:(m + 1) * C]) for m in range(4 * i, 4 * i + 4)], 0)
        spec = lax.dot_general(_bf16(self.dft[_rows(0, 2 * C), :]), blk, _NT_DIMS,
                               preferred_element_type=F32)
        for j in range(4):
            re = spec[:C, j * 128:(j + 1) * 128]
            im = spec[C:, j * 128:(j + 1) * 128]
            if self.prev is None:
                re = re + self.skip[:, _lanes(self.g)]
                self.kp[0, 0], self.kp[1, 0] = re, im
            else:
                self.kp[0, 4 * i + j] = re - self.prev[1]
                self.kp[1, 4 * i + j] = im + self.prev[0]
            self.prev = (re, im)

    def gate_keys(self, lo, hi):
        w = self.shift[:, _lanes(self.g)].astype(F32)
        w0, w1, w2, w3 = (jnp.broadcast_to(w[j:j + 1], (8, 128)) for j in range(4))
        for i in range(lo, hi):
            base = HALO // 2 + 8 * i
            p0 = self.kb[self.g, base:base + 8, :]
            p1 = self.kb[self.g, base - 1:base + 7, :]
            p2 = self.kb[self.g, base - 2:base + 6, :]
            pv = self.vb[self.g, 8 * i:8 * i + 8, :]
            e0, o0 = _even_rows(p0), _odd_rows(p0)
            e1, o1 = _even_rows(p1), _odd_rows(p1)
            o2 = _odd_rows(p2)
            even = (w0 * e0 + w1 * o1 + w2 * e1 + w3 * o2) * _even_rows(pv)
            odd = (w0 * o0 + w1 * e0 + w2 * o1 + w3 * e1) * _odd_rows(pv)
            self.kv_s[_rows(16 * i, 16), :] = _words(jnp.concatenate([even, odd], 0))

    def signal_spectrum(self, i):
        blk = jnp.concatenate(
            [_bf16(self.kv_s[_rows(c * C, C), :]) for c in range(4 * i, 4 * i + 4)], 1)
        spec = jnp.dot(_bf16(self.dft[_rows(2 * C, 2 * C), :]), blk, preferred_element_type=F32)
        for j in range(4):
            self.xp[0, 4 * i + j] = spec[:C, j * 128:(j + 1) * 128]
            self.xp[1, 4 * i + j] = spec[C:, j * 128:(j + 1) * 128]

    def combine(self):
        for r in range(C // 8):
            rows = slice(8 * r, 8 * r + 8)

            def product(signal, taps, init, subtract):
                ks, acc = {}, dict(init)
                for c in range(NB):
                    xc = signal(c)
                    for a in range(c, NB):
                        if a - c not in ks:
                            ks[a - c] = taps(self.kp[0, a - c, rows, :], self.kp[1, a - c, rows, :])
                        t = xc * ks[a - c]
                        if a not in acc:
                            acc[a] = t
                        else:
                            acc[a] = acc[a] - t if subtract else acc[a] + t
                        yield acc[a]
                return acc

            def keep(part, z):
                for a in range(NB):
                    self.z_s[part, a, rows, :] = z[a].astype(BF16)

            def x_re(c):
                return self.xp[0, c, rows, :]

            def x_im(c):
                return self.xp[1, c, rows, :]

            shared = yield from product(lambda c: x_re(c) + x_im(c), lambda re, im: re, {}, False)
            keep(1, (yield from product(x_re, lambda re, im: im - re, shared, False)))
            keep(0, (yield from product(x_im, lambda re, im: im + re, shared, True)))

    def finish(self, i):
        cos, sin = (
            jnp.dot(_bf16(self.dft[_rows(4 * C + part * C // 2, C // 2), :]),
                    jnp.concatenate([self.z_s[part, a] for a in range(4 * i, 4 * i + 4)], 1),
                    preferred_element_type=F32)
            for part in range(2))
        first, last = cos + sin, cos - sin
        y = jnp.concatenate(
            [first] + [_flip(last[n - 8:n]) for n in range(C // 2, 0, -8)], 0)
        for j in range(4):
            a = 4 * i + j
            q = _bf16(self.qb[self.g, _rows(a * C, C), :]).astype(F32)
            self.ob[self.g, a * C:(a + 1) * C, :] = (q * y[:, j * 128:(j + 1) * 128]).astype(BF16)


def _run_step(matmuls, conv, conv_done, pace, plan, before_unit=lambda unit: None):
    left = [UNITS]

    def matmul():
        before_unit(UNITS - left[0])
        left[0] -= 1
        return next(matmuls)

    for _ in range(plan.lead + (plan.lead > 0)):
        matmul()
    tiles = S // 16 // 4
    for i in range(4):
        conv.filter_spectrum(i)
        for u in range(plan.head):
            matmul()
            if u == 0 and i > 0:
                conv.signal_spectrum(i - 1)
            conv.gate_keys(i * tiles + u * tiles // plan.head, i * tiles + (u + 1) * tiles // plan.head)
    matmul()
    conv.signal_spectrum(3)

    products = 3 * (C // 8) * NB * (NB + 1) // 2
    batches = left[0] - plan.tail
    combine = conv.combine()
    for u in range(batches):
        result = matmul()
        if u:
            pace(result[:8, :128])
        recent = []
        for _ in range(u * products // batches, (u + 1) * products // batches):
            recent.append(next(combine))
            if len(recent) % PACE_EVERY == 0:
                pace(recent[-PACE_LAG])
    for _ in combine:
        pass
    matmul()

    for i in range(4):
        conv.finish(i)
        conv_done(i)
        if left[0]:
            matmul()
    while left[0]:
        matmul()


def _kernel(x_hbm, wqkv_hbm, wo_hbm, q_hbm, k_hbm, v_hbm, shift_hbm, sk_hbm, d_hbm, dft_hbm,
            out_hbm,
            x_v, w_v, wo_v, wkt, wqt, g_acc, z_acc, m_v, pk_s, o_s, oa,
            kb, vb, qb, skb, shift_v, d_v, skip_s, dft, kv_s, xp, kp, z_s, ob, zero,
            sem_x, sem_w, sem_first, sem_b, sem_oa, sem_ob):

    x_hbm, wqkv_hbm, wo_hbm, q_hbm, k_hbm, v_hbm, sk_hbm, dft_hbm = (
        ref.bitcast(jnp.uint32)
        for ref in (x_hbm, wqkv_hbm, wo_hbm, q_hbm, k_hbm, v_hbm, sk_hbm, dft_hbm))

    def x_copy(t):
        rows = _rows(t * ST, ST)
        return pltpu.make_async_copy(x_hbm.at[rows, :], x_v.at[rows, :], sem_x.at[t])

    def w_copy(j):
        return pltpu.make_async_copy(wqkv_hbm.at[:, pl.ds(j * D, D)], w_v.at[j], sem_w.at[j])

    def wo_copy():
        return pltpu.make_async_copy(wo_hbm, wo_v, sem_w.at[1])

    def b_copy(g, i):
        src, dst = (
            (sk_hbm.at[_rows(g * 128, 128), :], skb.at[g]),
            (k_hbm.at[:, _lanes(g)], kb.at[g, _rows(HALO, S), :]),
            (v_hbm.at[:, _lanes(g)], vb.at[g]),
            (q_hbm.at[:, _lanes(g)], qb.at[g]),
        )[i]
        return pltpu.make_async_copy(src, dst, sem_b.at[g, i])

    def b_copies(g):
        return [b_copy(g, i) for i in range(4)]

    def oa_copy(t, j):
        cols = pl.ds(OUT_EDGES[j], OUT_EDGES[j + 1] - OUT_EDGES[j])
        rows = pl.ds(t * ST if isinstance(t, int) else pl.multiple_of(t * ST, ST), ST)
        return pltpu.make_async_copy(oa.at[rows, cols], out_hbm.at[rows, cols], sem_oa.at[t, j])

    def ob_copy(g, i):
        rows = pl.ds(i * S // 4, S // 4)
        return pltpu.make_async_copy(
            ob.at[g, rows, :], out_hbm.at[rows, _lanes(NG + g)], sem_ob.at[g, i])

    def first_batch(b):
        def wk(lo, hi, sem):
            return pltpu.make_async_copy(
                wqkv_hbm.at[:, pl.ds(D + lo * 128, (hi - lo) * 128)],
                w_v.at[1, :, pl.ds(lo * 128, (hi - lo) * 128)], sem_first.at[sem])

        def x(lo, hi, sem):
            rows = _rows(lo * 128, (hi - lo) * 128)
            return pltpu.make_async_copy(x_hbm.at[rows, :], x_v.at[rows, :], sem_first.at[sem])

        def conv_half(h, sem):
            cols, rows = pl.ds(h * S // 2, S // 2), _rows(h * S // 2, S // 2)
            return [
                pltpu.make_async_copy(
                    sk_hbm.at[_rows(0, 128), cols], skb.at[0, :, cols], sem_first.at[sem]),
                pltpu.make_async_copy(
                    k_hbm.at[rows, _lanes(0)], kb.at[0, _rows(HALO + h * S // 2, S // 2), :],
                    sem_first.at[sem + 1]),
                pltpu.make_async_copy(
                    v_hbm.at[rows, _lanes(0)], vb.at[0, rows, :], sem_first.at[sem + 2]),
            ]

        if b == 0:
            return [wk(0, 2, 0), x(0, 2, 1)]
        if b == 1:
            return [x(2, ST // 128, 2)]
        if b == 2:
            return [wk(2, 4, 4)] + conv_half(0, 5) + [
                pltpu.make_async_copy(dft_hbm, dft, sem_first.at[13]),
                pltpu.make_async_copy(shift_hbm, shift_v, sem_first.at[14]),
                pltpu.make_async_copy(d_hbm, d_v, sem_first.at[15])]
        if b == 3:
            return conv_half(1, 8) + [wk(4, 6, 11)]
        return [wk(6, 8, 12), b_copy(0, 3)]

    def later_inputs():
        copies = []
        for t, weight in zip(range(1, NT), (w_copy(2), wo_copy(), w_copy(0))):
            copies += [x_copy(t)] + b_copies(t) + [weight]
        for g in range(NT, NG):
            copies += b_copies(g)
        return copies

    def conv(g):
        return _ConvGroup(g, kb, vb, qb, skb, shift_v, skip_s, dft, kv_s, xp, kp, z_s, ob)

    def transpose_weight(j, dst, i):
        dst[_rows(i * 128, 128), :] = _words(_bf16(w_v[j, :, i * 128:(i + 1) * 128]).T)

    def pace(tile):
        xp[2, 0, pl.ds(pl.multiple_of(zero[0], 8), 8), :] = tile

    for cp in first_batch(0) + first_batch(1):
        cp.start()
    zero[0] = 0
    for g in range(NG):
        kb[g, 0:HALO // 2, :] = jnp.zeros((HALO // 2, 128), jnp.uint32)

    def pieces(result, units):
        for i in range(units):
            yield result[i * 128:]

    def keys(t, first):
        def project(lo):
            pk = []
            for n in range(ST // 128):
                xs = _bf16(x_v[_rows(t * ST + n * 128, 128), :])
                pk.append(_phi(lax.dot_general(
                    _bf16(wkt[_rows(lo, ROWS), :]), xs, _NT_DIMS, preferred_element_type=F32)))
                if n == ST // 128 - 1:
                    rows, total = slice(lo, lo + ROWS), sum(pk[1:], pk[0])
                    z_acc[rows, :] = total if first else z_acc[rows, :] + total
                    pk_s[_rows(lo, ROWS), :] = _words(jnp.concatenate(pk, 1))
                yield from pieces(pk[-1], ROWS // 128)

        def accumulate(lo):
            for n in range(D // 256):
                rows, cols = slice(lo, lo + ROWS), slice(n * 256, (n + 1) * 256)
                g = jnp.dot(_bf16(pk_s[_rows(lo, ROWS), :]), _bf16(x_v[_rows(t * ST, ST), cols]),
                            preferred_element_type=F32)
                g_acc[rows, cols] = g if first else g_acc[rows, cols] + g
                yield from pieces(g, ROWS // 128)

        if first:
            yield from project(0)
            yield from accumulate(0)
        starts = range(ROWS if first else 0, D, ROWS)
        yield from project(starts[0])
        for lo in starts[1:]:
            yield from project(lo)
            yield from accumulate(lo - ROWS)
        yield from accumulate(starts[-1])

    def arrivals(unit):
        for b, (at, chunks) in enumerate(FIRST_BATCHES):
            if unit == at:
                for cp in first_batch(b):
                    cp.wait()
                ahead = first_batch(b + 2) if b + 2 < len(FIRST_BATCHES) else []
                for cp in ahead + (later_inputs() if b + 3 == len(FIRST_BATCHES) else []):
                    cp.start()
                for i in chunks:
                    transpose_weight(1, wkt, i)
                if b == 2:
                    skip_s[...] = d_v[...].astype(F32).reshape(1, D)

    _run_step(keys(0, True), conv(0), lambda i: ob_copy(0, i).start(), pace, FIRST_PLAN, arrivals)

    def phase1(t, carry):
        for cp in [x_copy(t)] + b_copies(t):
            cp.wait()
        _run_step(keys(t, False), conv(t), lambda i: ob_copy(t, i).start(), pace, KEYS_PLAN)
        return carry

    lax.fori_loop(1, NT, phase1, 0)

    for cp in (w_copy(2), wo_copy(), w_copy(0)):
        cp.wait()
    same_head = (lax.broadcasted_iota(jnp.int32, (128, 128), 0) // DH
                 == lax.broadcasted_iota(jnp.int32, (128, 128), 1) // DH)
    kvs = []
    for i in range(D // 128):
        blk = slice(i * 128, (i + 1) * 128)
        kv = jnp.dot(g_acc[blk, :].astype(BF16), _bf16(w_v[2, :, blk]), preferred_element_type=F32)
        kvs.append(jnp.where(same_head, kv, 0.0).astype(BF16))
        transpose_weight(0, wqt, i)
    for i in range(D // 128):
        m_v[_rows(i * 128, 128), :] = _words(
            jnp.dot(kvs[i], _bf16(wo_v[_rows(i * 128, 128), :]), preferred_element_type=F32))
    z_acc[...] = jnp.broadcast_to(jnp.sum(z_acc[...], axis=1, keepdims=True), (D, 128))

    def queries(t):
        for n in range(ST // 128):
            xs = _bf16(x_v[_rows(t * ST + n * 128, 128), :])
            for j in range(D // ROWS):
                chans = slice(j * ROWS, (j + 1) * ROWS)
                pq = _phi(lax.dot_general(
                    _bf16(wqt[_rows(j * ROWS, ROWS), :]), xs, _NT_DIMS, preferred_element_type=F32))
                pz = (pq * z_acc[chans, :]).reshape(ROWS // DH, DH, 128)
                den = jnp.sum(pz, axis=1, keepdims=True) + 1e-6
                o = (pq.reshape(ROWS // DH, DH, 128) * (1.0 / den)).reshape(ROWS, 128)
                o_s[_rows(n * 128, 128), chans] = _words(o.astype(BF16).T)
                yield from pieces(pq, ROWS // 128)
        for j in range(D // 128):
            cols = slice(j * 128, (j + 1) * 128)
            for n in range(ST // ROWS):
                rows = _rows(n * ROWS, ROWS)
                res = jnp.dot(_bf16(o_s[rows, :]), _bf16(m_v[:, cols]), preferred_element_type=F32)
                oa[pl.ds(pl.multiple_of(t * ST + n * ROWS, ROWS), ROWS), cols] = res.astype(BF16)
                if n == ST // ROWS - 1 and cols.stop in OUT_EDGES:
                    oa_copy(t, OUT_EDGES.index(cols.stop) - 1).start()
                yield from pieces(res, ROWS // 128)

    def phase2(t, carry):
        for cp in b_copies(NT + t):
            cp.wait()
        _run_step(queries(t), conv(NT + t), lambda i: ob_copy(NT + t, i).start(), pace, QUERIES_PLAN)
        return carry

    lax.fori_loop(0, NT, phase2, 0)
    for g in range(NG):
        for i in range(4):
            ob_copy(g, i).wait()
    for t in range(NT):
        for j in range(len(OUT_EDGES) - 1):
            oa_copy(t, j).wait()


@jax.jit
def pallas_concat_heads__linear_attn_block__ssm_conv_h3__prompt_kernel(
    A_x: jax.Array,
    A_wqkv: jax.Array,
    A_wo: jax.Array,
    B_q: jax.Array,
    B_k: jax.Array,
    B_v: jax.Array,
    B_shift_k: jax.Array,
    B_ssm_k: jax.Array,
    B_ssm_D: jax.Array,
):
    assert A_x.shape == (1, S, D) and B_shift_k.shape == (D, 4) and NG == 2 * NT
    hbm = pl.BlockSpec(memory_space=pl.ANY)
    out = pl.pallas_call(
        _kernel,
        out_shape=jax.ShapeDtypeStruct((S, 2 * D), BF16),
        in_specs=[hbm] * 10,
        out_specs=hbm,
        scratch_shapes=[
            _packed(S, D),
            _packed(3, D, D),
            _packed(D, D),
            _packed(D, D),
            _packed(D, D),
            pltpu.VMEM((D, D), F32),
            pltpu.VMEM((D, 128), F32),
            _packed(D, D),
            _packed(D, ST),
            _packed(ST, D),
            pltpu.VMEM((S, D), BF16),
            _packed(NG, HALO + S, 128),
            _packed(NG, S, 128),
            _packed(NG, S, 128),
            _packed(NG, 128, S),
            pltpu.VMEM((4, D), BF16),
            pltpu.VMEM((D,), BF16),
            pltpu.VMEM((1, D), F32),
            _packed(5 * C, C),
            _packed(S, 128),
            pltpu.VMEM((3, NB, C, 128), F32),
            pltpu.VMEM((2, NB, C, 128), F32),
            pltpu.VMEM((2, NB, C, 128), BF16),
            pltpu.VMEM((NG, S, 128), BF16),
            pltpu.SMEM((1,), jnp.int32),
            pltpu.SemaphoreType.DMA((NT,)),
            pltpu.SemaphoreType.DMA((3,)),
            pltpu.SemaphoreType.DMA((16,)),
            pltpu.SemaphoreType.DMA((NG, 4)),
            pltpu.SemaphoreType.DMA((NT, len(OUT_EDGES) - 1)),
            pltpu.SemaphoreType.DMA((NG, 4)),
        ],
        compiler_params=pltpu.CompilerParams(vmem_limit_bytes=100 * 2**20),
        name="linattn_h3",
    )(
        A_x.reshape(S, D), A_wqkv, A_wo,
        B_q.reshape(S, D), B_k.reshape(S, D), B_v.reshape(S, D),
        B_shift_k.T, B_ssm_k, B_ssm_D,
        _DFT,
    )
    return out.reshape(1, S, 2 * D)
```

```python
from typing import NamedTuple

import jax
import jax.numpy as jnp
import numpy as np
from jax import lax
import jax.experimental.pallas as pl
import jax.experimental.pallas.tpu as pltpu

S = 2048
D = 1024
DH = 32
C = 128
NB = S // C
NG = D // 128
ST = 512
NT = S // ST
ROWS = 256
HALO = 16
UNITS = 2 * (ST // 128) * (D // 128)
OUT_EDGES = (0, 512, 896, D)


class Plan(NamedTuple):
    lead: int
    head: int
    tail: int
    every: int


FIRST_PLAN, KEYS_PLAN, QUERIES_PLAN = Plan(14, 4, 4, 32), Plan(0, 4, 4, 34), Plan(0, 4, 10, 30)
PACE_LAG = 10
FIRST_BATCHES = ((0, (0, 1)), (4, ()), (FIRST_PLAN.lead, (2, 3)),
                 (FIRST_PLAN.lead + 2 * FIRST_PLAN.head, (4, 5)), (37, (6, 7)))

F32 = jnp.float32
BF16 = jnp.bfloat16


def _dft_matrices():
    n = np.arange(C, dtype=np.float64)
    theta = np.pi * (4.0 * np.arange(C, dtype=np.float64) + 1.0) / (2.0 * C)
    plain = theta[:, None] * n[None, :]
    centred = theta[:, None] * (n[None, :] - (C - 1) / 2)
    inv = np.concatenate([np.cos(centred).T[:C // 2], -np.sin(centred).T[:C // 2]], 0) / C
    centred = centred[:, np.arange(C).reshape(C // 16, 8, 2).transpose(0, 2, 1).reshape(C)]
    return np.concatenate(
        [np.cos(plain), -np.sin(plain), np.cos(centred), -np.sin(centred), inv], 0).astype(BF16)


_DFT = _dft_matrices()

_NT_DIMS = (((1,), (1,)), ((), ()))


def _packed(*shape):
    return pltpu.VMEM((*shape[:-2], shape[-2] // 2, shape[-1]), jnp.uint32)


def _phi(t):
    return jnp.where(t > 0, t + 1.0, jnp.exp(t)) + 1e-6


def _even_rows(words):
    return pltpu.bitcast(words << 16, F32)


def _odd_rows(words):
    return pltpu.bitcast(words & np.uint32(0xFFFF0000), F32)


def _rows(start, size):
    if isinstance(start, int):
        return pl.ds(start // 2, size // 2)
    return pl.ds(pl.multiple_of(start // 2, 8), size // 2)


def _lanes(g):
    return pl.ds(g * 128 if isinstance(g, int) else pl.multiple_of(g * 128, 128), 128)


def _bf16(words):
    return pltpu.bitcast(words, BF16)


def _words(x):
    return pltpu.bitcast(x.astype(BF16), jnp.uint32)


def _flip(x):
    order = 7 - lax.broadcasted_iota(jnp.int32, (8, 128), 0)
    return jnp.concatenate(
        [jnp.take_along_axis(x[:, j:j + 128], order, axis=0) for j in range(0, x.shape[1], 128)], 1)


class _ConvGroup:
    def __init__(self, g, kb, vb, qb, skb, shift, skip, dft, kv_s, xp, kp, z_s, ob):
        self.g, self.kb, self.vb, self.qb, self.skb, self.shift, self.skip = (
            g, kb, vb, qb, skb, shift, skip)
        self.dft, self.kv_s, self.xp, self.kp, self.z_s, self.ob = (
            dft, kv_s, xp, kp, z_s, ob)
        self.prev = None

    def filter_spectrum(self, i):
        blk = jnp.concatenate(
            [_bf16(self.skb[self.g, :, m * C:(m + 1) * C]) for m in range(4 * i, 4 * i + 4)], 0)
        spec = lax.dot_general(_bf16(self.dft[_rows(0, 2 * C), :]), blk, _NT_DIMS,
                               preferred_element_type=F32)
        for j in range(4):
            re = spec[:C, j * 128:(j + 1) * 128]
            im = spec[C:, j * 128:(j + 1) * 128]
            if self.prev is None:
                re = re + self.skip[:, _lanes(self.g)]
                self.kp[0, 0], self.kp[1, 0] = re, im
            else:
                self.kp[0, 4 * i + j] = re - self.prev[1]
                self.kp[1, 4 * i + j] = im + self.prev[0]
            self.prev = (re, im)

    def gate_keys(self, lo, hi):
        w = self.shift[:, _lanes(self.g)].astype(F32)
        w0, w1, w2, w3 = (jnp.broadcast_to(w[j:j + 1], (8, 128)) for j in range(4))
        for i in range(lo, hi):
            base = HALO // 2 + 8 * i
            p0 = self.kb[self.g, base:base + 8, :]
            p1 = self.kb[self.g, base - 1:base + 7, :]
            p2 = self.kb[self.g, base - 2:base + 6, :]
            pv = self.vb[self.g, 8 * i:8 * i + 8, :]
            e0, o0 = _even_rows(p0), _odd_rows(p0)
            e1, o1 = _even_rows(p1), _odd_rows(p1)
            o2 = _odd_rows(p2)
            even = (w0 * e0 + w1 * o1 + w2 * e1 + w3 * o2) * _even_rows(pv)
            odd = (w0 * o0 + w1 * e0 + w2 * o1 + w3 * e1) * _odd_rows(pv)
            self.kv_s[_rows(16 * i, 16), :] = _words(jnp.concatenate([even, odd], 0))

    def signal_spectrum(self, i):
        blk = jnp.concatenate(
            [_bf16(self.kv_s[_rows(c * C, C), :]) for c in range(4 * i, 4 * i + 4)], 1)
        spec = jnp.dot(_bf16(self.dft[_rows(2 * C, 2 * C), :]), blk, preferred_element_type=F32)
        for j in range(4):
            self.xp[0, 4 * i + j] = spec[:C, j * 128:(j + 1) * 128]
            self.xp[1, 4 * i + j] = spec[C:, j * 128:(j + 1) * 128]

    def combine(self):
        for r in range(C // 8):
            rows = slice(8 * r, 8 * r + 8)

            def product(signal, taps, init, subtract):
                ks, acc = {}, dict(init)
                for c in range(NB):
                    xc = signal(c)
                    for a in range(c, NB):
                        if a - c not in ks:
                            ks[a - c] = taps(self.kp[0, a - c, rows, :], self.kp[1, a - c, rows, :])
                        t = xc * ks[a - c]
                        if a not in acc:
                            acc[a] = t
                        else:
                            acc[a] = acc[a] - t if subtract else acc[a] + t
                        yield acc[a]
                return acc

            def keep(part, z):
                for a in range(NB):
                    self.z_s[part, a, rows, :] = z[a].astype(BF16)

            def x_re(c):
                return self.xp[0, c, rows, :]

            def x_im(c):
                return self.xp[1, c, rows, :]

            shared = yield from product(lambda c: x_re(c) + x_im(c), lambda re, im: re, {}, False)
            keep(1, (yield from product(x_re, lambda re, im: im - re, shared, False)))
            keep(0, (yield from product(x_im, lambda re, im: im + re, shared, True)))

    def finish(self, i):
        cos, sin = (
            jnp.dot(_bf16(self.dft[_rows(4 * C + part * C // 2, C // 2), :]),
                    jnp.concatenate([self.z_s[part, a] for a in range(4 * i, 4 * i + 4)], 1),
                    preferred_element_type=F32)
            for part in range(2))
        first, last = cos + sin, cos - sin
        y = jnp.concatenate(
            [first] + [_flip(last[n - 8:n]) for n in range(C // 2, 0, -8)], 0)
        for j in range(4):
            a = 4 * i + j
            q = _bf16(self.qb[self.g, _rows(a * C, C), :]).astype(F32)
            self.ob[self.g, a * C:(a + 1) * C, :] = (q * y[:, j * 128:(j + 1) * 128]).astype(BF16)


def _run_step(matmuls, conv, conv_done, pace, plan, before_unit=lambda unit: None):
    left = [UNITS]

    def matmul():
        before_unit(UNITS - left[0])
        left[0] -= 1
        return next(matmuls)

    for _ in range(plan.lead + (plan.lead > 0)):
        matmul()
    tiles = S // 16 // 4
    for i in range(4):
        conv.filter_spectrum(i)
        for u in range(plan.head):
            matmul()
            if u == 0 and i > 0:
                conv.signal_spectrum(i - 1)
            conv.gate_keys(i * tiles + u * tiles // plan.head, i * tiles + (u + 1) * tiles // plan.head)
    matmul()
    conv.signal_spectrum(3)

    products = 3 * (C // 8) * NB * (NB + 1) // 2
    batches = left[0] - plan.tail
    combine = conv.combine()
    for u in range(batches):
        result = matmul()
        if u:
            pace(result[:8, :128])
        recent = []
        for _ in range(u * products // batches, (u + 1) * products // batches):
            recent.append(next(combine))
            if len(recent) % plan.every == 0:
                pace(recent[-PACE_LAG])
    for _ in combine:
        pass
    matmul()

    for i in range(4):
        conv.finish(i)
        conv_done(i)
        if left[0]:
            matmul()
    while left[0]:
        matmul()


def _kernel(x_hbm, wqkv_hbm, wo_hbm, q_hbm, k_hbm, v_hbm, shift_hbm, sk_hbm, d_hbm, dft_hbm,
            out_hbm,
            x_v, w_v, wo_v, wkt, wqt, g_acc, z_acc, m_v, pk_s, o_s, oa,
            kb, vb, qb, skb, shift_v, d_v, skip_s, dft, kv_s, xp, kp, z_s, ob, zero,
            sem_x, sem_w, sem_first, sem_b, sem_oa, sem_ob):

    x_hbm, wqkv_hbm, wo_hbm, q_hbm, k_hbm, v_hbm, sk_hbm, dft_hbm = (
        ref.bitcast(jnp.uint32)
        for ref in (x_hbm, wqkv_hbm, wo_hbm, q_hbm, k_hbm, v_hbm, sk_hbm, dft_hbm))

    def x_copy(t):
        rows = _rows(t * ST, ST)
        return pltpu.make_async_copy(x_hbm.at[rows, :], x_v.at[rows, :], sem_x.at[t])

    def w_copy(j):
        return pltpu.make_async_copy(wqkv_hbm.at[:, pl.ds(j * D, D)], w_v.at[j], sem_w.at[j])

    def wo_copy():
        return pltpu.make_async_copy(wo_hbm, wo_v, sem_w.at[1])

    def b_copy(g, i):
        src, dst = (
            (sk_hbm.at[_rows(g * 128, 128), :], skb.at[g]),
            (k_hbm.at[:, _lanes(g)], kb.at[g, _rows(HALO, S), :]),
            (v_hbm.at[:, _lanes(g)], vb.at[g]),
            (q_hbm.at[:, _lanes(g)], qb.at[g]),
        )[i]
        return pltpu.make_async_copy(src, dst, sem_b.at[g, i])

    def b_copies(g):
        return [b_copy(g, i) for i in range(4)]

    def oa_copy(t, j):
        cols = pl.ds(OUT_EDGES[j], OUT_EDGES[j + 1] - OUT_EDGES[j])
        rows = pl.ds(t * ST if isinstance(t, int) else pl.multiple_of(t * ST, ST), ST)
        return pltpu.make_async_copy(oa.at[rows, cols], out_hbm.at[rows, cols], sem_oa.at[t, j])

    def ob_copy(g, i):
        rows = pl.ds(i * S // 4, S // 4)
        return pltpu.make_async_copy(
            ob.at[g, rows, :], out_hbm.at[rows, _lanes(NG + g)], sem_ob.at[g, i])

    def first_batch(b):
        def wk(lo, hi, sem):
            return pltpu.make_async_copy(
                wqkv_hbm.at[:, pl.ds(D + lo * 128, (hi - lo) * 128)],
                w_v.at[1, :, pl.ds(lo * 128, (hi - lo) * 128)], sem_first.at[sem])

        def x(lo, hi, sem):
            rows = _rows(lo * 128, (hi - lo) * 128)
            return pltpu.make_async_copy(x_hbm.at[rows, :], x_v.at[rows, :], sem_first.at[sem])

        def conv_half(h, sem):
            cols, rows = pl.ds(h * S // 2, S // 2), _rows(h * S // 2, S // 2)
            return [
                pltpu.make_async_copy(
                    sk_hbm.at[_rows(0, 128), cols], skb.at[0, :, cols], sem_first.at[sem]),
                pltpu.make_async_copy(
                    k_hbm.at[rows, _lanes(0)], kb.at[0, _rows(HALO + h * S // 2, S // 2), :],
                    sem_first.at[sem + 1]),
                pltpu.make_async_copy(
                    v_hbm.at[rows, _lanes(0)], vb.at[0, rows, :], sem_first.at[sem + 2]),
            ]

        if b == 0:
            return [wk(0, 2, 0), x(0, 2, 1)]
        if b == 1:
            return [x(2, ST // 128, 2)]
        if b == 2:
            return [wk(2, 4, 4)] + conv_half(0, 5) + [
                pltpu.make_async_copy(dft_hbm, dft, sem_first.at[13]),
                pltpu.make_async_copy(shift_hbm, shift_v, sem_first.at[14]),
                pltpu.make_async_copy(d_hbm, d_v, sem_first.at[15])]
        if b == 3:
            return conv_half(1, 8) + [wk(4, 6, 11)]
        return [wk(6, 8, 12), b_copy(0, 3)]

    def later_inputs():
        copies = []
        for t, weight in zip(range(1, NT), (w_copy(2), wo_copy(), w_copy(0))):
            copies += [x_copy(t)] + b_copies(t) + [weight]
        for g in range(NT, NG):
            copies += b_copies(g)
        return copies

    def conv(g):
        return _ConvGroup(g, kb, vb, qb, skb, shift_v, skip_s, dft, kv_s, xp, kp, z_s, ob)

    def transpose_weight(j, dst, i):
        dst[_rows(i * 128, 128), :] = _words(_bf16(w_v[j, :, i * 128:(i + 1) * 128]).T)

    def pace(tile):
        xp[2, 0, pl.ds(pl.multiple_of(zero[0], 8), 8), :] = tile

    for cp in first_batch(0) + first_batch(1):
        cp.start()
    zero[0] = 0
    for g in range(NG):
        kb[g, 0:HALO // 2, :] = jnp.zeros((HALO // 2, 128), jnp.uint32)

    def pieces(result, units):
        for i in range(units):
            yield result[i * 128:]

    def keys(t, first):
        def project(lo):
            pk = []
            for n in range(ST // 128):
                xs = _bf16(x_v[_rows(t * ST + n * 128, 128), :])
                pk.append(_phi(lax.dot_general(
                    _bf16(wkt[_rows(lo, ROWS), :]), xs, _NT_DIMS, preferred_element_type=F32)))
                if n == ST // 128 - 1:
                    rows, total = slice(lo, lo + ROWS), sum(pk[1:], pk[0])
                    z_acc[rows, :] = total if first else z_acc[rows, :] + total
                    pk_s[_rows(lo, ROWS), :] = _words(jnp.concatenate(pk, 1))
                yield from pieces(pk[-1], ROWS // 128)

        def accumulate(lo):
            for n in range(D // 256):
                rows, cols = slice(lo, lo + ROWS), slice(n * 256, (n + 1) * 256)
                g = jnp.dot(_bf16(pk_s[_rows(lo, ROWS), :]), _bf16(x_v[_rows(t * ST, ST), cols]),
                            preferred_element_type=F32)
                g_acc[rows, cols] = g if first else g_acc[rows, cols] + g
                yield from pieces(g, ROWS // 128)

        if first:
            yield from project(0)
            yield from accumulate(0)
        starts = range(ROWS if first else 0, D, ROWS)
        yield from project(starts[0])
        for lo in starts[1:]:
            yield from project(lo)
            yield from accumulate(lo - ROWS)
        yield from accumulate(starts[-1])

    def arrivals(unit):
        for b, (at, chunks) in enumerate(FIRST_BATCHES):
            if unit == at:
                for cp in first_batch(b):
                    cp.wait()
                ahead = first_batch(b + 2) if b + 2 < len(FIRST_BATCHES) else []
                for cp in ahead + (later_inputs() if b + 3 == len(FIRST_BATCHES) else []):
                    cp.start()
                for i in chunks:
                    transpose_weight(1, wkt, i)
                if b == 2:
                    skip_s[...] = d_v[...].astype(F32).reshape(1, D)

    _run_step(keys(0, True), conv(0), lambda i: ob_copy(0, i).start(), pace, FIRST_PLAN, arrivals)

    def phase1(t, carry):
        for cp in [x_copy(t)] + b_copies(t):
            cp.wait()
        _run_step(keys(t, False), conv(t), lambda i: ob_copy(t, i).start(), pace, KEYS_PLAN)
        return carry

    lax.fori_loop(1, NT, phase1, 0)

    for cp in (w_copy(2), wo_copy(), w_copy(0)):
        cp.wait()
    same_head = (lax.broadcasted_iota(jnp.int32, (128, 128), 0) // DH
                 == lax.broadcasted_iota(jnp.int32, (128, 128), 1) // DH)
    kvs = []
    for i in range(D // 128):
        blk = slice(i * 128, (i + 1) * 128)
        kv = jnp.dot(g_acc[blk, :].astype(BF16), _bf16(w_v[2, :, blk]), preferred_element_type=F32)
        kvs.append(jnp.where(same_head, kv, 0.0).astype(BF16))
        transpose_weight(0, wqt, i)
    for i in range(D // 128):
        m_v[_rows(i * 128, 128), :] = _words(
            jnp.dot(kvs[i], _bf16(wo_v[_rows(i * 128, 128), :]), preferred_element_type=F32))
    z_acc[...] = jnp.broadcast_to(jnp.sum(z_acc[...], axis=1, keepdims=True), (D, 128))

    def queries(t):
        for n in range(ST // 128):
            xs = _bf16(x_v[_rows(t * ST + n * 128, 128), :])
            for j in range(D // ROWS):
                chans = slice(j * ROWS, (j + 1) * ROWS)
                pq = _phi(lax.dot_general(
                    _bf16(wqt[_rows(j * ROWS, ROWS), :]), xs, _NT_DIMS, preferred_element_type=F32))
                pz = (pq * z_acc[chans, :]).reshape(ROWS // DH, DH, 128)
                den = jnp.sum(pz, axis=1, keepdims=True) + 1e-6
                o = (pq.reshape(ROWS // DH, DH, 128) * (1.0 / den)).reshape(ROWS, 128)
                o_s[_rows(n * 128, 128), chans] = _words(o.astype(BF16).T)
                yield from pieces(pq, ROWS // 128)
        for j in range(D // 128):
            cols = slice(j * 128, (j + 1) * 128)
            for n in range(ST // ROWS):
                rows = _rows(n * ROWS, ROWS)
                res = jnp.dot(_bf16(o_s[rows, :]), _bf16(m_v[:, cols]), preferred_element_type=F32)
                oa[pl.ds(pl.multiple_of(t * ST + n * ROWS, ROWS), ROWS), cols] = res.astype(BF16)
                if n == ST // ROWS - 1 and cols.stop in OUT_EDGES:
                    oa_copy(t, OUT_EDGES.index(cols.stop) - 1).start()
                yield from pieces(res, ROWS // 128)

    def phase2(t, carry):
        for cp in b_copies(NT + t):
            cp.wait()
        _run_step(queries(t), conv(NT + t), lambda i: ob_copy(NT + t, i).start(), pace, QUERIES_PLAN)
        return carry

    lax.fori_loop(0, NT, phase2, 0)
    for g in range(NG):
        for i in range(4):
            ob_copy(g, i).wait()
    for t in range(NT):
        for j in range(len(OUT_EDGES) - 1):
            oa_copy(t, j).wait()


@jax.jit
def pallas_concat_heads__linear_attn_block__ssm_conv_h3__prompt_kernel(
    A_x: jax.Array,
    A_wqkv: jax.Array,
    A_wo: jax.Array,
    B_q: jax.Array,
    B_k: jax.Array,
    B_v: jax.Array,
    B_shift_k: jax.Array,
    B_ssm_k: jax.Array,
    B_ssm_D: jax.Array,
):
    assert A_x.shape == (1, S, D) and B_shift_k.shape == (D, 4) and NG == 2 * NT
    hbm = pl.BlockSpec(memory_space=pl.ANY)
    out = pl.pallas_call(
        _kernel,
        out_shape=jax.ShapeDtypeStruct((S, 2 * D), BF16),
        in_specs=[hbm] * 10,
        out_specs=hbm,
        scratch_shapes=[
            _packed(S, D),
            _packed(3, D, D),
            _packed(D, D),
            _packed(D, D),
            _packed(D, D),
            pltpu.VMEM((D, D), F32),
            pltpu.VMEM((D, 128), F32),
            _packed(D, D),
            _packed(D, ST),
            _packed(ST, D),
            pltpu.VMEM((S, D), BF16),
            _packed(NG, HALO + S, 128),
            _packed(NG, S, 128),
            _packed(NG, S, 128),
            _packed(NG, 128, S),
            pltpu.VMEM((4, D), BF16),
            pltpu.VMEM((D,), BF16),
            pltpu.VMEM((1, D), F32),
            _packed(5 * C, C),
            _packed(S, 128),
            pltpu.VMEM((3, NB, C, 128), F32),
            pltpu.VMEM((2, NB, C, 128), F32),
            pltpu.VMEM((2, NB, C, 128), BF16),
            pltpu.VMEM((NG, S, 128), BF16),
            pltpu.SMEM((1,), jnp.int32),
            pltpu.SemaphoreType.DMA((NT,)),
            pltpu.SemaphoreType.DMA((3,)),
            pltpu.SemaphoreType.DMA((16,)),
            pltpu.SemaphoreType.DMA((NG, 4)),
            pltpu.SemaphoreType.DMA((NT, len(OUT_EDGES) - 1)),
            pltpu.SemaphoreType.DMA((NG, 4)),
        ],
        compiler_params=pltpu.CompilerParams(vmem_limit_bytes=100 * 2**20),
        name="linattn_h3",
    )(
        A_x.reshape(S, D), A_wqkv, A_wo,
        B_q.reshape(S, D), B_k.reshape(S, D), B_v.reshape(S, D),
        B_shift_k.T, B_ssm_k, B_ssm_D,
        _DFT,
    )
    return out.reshape(1, S, 2 * D)
```
